```python
import jax
import jax.numpy as jnp

def _softmax(x, axis=-1):
    return jax.nn.softmax(x, axis=axis)

def _gelu(x):
    return jax.nn.gelu(x, approximate=True)

def _silu(x):
    return jax.nn.silu(x)

def _sigmoid(x):
    return jax.nn.sigmoid(x)

def _layernorm(x, axis=-1, eps=1e-05):
    m = jnp.mean(x, axis=axis, keepdims=True)
    v = jnp.var(x, axis=axis, keepdims=True)
    return (x - m) / jnp.sqrt(v + eps)

def _scatter_add(tgt, idx, src, axis=0):
    return tgt.at[idx].add(src)

def _segment_sum(src, seg, n):
    return jax.ops.segment_sum(src, seg, n)

class _Rng:

    def __init__(self, key):
        self._k = key

    def _next(self):
        self._k, sub = jax.random.split(self._k)
        return sub

    def normal(self, shape):
        return jax.random.normal(self._next(), shape, dtype=jnp.bfloat16)

    def randint(self, lo, hi, shape):
        return jax.random.randint(self._next(), shape, lo, hi, dtype=jnp.int32)

    def uniform(self, shape, lo=0.0, hi=1.0):
        return jax.random.uniform(self._next(), shape, jnp.bfloat16, lo, hi)

    def permutation(self, n):
        return jax.random.permutation(self._next(), n)
kernel_name = 'adaLN_cond__gqa_block_cached__moe_arch_mod__prompt'

def setup_inputs():
    _rng = _Rng(jax.random.key(int.from_bytes(__import__("os").urandom(4), "little")))
    _w = lambda a: (lambda t: t.astype(jnp.bfloat16) if jnp.issubdtype(t.dtype, jnp.floating) else t)(jnp.asarray(a))

    def _A_setup():
        B, Sq, D = (1, 2048, 576)
        Hq, Hkv, Sk, Dh = (32, 16, 2048, 128)
        assert Hq % Hkv == 0, (Hq, Hkv)
        return {'x': _w((lambda *s: _rng.normal(s) * 0.05)(B, Sq, D)), 'k_cache': _w((lambda *s: _rng.normal(s) * 0.05)(B, Hkv, Sk, Dh)), 'v_cache': _w((lambda *s: _rng.normal(s) * 0.05)(B, Hkv, Sk, Dh)), 'wq': _w((lambda *s: _rng.normal(s) * 0.05)(D, Hq * Dh) * D ** (-0.5)), 'wo': _w((lambda *s: _rng.normal(s) * 0.05)(Hq * Dh, D) * (Hq * Dh) ** (-0.5))}
    _A_in = _A_setup()

    def _B_setup():
        B, S, D, F, C = (1, 2048, 576, 4608, 8)
        return {'x': _w((lambda *s: _rng.normal(s) * 0.05)(B, S, D)), 'w_r': _w((lambda *s: _rng.normal(s) * 0.05)(D)), 'w_gate': _w((lambda *s: _rng.normal(s) * 0.05)(D, F)), 'w_up': _w((lambda *s: _rng.normal(s) * 0.05)(D, F)), 'w_down': _w((lambda *s: _rng.normal(s) * 0.05)(F, D))}
    _B_in = _B_setup()
    return {'A_x': _A_in['x'], 'A_k_cache': _A_in['k_cache'], 'A_v_cache': _A_in['v_cache'], 'A_wq': _A_in['wq'], 'A_wo': _A_in['wo'], 'B_x': _B_in['x'], 'B_w_r': _B_in['w_r'], 'B_w_gate': _B_in['w_gate'], 'B_w_up': _B_in['w_up'], 'B_w_down': _B_in['w_down'], 'c': _w((lambda *s: _rng.normal(s) * 0.05)(1, 576)), 'w_mod': _w((lambda *s: _rng.normal(s) * 0.05)(576, 6 * 576) * 576 ** (-0.5))}

def reference(A_x, A_k_cache, A_v_cache, A_wq, A_wo, B_x, B_w_r, B_w_gate, B_w_up, B_w_down, c, w_mod):

    def _A_ref(x, k_cache, v_cache, wq, wo):
        B, Sq, D = x.shape
        Hq, Dh = (32, 128)
        Hkv = k_cache.shape[1]
        rep = Hq // Hkv
        q = (lambda x, *d: x.transpose(*d))((x @ wq).reshape(B, Sq, Hq, Dh), 0, 2, 1, 3)
        k = jnp.repeat(k_cache, rep, axis=1)
        v = jnp.repeat(v_cache, rep, axis=1)
        scores = jnp.einsum('bhqd,bhkd->bhqk', q, k) * Dh ** (-0.5)
        p = _softmax(scores, axis=-1)
        o = jnp.einsum('bhqk,bhkd->bhqd', p, v)
        return (lambda x, *d: x.transpose(*d))(o, 0, 2, 1, 3).reshape(B, Sq, Hq * Dh) @ wo

    def _B_ref(x, w_r, w_gate, w_up, w_down):
        B, S, D = x.shape
        C = 8
        r = x @ w_r
        idx = jnp.argsort(-r, axis=-1)[:, :C]
        idx_e = jnp.repeat(idx.reshape(B, C, 1), D, axis=2)
        x_sel = jnp.take_along_axis(x, idx_e, axis=1)
        g = _silu(x_sel @ w_gate)
        u = x_sel @ w_up
        y = g * u @ w_down
        r_sel = _sigmoid(jnp.take_along_axis(r, idx, axis=1))
        y = y * r_sel.reshape(B, C, 1)
        b_off = (jnp.arange(B) * S).reshape(B, 1)
        flat_idx = (idx + b_off).reshape(B * C)
        zero = (x * 0.0).reshape(B * S, D)
        upd = _scatter_add(zero, flat_idx, y.reshape(B * C, D), axis=0)
        return x + upd.reshape(B, S, D)
    x = A_x
    mod = (_silu(c) @ w_mod).reshape(c.shape[0], 6, 1, -1)
    sa, ca, ga, sb, cb, gb = (mod[:, 0].copy(), mod[:, 1].copy(), mod[:, 2].copy(), mod[:, 3].copy(), mod[:, 4].copy(), mod[:, 5].copy())
    h = _layernorm(x, axis=-1) * (1 + ca) + sa
    x = x + ga * _A_ref(h, A_k_cache, A_v_cache, A_wq, A_wo)
    h = _layernorm(x, axis=-1) * (1 + cb) + sb
    x = x + gb * _B_ref(h, B_w_r, B_w_gate, B_w_up, B_w_down)
    return x
```

```python
import math
import jax
import jax.numpy as jnp
from jax import lax
import jax.experimental.pallas as pl
import jax.experimental.pallas.tpu as pltpu

F32 = jnp.float32
BF16 = jnp.bfloat16
U32 = jnp.uint32
I32 = jnp.int32
EPS = 1e-05
TOPC = 8
NT = (((1,), (1,)), ((), ()))
TQ = 128
KEY_BIAS = 0x20000000


def _pk(x):
    return pltpu.bitcast(x, U32)


def _upk(x):
    return pltpu.bitcast(x, BF16)


def _rb(x):
    return x.astype(BF16).astype(F32)


def _tree(xs, op):
    while len(xs) > 1:
        xs = [op(xs[i], xs[i + 1]) if i + 1 < len(xs) else xs[i] for i in range(0, len(xs), 2)]
    return xs[0]


def _red0(x, op, red, grp):
    n = x.shape[0]
    acc = None
    for t in range(0, n, 8 * grp):
        part = _tree([x[j:j + 8, :] for j in range(t, min(t + 8 * grp, n), 8)], op)
        acc = part if acc is None else op(acc, part)
    return red(acc, axis=0, keepdims=True)


def _ln_t(x):
    d = x.shape[0]
    mu = _red0(x, jnp.add, jnp.sum, 8) * (1.0 / d)
    xc = x - mu
    var = _red0(xc * xc, jnp.add, jnp.sum, 8) * (1.0 / d)
    den = _rb(jnp.sqrt(_rb(_rb(var) + EPS)))
    return xc * (1.0 / den)


def make(scopes=0, gm=4, gs=16):
    def scope(name):
        return jax.named_scope(name) if scopes else jax.named_scope("")

    def kernel(c_ref, wr_ref, xt_hbm, k_hbm, v_hbm, wq_hbm, wot_hbm, wmod_hbm,
               wg_hbm, wu_hbm, wdt_hbm, out_hbm,
               x_sc, wmod_sc, kst, vst, wqst, wost, k_sc, vt_sc, wq_sc, wot_sc,
               h_sc, q_sc, s_sc, acc_sc, mod_sc, modt_sc, w_sc, out_sc, r_sc, xs_sc,
               wg_sc, wu_sc, wdt_sc, sems, xsems, lsems, osems):
        D, S = x_sc.shape
        Hkv, Sk, Dh = k_hbm.shape
        G = 2 * Dh
        nblk = S // TQ
        ngrp = nblk // 2
        GW = 2 * TQ
        qscale = (Dh ** -0.5) * math.log2(math.e)

        def ds(i, n):
            return slice(i * n, (i + 1) * n) if isinstance(i, int) else pl.ds(pl.multiple_of(i * n, n), n)

        def cp_k(g, slot):
            return pltpu.make_async_copy(k_hbm.at[g], kst.at[slot], lsems.at[0, slot])

        def cp_wq(g, slot):
            return pltpu.make_async_copy(wq_hbm.at[:, ds(g, G)], wqst.at[slot], lsems.at[1, slot])

        def cp_v(g, slot):
            return pltpu.make_async_copy(v_hbm.at[g], vst.at[slot], lsems.at[2, slot])

        def cp_wo(g, slot):
            return pltpu.make_async_copy(wot_hbm.at[:, ds(g, G)], wost.at[slot], lsems.at[3, slot])

        def cp_x(j):
            return pltpu.make_async_copy(xt_hbm.at[:, ds(j, GW)], x_sc.at[:, ds(j, GW)], xsems.at[j])

        def cp_out(b):
            return pltpu.make_async_copy(out_sc.at[b], out_hbm.at[:, ds(b, TQ)], osems.at[b])

        moe = [pltpu.make_async_copy(wg_hbm, wg_sc, sems.at[0]),
               pltpu.make_async_copy(wu_hbm, wu_sc, sems.at[1]),
               pltpu.make_async_copy(wdt_hbm, wdt_sc, sems.at[2])]
        cp_m0 = pltpu.make_async_copy(wmod_hbm.at[:, 0:2 * D], wmod_sc.at[:, 0:2 * D], sems.at[3])
        cp_m1 = pltpu.make_async_copy(wmod_hbm.at[:, 2 * D:6 * D], wmod_sc.at[:, 2 * D:6 * D], sems.at[4])

        def ln1(c):
            sa = mod_sc[0:1, 0:D]
            ca1 = mod_sc[1:2, 0:D]
            x = x_sc[:, ds(c, TQ)].astype(F32)
            h = _ln_t(x).T * ca1 + sa
            h_sc[ds(c, TQ // 2), :] = _pk(h.astype(BF16))

        def qproj(c):
            h = _upk(h_sc[ds(c, TQ // 2), :])
            q = jnp.dot(h, _upk(wq_sc[...]), preferred_element_type=F32)
            q = (q * qscale).astype(BF16)
            return jnp.concatenate([q[:, :Dh], q[:, Dh:]], axis=0)

        def qk(c, q, split=False):
            if split:
                st = jnp.concatenate([
                    lax.dot_general(_upk(k_sc[ds(j, Sk // 4), :]), q, NT, preferred_element_type=F32)
                    for j in range(2)], axis=0)
            else:
                st = lax.dot_general(_upk(k_sc[...]), q, NT, preferred_element_type=F32)
            s_sc[c, 0:Sk, :] = st
            s_sc[c, Sk:Sk + 8, :] = jnp.broadcast_to(_red0(st, jnp.maximum, jnp.max, gm), (8, 2 * TQ))

        def pv(c):
            m = s_sc[c, Sk:Sk + 1, :]
            p = jnp.exp2(s_sc[c, 0:Sk, :] - m)
            l = _red0(p, jnp.add, jnp.sum, gs)
            ot = jnp.dot(_upk(vt_sc[...]), p.astype(BF16), preferred_element_type=F32)
            ot = (ot * (1.0 / l)).astype(BF16)
            return jnp.concatenate([ot[:, :TQ], ot[:, TQ:]], axis=0)

        def oproj(c, o2t, split=False):
            if split:
                d = jnp.concatenate([
                    jnp.dot(_upk(wot_sc[ds(j, D // 4), :]), o2t, preferred_element_type=F32)
                    for j in range(2)], axis=0)
            else:
                d = jnp.dot(_upk(wot_sc[...]), o2t, preferred_element_type=F32)
            acc_sc[c] += d

        def post(c):
            ga = modt_sc[0:D, :]
            sb = modt_sc[D:2 * D, :]
            cb1 = modt_sc[2 * D:3 * D, :]
            gb = modt_sc[3 * D:4 * D, :]
            wr = modt_sc[4 * D:5 * D, :]
            x1 = _rb(x_sc[:, ds(c, TQ)].astype(F32) + ga * acc_sc[c])
            h2 = _rb(_ln_t(x1) * cb1 + sb)
            out_sc[c] = (x1 + gb * h2).astype(BF16)
            word = pltpu.bitcast(x1, U32) | (pltpu.bitcast(h2, U32) >> 16)
            w_sc[ds(c, TQ), :] = pltpu.bitcast(word, F32).T
            r_sc[pl.ds(c, 1), :] = _red0(h2 * wr, jnp.add, jnp.sum, 8)

        with scope("prologue"):
            cp_m0.start()
            cp_x(0).start()
            cp_wq(0, 0).start()
            cp_x(1).start()
            cp_k(0, 0).start()
            for j in range(2, ngrp):
                cp_x(j).start()
            acc_sc[...] = jnp.zeros(acc_sc.shape, F32)
            c = c_ref[...].astype(F32)
            sc8 = jnp.broadcast_to((c * jax.nn.sigmoid(c)).astype(BF16), (8, D))
            cp_m0.wait()
            m = _rb(jnp.dot(sc8, wmod_sc[:, 0:2 * D], preferred_element_type=F32))
            mod_sc[0:1, :] = m[0:1, 0:D]
            mod_sc[1:2, :] = _rb(1.0 + m[0:1, D:2 * D])
            cp_x(0).wait()
            cp_x(1).wait()

            def body(i, _):
                ln1(i)
                return 0
            lax.fori_loop(0, 4, body, 0)
            cp_wq(0, 0).wait()
            wq_sc[...] = _pk(wqst[0])
            q_sc[0] = _pk(qproj(0))
            q_sc[1] = _pk(qproj(1))
            cp_k(0, 0).wait()
            k_sc[...] = _pk(kst[0])
            cp_v(0, 0).start()
            for cp in (cp_k(1, 1), cp_wq(1, 1), cp_v(1, 1), cp_wo(0, 1), cp_m1):
                cp.start()

        def fbody(j, _):
            @pl.when(j + 2 < ngrp)
            def _():
                cp_x(j + 2).wait()
            with scope("first"):
                q0 = _upk(q_sc[0])
                q1 = _upk(q_sc[1])
                jn = jnp.minimum(j + 1, ngrp - 1)
                qn0 = qproj(2 * jn)
                qn1 = qproj(2 * jn + 1)
                qk(2 * j, q0)
                qk(2 * j + 1, q1)
                q_sc[0] = _pk(qn0)
                q_sc[1] = _pk(qn1)
                jl = jnp.minimum(j + 2, ngrp - 1)
                ln1(2 * jl)
                ln1(2 * jl + 1)
            return 0
        lax.fori_loop(0, ngrp, fbody, 0)

        with scope("mid"):
            cp_v(0, 0).wait()
            vt_sc[...] = _pk(vst[0].T)
            cp_m1.wait()
            for cp in moe:
                cp.start()
            m = _rb(jnp.dot(sc8, wmod_sc[:, 2 * D:6 * D], preferred_element_type=F32))
            lane = lax.broadcasted_iota(I32, m.shape, 1)
            m = jnp.where((lane >= 2 * D) & (lane < 3 * D), _rb(1.0 + m), m)
            mod_sc[2:3, :] = m[0:1, 3 * D:4 * D]
            modt_sc[0:4 * D, :] = jnp.broadcast_to(m[0:1], (128, 4 * D)).T
            modt_sc[4 * D:5 * D, :] = jnp.broadcast_to(wr_ref[...].astype(F32), (128, D)).T

        def step(i, _):
            slot = i % 2
            for cp in (cp_k(i, slot), cp_wq(i, slot), cp_v(i, slot), cp_wo(i - 1, slot)):
                cp.wait()

            @pl.when(i + 1 < Hkv)
            def _():
                for cp in (cp_k(i + 1, 1 - slot), cp_wq(i + 1, 1 - slot), cp_v(i + 1, 1 - slot)):
                    cp.start()
            cp_wo(i, 1 - slot).start()

            with scope("main"):
                wq_sc[...] = _pk(wqst[slot])
                k_sc[...] = _pk(kst[slot])
                wot_sc[...] = _pk(wost[slot])
                q = None
                for c in range(nblk):
                    last = c == nblk - 1
                    o = pv(c)
                    if c == 0:
                        q = qproj(0)
                    qn = None if last else qproj(c + 1)
                    qk(c, q, split=last)
                    oproj(c, o, split=last)
                    q = qn
                vt_sc[...] = _pk(vst[slot].T)
            return 0
        lax.fori_loop(1, Hkv, step, 0)

        cp_wo(Hkv - 1, Hkv % 2).wait()
        wot_sc[...] = _pk(wost[Hkv % 2])

        def lbody(j, _):
            with scope("last"):
                jp = jnp.maximum(j - 1, 0)
                post(2 * jp)
                post(2 * jp + 1)
                o0 = pv(2 * j)
                o1 = pv(2 * j + 1)
                oproj(2 * j, o0, split=True)
                oproj(2 * j + 1, o1, split=True)
            return 0
        lax.fori_loop(0, ngrp, lbody, 0)

        with scope("tail"):
            post(nblk - 2)
            post(nblk - 1)
            r = _rb(r_sc[...]) + 0.0
            b16 = pltpu.bitcast(r, U32) >> 16
            ordk = jnp.where(b16 >= 0x8000, 0xFFFF - b16, b16 + 0x8000)
            tok = (lax.broadcasted_iota(U32, r.shape, 0) * TQ + lax.broadcasted_iota(U32, r.shape, 1))
            key = pltpu.bitcast((ordk << 11) + (S - 1 - tok) + KEY_BIAS, F32)
            sub = lax.broadcasted_iota(I32, (TOPC, 128), 0)
            top = jnp.zeros((TOPC, 128), F32)
            idxs = []
            for t in range(TOPC):
                mx = jnp.max(jnp.max(key, axis=0, keepdims=True), axis=1, keepdims=True)
                key = jnp.where(key == mx, 0.0, key)
                top = jnp.where(sub == t, mx, top)
                bits = pltpu.bitcast(jnp.broadcast_to(mx, (8, 128)), I32)
                idxs.append(S - 1 - (bits[0, 0] & (S - 1)))
            blks = [ix // TQ for ix in idxs]
            for t in range(TOPC):
                xs_sc[t:t + 1, :] = w_sc[pl.ds(idxs[t], 1), :]
            hit = []
            for b in range(nblk):
                h = blks[0] == b
                for t in range(1, TOPC):
                    h = jnp.logical_or(h, blks[t] == b)
                hit.append(h)

                @pl.when(jnp.logical_not(h))
                def _():
                    cp_out(b).start()
            ordt = (pltpu.bitcast(top, U32) - KEY_BIAS) >> 11
            rsel = pltpu.bitcast(jnp.where(ordt >= 0x8000, ordt - 0x8000, 0xFFFF - ordt) << 16, F32)[:, 0:1]
            words = pltpu.bitcast(xs_sc[...], U32)
            x1s = pltpu.bitcast(words & jnp.uint32(0xFFFF0000), F32)
            h2s = pltpu.bitcast(words << 16, F32)
            xsel = h2s.astype(BF16)
            for cp in moe:
                cp.wait()
            gt = _rb(jnp.dot(xsel, wg_sc[...], preferred_element_type=F32))
            ut = _rb(jnp.dot(xsel, wu_sc[...], preferred_element_type=F32))
            a = (_rb(gt * jax.nn.sigmoid(gt)) * ut).astype(BF16)
            y = _rb(lax.dot_general(a, wdt_sc[...], NT, preferred_element_type=F32))
            y = _rb(y * _rb(jax.nn.sigmoid(rsel)))
            new = x1s + mod_sc[2:3, :] * _rb(h2s + y)
            newt = _pk(jnp.concatenate([new, jnp.zeros((TQ - TOPC, D), F32)], axis=0).T.astype(BF16))
            lane = lax.broadcasted_iota(I32, newt.shape, 1)
            for t in range(TOPC):
                ln = idxs[t] % TQ
                rolled = pltpu.roll(newt, (ln + (TQ - t)) % TQ, 1)
                out_sc[blks[t]] = _upk(jnp.where(lane == ln, rolled, _pk(out_sc[blks[t]])))
            for b in range(nblk):
                @pl.when(hit[b])
                def _():
                    cp_out(b).start()
            for b in range(nblk):
                cp_out(b).wait()

    def fn(A_x, A_k_cache, A_v_cache, A_wq, A_wo, B_x, B_w_r, B_w_gate, B_w_up, B_w_down, c, w_mod):
        B, S, D = A_x.shape
        _, Hkv, Sk, Dh = A_k_cache.shape
        G = A_wq.shape[1] // Hkv
        Fd = B_w_gate.shape[1]
        nblk = S // TQ
        xt = A_x.reshape(S, D).T
        k = A_k_cache.reshape(Hkv, Sk, Dh)
        v = A_v_cache.reshape(Hkv, Sk, Dh)
        anyspec = pl.BlockSpec(memory_space=pl.ANY)
        vm = pl.BlockSpec(memory_space=pltpu.VMEM)
        out = pl.pallas_call(
            kernel,
            in_specs=[vm, vm] + [anyspec] * 9,
            out_specs=anyspec,
            out_shape=jax.ShapeDtypeStruct((D, S), BF16),
            scratch_shapes=[
                pltpu.VMEM((D, S), BF16),
                pltpu.VMEM((D, 6 * D), BF16),
                pltpu.VMEM((2, Sk, Dh), BF16),
                pltpu.VMEM((2, Sk, Dh), BF16),
                pltpu.VMEM((2, D, G), BF16),
                pltpu.VMEM((2, D, G), BF16),
                pltpu.VMEM((Sk // 2, Dh), U32),
                pltpu.VMEM((Dh // 2, Sk), U32),
                pltpu.VMEM((D // 2, G), U32),
                pltpu.VMEM((D // 2, G), U32),
                pltpu.VMEM((S // 2, D), U32),
                pltpu.VMEM((2, TQ, Dh), U32),
                pltpu.VMEM((nblk, Sk + 8, 2 * TQ), F32),
                pltpu.VMEM((nblk, D, TQ), F32),
                pltpu.VMEM((8, D), F32),
                pltpu.VMEM((5 * D, 128), F32),
                pltpu.VMEM((S, D), F32),
                pltpu.VMEM((nblk, D, TQ), BF16),
                pltpu.VMEM((nblk, TQ), F32),
                pltpu.VMEM((TOPC, D), F32),
                pltpu.VMEM((D, Fd), BF16),
                pltpu.VMEM((D, Fd), BF16),
                pltpu.VMEM((D, Fd), BF16),
                pltpu.SemaphoreType.DMA((5,)),
                pltpu.SemaphoreType.DMA((nblk // 2,)),
                pltpu.SemaphoreType.DMA((4, 2)),
                pltpu.SemaphoreType.DMA((nblk,)),
            ],
            compiler_params=pltpu.CompilerParams(vmem_limit_bytes=110 * 1024 * 1024),
        )(c, B_w_r.reshape(1, D), xt, k, v, A_wq, A_wo.T, w_mod, B_w_gate, B_w_up, B_w_down.T)
        return out.T.reshape(B, S, D)
    return fn


_impl = make()


@jax.jit
def pallas_adaLN_cond__gqa_block_cached__moe_arch_mod__prompt_kernel(
    A_x: jax.Array,
    A_k_cache: jax.Array,
    A_v_cache: jax.Array,
    A_wq: jax.Array,
    A_wo: jax.Array,
    B_x: jax.Array,
    B_w_r: jax.Array,
    B_w_gate: jax.Array,
    B_w_up: jax.Array,
    B_w_down: jax.Array,
    c: jax.Array,
    w_mod: jax.Array,
):
    return _impl(A_x, A_k_cache, A_v_cache, A_wq, A_wo, B_x, B_w_r, B_w_gate, B_w_up, B_w_down, c, w_mod)
```

```python
import math
import jax
import jax.numpy as jnp
from jax import lax
import jax.experimental.pallas as pl
import jax.experimental.pallas.tpu as pltpu

F32 = jnp.float32
BF16 = jnp.bfloat16
U32 = jnp.uint32
I32 = jnp.int32
EPS = 1e-05
TOPC = 8
NT = (((1,), (1,)), ((), ()))
TQ = 128
KEY_BIAS = 0x20000000


def _pk(x):
    return pltpu.bitcast(x, U32)


def _upk(x):
    return pltpu.bitcast(x, BF16)


def _rb(x):
    return x.astype(BF16).astype(F32)


def _tree(xs, op):
    while len(xs) > 1:
        xs = [op(xs[i], xs[i + 1]) if i + 1 < len(xs) else xs[i] for i in range(0, len(xs), 2)]
    return xs[0]


def _red0(x, op, red, grp):
    n = x.shape[0]
    acc = None
    for t in range(0, n, 8 * grp):
        part = _tree([x[j:j + 8, :] for j in range(t, min(t + 8 * grp, n), 8)], op)
        acc = part if acc is None else op(acc, part)
    return red(acc, axis=0, keepdims=True)


def _ln_t(x):
    d = x.shape[0]
    mu = _red0(x, jnp.add, jnp.sum, 8) * (1.0 / d)
    xc = x - mu
    var = _red0(xc * xc, jnp.add, jnp.sum, 8) * (1.0 / d)
    den = _rb(jnp.sqrt(_rb(_rb(var) + EPS)))
    return xc * (1.0 / den)


def _stats_t(x, w=None):
    d = x.shape[0]
    piv = x[0:1, :]
    xd = x - piv
    s1 = _red0(xd, jnp.add, jnp.sum, 8) * (1.0 / d)
    s2 = _red0(xd * xd, jnp.add, jnp.sum, 8) * (1.0 / d)
    var = jnp.maximum(s2 - s1 * s1, 0.0)
    den = _rb(jnp.sqrt(_rb(_rb(var) + EPS)))
    mu = _rb(piv + s1)
    if w is None:
        return mu, 1.0 / den
    return mu, 1.0 / den, _red0(xd * w, jnp.add, jnp.sum, 8), piv


def make(scopes=0, gm=4, gs=16, mimic=1, prow=32, chain=1, xin=0, inl=1, lu=2, nsplit=1, late=1, cd=1, cwd=1, tprow=32, tcd=1, pad=1, order=0):
    def scope(name):
        return jax.named_scope(name) if scopes else jax.named_scope("")

    def kernel(c_ref, wr_ref, xt_hbm, k_hbm, v_hbm, wq_hbm, wot_hbm, wmod_hbm,
               wg_hbm, wu_hbm, wdt_hbm, out_hbm,
               x_sc, wmod_sc, kst, vst, wqst, wost, k_sc, vt_sc, wq_sc, wot_sc,
               h_sc, q_sc, s_sc, acc_sc, mod_sc, modt_sc, w_sc, out_sc, x1_sc, xs_sc, st_sc, zv_sc, z_ref, o_sc,
               wg_sc, wu_sc, wdt_sc, sems, xsems, lsems, osems):
        D, S = x_sc.shape
        Hkv, Sk, Dh = k_hbm.shape
        G = 2 * Dh
        nblk = S // TQ
        ngrp = nblk // 2
        GW = 2 * TQ
        qscale = (Dh ** -0.5) * math.log2(math.e)

        def ds(i, n):
            return slice(i * n, (i + 1) * n) if isinstance(i, int) else pl.ds(pl.multiple_of(i * n, n), n)

        def cp_k(g, slot):
            return pltpu.make_async_copy(k_hbm.at[g], kst.at[slot], lsems.at[0, slot])

        def cp_wq(g, slot):
            return pltpu.make_async_copy(wq_hbm.at[:, ds(g, G)], wqst.at[slot], lsems.at[1, slot])

        def cp_v(g, slot):
            return pltpu.make_async_copy(v_hbm.at[g], vst.at[slot], lsems.at[2, slot])

        def cp_wo(g, slot):
            return pltpu.make_async_copy(wot_hbm.at[:, ds(g, G)], wost.at[slot], lsems.at[3, slot])

        def cp_x(j):
            return pltpu.make_async_copy(xt_hbm.at[:, ds(j, GW)], x_sc.at[:, ds(j, GW)], xsems.at[j])

        def cp_out(b):
            return pltpu.make_async_copy(out_sc.at[b + 1], out_hbm.at[:, ds(b, TQ)], osems.at[b])

        moe = [pltpu.make_async_copy(wg_hbm, wg_sc, sems.at[0]),
               pltpu.make_async_copy(wu_hbm, wu_sc, sems.at[1]),
               pltpu.make_async_copy(wdt_hbm, wdt_sc, sems.at[2])]
        cp_m0 = pltpu.make_async_copy(wmod_hbm.at[:, 0:2 * D], wmod_sc.at[:, 0:2 * D], sems.at[3])
        cp_m1 = pltpu.make_async_copy(wmod_hbm.at[:, 2 * D:6 * D], wmod_sc.at[:, 2 * D:6 * D], sems.at[4])

        def ln1(c):
            sa = mod_sc[0:1, 0:D]
            ca1 = mod_sc[1:2, 0:D]
            x = x_sc[:, ds(c, TQ)].astype(F32)
            mu, inv = _stats_t(x)
            h = (((x - mu) * inv).T * ca1 + sa).astype(BF16)
            h_sc[ds(c, TQ // 2), :] = _pk(h)
            return h

        def qproj(c, h=None):
            if h is None:
                h = _upk(h_sc[ds(c, TQ // 2), :])
            q = jnp.dot(h, _upk(wq_sc[...]), preferred_element_type=F32)
            q = (q * qscale).astype(BF16)
            return jnp.concatenate([q[:, :Dh], q[:, Dh:]], axis=0)

        def qk(c, q, split=False):
            if split:
                st = jnp.concatenate([
                    lax.dot_general(_upk(k_sc[ds(j, Sk // 4), :]), q, NT, preferred_element_type=F32)
                    for j in range(2)], axis=0)
            else:
                st = lax.dot_general(_upk(k_sc[...]), q, NT, preferred_element_type=F32)
            s_sc[c, 0:Sk, :] = st
            s_sc[c, Sk:Sk + 8, :] = jnp.broadcast_to(_red0(st, jnp.maximum, jnp.max, gm), (8, 2 * TQ))

        def tie(v, dep):
            return pltpu.bitcast(pltpu.bitcast(v, U32) | (dep & zv_sc[...]), v.dtype)

        def pv(c):
            m = s_sc[c, Sk:Sk + 1, :]
            p = jnp.exp2(s_sc[c, 0:Sk, :] - m)
            l = _red0(p, jnp.add, jnp.sum, gs)
            ot = jnp.dot(_upk(vt_sc[...]), p.astype(BF16), preferred_element_type=F32)
            ot = (ot * (1.0 / l)).astype(BF16)
            return jnp.concatenate([ot[:, :TQ], ot[:, TQ:]], axis=0)

        def pvh(c, n):
            cols = slice(n * TQ, (n + 1) * TQ)
            m = s_sc[c, Sk:Sk + 1, cols]
            p = jnp.exp2(s_sc[c, 0:Sk, cols] - m)
            l = _red0(p, jnp.add, jnp.sum, gs)
            ot = jnp.dot(_upk(vt_sc[...]), p.astype(BF16), preferred_element_type=F32)
            return ot * (1.0 / l)

        def oproj(c, o2t, split=False, final=False):
            if split:
                d = jnp.concatenate([
                    jnp.dot(_upk(wot_sc[ds(j, D // 4), :]), o2t, preferred_element_type=F32)
                    for j in range(2)], axis=0)
            else:
                d = jnp.dot(_upk(wot_sc[...]), o2t, preferred_element_type=F32)
            if not final:
                acc_sc[c] += d
            else:
                x1 = _rb(x_sc[:, ds(c, TQ)].astype(F32) + modt_sc[0:D, :] * (acc_sc[c] + d))
                xb = x1_sc.at[final - 1]
                xb[0:D, :] = x1
                mu, inv, rw, piv = _stats_t(x1, modt_sc[3 * D:4 * D, :])
                xb[D:D + 8, :] = jnp.broadcast_to(mu, (8, TQ))
                xb[D + 8:D + 16, :] = jnp.broadcast_to(inv, (8, TQ))
                st_sc[0, pl.ds(c, 1), :] = mu
                st_sc[1, pl.ds(c, 1), :] = inv
                st_sc[2, pl.ds(c, 1), :] = (rw - (mu - piv) * mod_sc[5:6, 0:TQ]) * inv + mod_sc[6:7, 0:TQ]

        def post(v0, slots, ch, cw, prow, cd, pad=0):
            mu0 = [x1_sc[u, D:D + 8, :] for u in slots]
            inv0 = [x1_sc[u, D + 8:D + 16, :] for u in slots]
            for f0 in range(0, D, 128):
                fw = min(128, D - f0)
                words = []
                for r0 in range(f0, f0 + fw, prow):
                    pr = min(prow, f0 + fw - r0)
                    gc = modt_sc[D + r0:D + r0 + pr, :]
                    gs_ = modt_sc[2 * D + r0:2 * D + r0 + pr, :]
                    dep = ch[-cd] if len(ch) >= cd else None
                    if r0 == f0 and len(cw) >= cwd:
                        dep = cw[-cwd] if dep is None else dep | cw[-cwd]
                    xs = []
                    for u in range(len(slots)):
                        x1 = x1_sc[slots[u], r0:r0 + pr, :]
                        xs.append(x1)
                        mu = mu0[u] if dep is None else tie(mu0[u], dep)
                        mu = jnp.concatenate([mu] * (pr // 8), axis=0)
                        inv = jnp.concatenate([inv0[u]] * (pr // 8), axis=0)
                        o = x1 + ((x1 - mu) * inv * gc + gs_)
                        out_sc[v0 + u, r0:r0 + pr, :] = o.astype(BF16)
                    wd = pltpu.bitcast(xs[0], U32)
                    if len(xs) > 1:
                        wd = wd | (pltpu.bitcast(xs[1], U32) >> 16)
                    words.append(wd)
                    dd = _pk(out_sc[z_ref[0], 0:16, :])
                    for _ in range(pad):
                        dd = pltpu.roll(dd, 1, 1)
                    ch.append(dd)
                wt = pltpu.bitcast(jnp.concatenate(words, axis=0), F32).T
                w_sc[ds(v0 // 2, TQ), f0:f0 + fw] = wt
                cw.append(pltpu.bitcast(w_sc[pl.ds(pl.multiple_of(z_ref[0], 8), 8), 0:128], U32))

        with scope("p0_start"):
            for cp in (cp_x(0), cp_m0, cp_wq(0, 0), cp_k(0, 0)):
                cp.start()
        with scope("p0_zero"):
            acc_sc[...] = jnp.zeros(acc_sc.shape, F32)
            x1_sc[...] = jnp.zeros(x1_sc.shape, F32)
            o_sc[...] = jnp.zeros(o_sc.shape, U32)
            st_sc[...] = jnp.zeros(st_sc.shape, F32)
            zv_sc[...] = jnp.zeros(zv_sc.shape, U32)
            z_ref[0] = 0
            c = c_ref[...].astype(F32)
            sc8 = jnp.broadcast_to((c * jax.nn.sigmoid(c)).astype(BF16), (8, D))
        with scope("p1_wait_x0"):
            cp_x(0).wait()
        with scope("p2_ln"):
            for cc in range(2):
                x = x_sc[:, ds(cc, TQ)].astype(F32)
                mu, inv = _stats_t(x)
                w_sc[ds(cc, TQ), :] = ((x - mu) * inv).T
        with scope("p3_wait_m0"):
            cp_m0.wait()
        with scope("p4_start"):
            cp_x(1).start()
            cp_v(0, 0).start()
        with scope("p4_mod"):
            m = _rb(jnp.dot(sc8, wmod_sc[:, 0:2 * D], preferred_element_type=F32))
            sa = m[0:1, 0:D]
            ca1 = _rb(1.0 + m[0:1, D:2 * D])
            mod_sc[0:1, :] = sa
            mod_sc[1:2, :] = ca1
            h_sc[0:TQ, :] = _pk((w_sc[0:2 * TQ, :] * ca1 + sa).astype(BF16))
        with scope("p5_wait_wq"):
            cp_wq(0, 0).wait()
        with scope("p6_qp"):
            wq_sc[...] = _pk(wqst[0])
            q_sc[0] = _pk(qproj(0))
            q_sc[1] = _pk(qproj(1))
        with scope("p7_wait_k"):
            cp_k(0, 0).wait()
        with scope("p8"):
            k_sc[...] = _pk(kst[0])
            for j in range(2, ngrp):
                cp_x(j).start()

        def fbody(j, _):
            @pl.when(j + 1 < ngrp)
            def _():
                cp_x(j + 1).wait()

            @pl.when(j == 0)
            def _():
                cp_v(0, 0).wait()

            @pl.when(j == 2)
            def _():
                for cp in (cp_k(1, 1), cp_wq(1, 1), cp_v(1, 1), cp_wo(0, 1), cp_m1):
                    cp.start()
            with scope("first"):
                jn = jnp.minimum(j + 1, ngrp - 1)
                qk(2 * j, _upk(q_sc[0]))
                qk(2 * j + 1, _upk(q_sc[1]))
                q_sc[0] = _pk(qproj(2 * jn, ln1(2 * jn)))
                q_sc[1] = _pk(qproj(2 * jn + 1, ln1(2 * jn + 1)))
                vt_sc[:, ds(j, GW)] = _pk(vst[0, ds(j, GW), :].T)
            return 0
        lax.fori_loop(0, ngrp, fbody, 0)

        with scope("mid"):
            cp_m1.wait()
            for cp in moe:
                cp.start()
            m = _rb(jnp.dot(sc8, wmod_sc[:, 2 * D:6 * D], preferred_element_type=F32))
            ga = m[0:1, 0:D]
            sb = m[0:1, D:2 * D]
            cb1 = _rb(1.0 + m[0:1, 2 * D:3 * D])
            gb = m[0:1, 3 * D:4 * D]
            wr = wr_ref[...].astype(F32)
            mod_sc[2:3, :] = gb
            mod_sc[3:4, :] = sb
            mod_sc[4:5, :] = cb1
            mod_sc[5:6, :] = jnp.broadcast_to(jnp.sum(wr * cb1, axis=1, keepdims=True), (1, D))
            mod_sc[6:7, :] = jnp.broadcast_to(jnp.sum(wr * sb, axis=1, keepdims=True), (1, D))
            for i, vec in enumerate((ga, gb * cb1, gb * sb, wr * cb1)):
                modt_sc[i * D:(i + 1) * D, :] = jnp.broadcast_to(vec, (128, D)).T

        def step(i, _):
            slot = i % 2
            for cp in (cp_k(i, slot), cp_wq(i, slot), cp_v(i, slot), cp_wo(i - 1, slot)):
                cp.wait()

            @pl.when(i + 1 < Hkv)
            def _():
                for cp in (cp_k(i + 1, 1 - slot), cp_wq(i + 1, 1 - slot), cp_v(i + 1, 1 - slot)):
                    cp.start()
            cp_wo(i, 1 - slot).start()

            with scope("main"):
                wq_sc[...] = _pk(wqst[slot])
                k_sc[...] = _pk(kst[slot])
                wot_sc[...] = _pk(wost[slot])
                q = None
                for c in range(nblk):
                    last = c == nblk - 1
                    o = pv(c)
                    if c == 0:
                        q = qproj(0)
                    qn = None if last else qproj(c + 1)
                    qk(c, q, split=last)
                    oproj(c, o, split=last)
                    q = qn
                vt_sc[...] = _pk(vst[slot].T)
            return 0
        lax.fori_loop(1, Hkv, step, 0)

        cp_wo(Hkv - 1, Hkv % 2).wait()
        wot_sc[...] = _pk(wost[Hkv % 2])

        def lbody(j, _):
            with scope("last"):
                ch, cw = [], []
                for u0 in range(0, lu, 2):
                    post(lu * jnp.maximum(j - 1, 0) + u0, (u0, u0 + 1), ch, cw, prow, cd, pad)
                o = _upk(o_sc[...])
                for u in range(lu):
                    c = lu * j + u - 1
                    if order == 0:
                        oproj(jnp.maximum(c, 0) if u == 0 else c, o, final=u + 1)
                        o = pv(c + 1)
                    elif order == 2:
                        if u == 0:
                            oproj(jnp.maximum(c, 0), o, final=u + 1)
                            o0 = pvh(c + 1, 0)
                        else:
                            o0 = pvh(c + 1, 0)
                            oproj(c, o, final=u + 1)
                        o1 = pvh(c + 1, 1)
                        o = jnp.concatenate([o0, o1], axis=0).astype(BF16)
                    else:
                        on = pv(c + 1)
                        oproj(jnp.maximum(c, 0) if u == 0 else c, o, final=u + 1, split=(u == lu - 1))
                        o = on
                o_sc[...] = _pk(o)
            return 0
        lax.fori_loop(0, nblk // lu, lbody, 0)

        with scope("tail"):
            oproj(nblk - 1, _upk(o_sc[...]), split=True, final=lu + 1)
            r = _rb(st_sc[2]) + 0.0
            b16 = pltpu.bitcast(r, U32) >> 16
            ordk = jnp.where(b16 >= 0x8000, 0xFFFF - b16, b16 + 0x8000)
            tok = (lax.broadcasted_iota(U32, r.shape, 0) * TQ + lax.broadcasted_iota(U32, r.shape, 1))
            key = pltpu.bitcast((ordk << 11) + (S - 1 - tok) + KEY_BIAS, F32)
            sub = lax.broadcasted_iota(I32, (TOPC, 128), 0)
            top = jnp.zeros((TOPC, 128), F32)
            idxs = []
            mus = jnp.zeros((TOPC, TQ), F32)
            invs = jnp.zeros((TOPC, TQ), F32)
            for t in range(TOPC):
                mx = jnp.max(jnp.max(key, axis=0, keepdims=True), axis=1, keepdims=True)
                sel = key == mx
                key = jnp.where(sel, 0.0, key)
                top = jnp.where(sub == t, mx, top)
                mus = jnp.where(sub == t, jnp.sum(jnp.where(sel, st_sc[0], 0.0), axis=0, keepdims=True), mus)
                invs = jnp.where(sub == t, jnp.sum(jnp.where(sel, st_sc[1], 0.0), axis=0, keepdims=True), invs)
            ch, cw = [], []
            for u0 in range(0, lu, 2):
                post(nblk - lu + u0, (u0, u0 + 1), ch, cw, tprow, tcd)
            post(nblk, (lu,), ch, cw, tprow, tcd)
            topi = S - 1 - (pltpu.bitcast(top, I32) & (S - 1))
            idxs = [topi[t, 0] for t in range(TOPC)]
            blks = [ix // TQ for ix in idxs]
            for t in range(TOPC):
                xs_sc[t:t + 1, :] = w_sc[pl.ds(((blks[t] + 1) // 2) * TQ + idxs[t] % TQ, 1), :]
            hit = []
            for b in range(nblk):
                h = blks[0] == b
                for t in range(1, TOPC):
                    h = jnp.logical_or(h, blks[t] == b)
                hit.append(h)

                @pl.when(jnp.logical_not(h))
                def _():
                    cp_out(b).start()
            ordt = (pltpu.bitcast(top, U32) - KEY_BIAS) >> 11
            rsel = pltpu.bitcast(jnp.where(ordt >= 0x8000, ordt - 0x8000, 0xFFFF - ordt) << 16, F32)[:, 0:1]
            mus = jnp.sum(mus, axis=1, keepdims=True)
            invs = jnp.sum(invs, axis=1, keepdims=True)
            words = pltpu.bitcast(xs_sc[...], U32)
            odd = ((topi[:, 0:1] // TQ) % 2) == 0
            x1s = pltpu.bitcast(jnp.where(odd, words << 16, words & jnp.uint32(0xFFFF0000)), F32)
            h2s = _rb(_rb(_rb(_rb(x1s - mus) * invs) * mod_sc[4:5, :]) + mod_sc[3:4, :])
            xsel = h2s.astype(BF16)
            for cp in moe:
                cp.wait()
            gt = _rb(jnp.dot(xsel, wg_sc[...], preferred_element_type=F32))
            ut = _rb(jnp.dot(xsel, wu_sc[...], preferred_element_type=F32))
            a = (_rb(gt * jax.nn.sigmoid(gt)) * ut).astype(BF16)
            y = _rb(lax.dot_general(a, wdt_sc[...], NT, preferred_element_type=F32))
            y = _rb(y * _rb(jax.nn.sigmoid(rsel)))
            new = x1s + mod_sc[2:3, :] * _rb(h2s + y)
            newt = _pk(jnp.concatenate([new, jnp.zeros((TQ - TOPC, D), F32)], axis=0).T.astype(BF16))
            lane = lax.broadcasted_iota(I32, newt.shape, 1)
            for t in range(TOPC):
                ln = idxs[t] % TQ
                rolled = pltpu.roll(newt, (ln + (TQ - t)) % TQ, 1)
                pltpu.store(out_sc.bitcast(U32).at[blks[t] + 1], rolled, mask=lane == ln)
            for b in range(nblk):
                @pl.when(hit[b])
                def _():
                    cp_out(b).start()
            for b in range(nblk):
                cp_out(b).wait()

    def fn(A_x, A_k_cache, A_v_cache, A_wq, A_wo, B_x, B_w_r, B_w_gate, B_w_up, B_w_down, c, w_mod):
        B, S, D = A_x.shape
        _, Hkv, Sk, Dh = A_k_cache.shape
        G = A_wq.shape[1] // Hkv
        Fd = B_w_gate.shape[1]
        nblk = S // TQ
        xt = A_x.reshape(S, D).T
        k = A_k_cache.reshape(Hkv, Sk, Dh)
        v = A_v_cache.reshape(Hkv, Sk, Dh)
        anyspec = pl.BlockSpec(memory_space=pl.ANY)
        vm = pl.BlockSpec(memory_space=pltpu.VMEM)
        out = pl.pallas_call(
            kernel,
            in_specs=[vm, vm] + [anyspec] * 9,
            out_specs=anyspec,
            out_shape=jax.ShapeDtypeStruct((D, S), BF16),
            scratch_shapes=[
                pltpu.VMEM((D, S), BF16),
                pltpu.VMEM((D, 6 * D), BF16),
                pltpu.VMEM((2, Sk, Dh), BF16),
                pltpu.VMEM((2, Sk, Dh), BF16),
                pltpu.VMEM((2, D, G), BF16),
                pltpu.VMEM((2, D, G), BF16),
                pltpu.VMEM((Sk // 2, Dh), U32),
                pltpu.VMEM((Dh // 2, Sk), U32),
                pltpu.VMEM((D // 2, G), U32),
                pltpu.VMEM((D // 2, G), U32),
                pltpu.VMEM((S // 2, D), U32),
                pltpu.VMEM((2, TQ, Dh), U32),
                pltpu.VMEM((nblk, Sk + 8, 2 * TQ), F32),
                pltpu.VMEM((nblk, D, TQ), F32),
                pltpu.VMEM((8, D), F32),
                pltpu.VMEM((4 * D, 128), F32),
                pltpu.VMEM((S // 2 + TQ, D), F32),
                pltpu.VMEM((nblk + 1, D, TQ), BF16),
                pltpu.VMEM((lu + 1, D + 16, TQ), F32),
                pltpu.VMEM((TOPC, D), F32),
                pltpu.VMEM((3, nblk, TQ), F32),
                pltpu.VMEM((8, 128), U32),
                pltpu.SMEM((1,), I32),
                pltpu.VMEM((Dh, TQ), U32),
                pltpu.VMEM((D, Fd), BF16),
                pltpu.VMEM((D, Fd), BF16),
                pltpu.VMEM((D, Fd), BF16),
                pltpu.SemaphoreType.DMA((5,)),
                pltpu.SemaphoreType.DMA((nblk // 2,)),
                pltpu.SemaphoreType.DMA((4, 2)),
                pltpu.SemaphoreType.DMA((nblk,)),
            ],
            compiler_params=pltpu.CompilerParams(vmem_limit_bytes=110 * 1024 * 1024),
        )(c, B_w_r.reshape(1, D), xt, k, v, A_wq, A_wo.T, w_mod, B_w_gate, B_w_up, B_w_down.T)
        return out.T.reshape(B, S, D)
    return fn


_impl = make(lu=4, prow=32, cd=1, cwd=2, pad=1, order=2)


@jax.jit
def pallas_adaLN_cond__gqa_block_cached__moe_arch_mod__prompt_kernel(
    A_x: jax.Array,
    A_k_cache: jax.Array,
    A_v_cache: jax.Array,
    A_wq: jax.Array,
    A_wo: jax.Array,
    B_x: jax.Array,
    B_w_r: jax.Array,
    B_w_gate: jax.Array,
    B_w_up: jax.Array,
    B_w_down: jax.Array,
    c: jax.Array,
    w_mod: jax.Array,
):
    return _impl(A_x, A_k_cache, A_v_cache, A_wq, A_wo, B_x, B_w_r, B_w_gate, B_w_up, B_w_down, c, w_mod)
```

```python
import math
import jax
import jax.numpy as jnp
from jax import lax
import jax.experimental.pallas as pl
import jax.experimental.pallas.tpu as pltpu

F32 = jnp.float32
BF16 = jnp.bfloat16
U32 = jnp.uint32
I32 = jnp.int32
EPS = 1e-05
TOPC = 8
NT = (((1,), (1,)), ((), ()))
TQ = 128
KEY_BIAS = 0x20000000


def _pk(x):
    return pltpu.bitcast(x, U32)


def _upk(x):
    return pltpu.bitcast(x, BF16)


def _rb(x):
    return x.astype(BF16).astype(F32)


def _tree(xs, op):
    while len(xs) > 1:
        xs = [op(xs[i], xs[i + 1]) if i + 1 < len(xs) else xs[i] for i in range(0, len(xs), 2)]
    return xs[0]


def _red0(x, op, red, grp):
    n = x.shape[0]
    acc = None
    for t in range(0, n, 8 * grp):
        part = _tree([x[j:j + 8, :] for j in range(t, min(t + 8 * grp, n), 8)], op)
        acc = part if acc is None else op(acc, part)
    return red(acc, axis=0, keepdims=True)


def _ln_t(x):
    d = x.shape[0]
    mu = _red0(x, jnp.add, jnp.sum, 8) * (1.0 / d)
    xc = x - mu
    var = _red0(xc * xc, jnp.add, jnp.sum, 8) * (1.0 / d)
    den = _rb(jnp.sqrt(_rb(_rb(var) + EPS)))
    return xc * (1.0 / den)


def _stats_t(x, w=None):
    d = x.shape[0]
    piv = x[0:1, :]
    xd = x - piv
    s1 = _red0(xd, jnp.add, jnp.sum, 8) * (1.0 / d)
    s2 = _red0(xd * xd, jnp.add, jnp.sum, 8) * (1.0 / d)
    var = jnp.maximum(s2 - s1 * s1, 0.0)
    den = _rb(jnp.sqrt(_rb(_rb(var) + EPS)))
    mu = _rb(piv + s1)
    if w is None:
        return mu, 1.0 / den
    return mu, 1.0 / den, _red0(xd * w, jnp.add, jnp.sum, 8), piv


def make(scopes=0, gm=4, gs=16, mimic=1, prow=32, chain=1, xin=0, inl=1, lu=4, nsplit=1, late=1, cd=1, cwd=2, tprow=32, tcd=1, pad=1, order=2, fchain=0, srow=16, pv_=0, qfirst=1, nochk=1):
    def scope(name):
        return jax.named_scope(name) if scopes else jax.named_scope("")

    def kernel(c_hbm, wr_hbm, xt_hbm, k_hbm, v_hbm, wq_hbm, wot_hbm, wmod_hbm,
               wg_hbm, wu_hbm, wdt_hbm, out_hbm,
               x_sc, wmod_sc, kst, vst, wqst, wost, k_sc, vt_sc, wq_sc, wot_sc,
               h_sc, q_sc, s_sc, acc_sc, mod_sc, modt_sc, w_sc, out_sc, x1_sc, xs_sc, st_sc, zv_sc, z_ref, o_sc, c_sc, wr_sc,
               wg_sc, wu_sc, wd_sc, wdst, u_sc, sems, xsems, lsems, osems):
        D, S = x_sc.shape
        Hkv, Sk, Dh = k_hbm.shape
        G = 2 * Dh
        nblk = S // TQ
        ngrp = nblk // 2
        GW = 2 * TQ
        qscale = (Dh ** -0.5) * math.log2(math.e)

        def ds(i, n):
            return slice(i * n, (i + 1) * n) if isinstance(i, int) else pl.ds(pl.multiple_of(i * n, n), n)

        def cp_k(g, slot):
            return pltpu.make_async_copy(k_hbm.at[g], kst.at[slot], lsems.at[0, slot])

        def cp_wq(g, slot):
            return pltpu.make_async_copy(wq_hbm.at[:, ds(g, G)], wqst.at[slot], lsems.at[1, slot])

        def cp_v(g, slot):
            return pltpu.make_async_copy(v_hbm.at[g], vst.at[slot], lsems.at[2, slot])

        def cp_wo(g, slot):
            return pltpu.make_async_copy(wot_hbm.at[:, ds(g, G)], wost.at[slot], lsems.at[3, slot])

        FW = 3 * 128
        NF = wdt_hbm.shape[1] // FW

        def cp_wd(i, slot):
            return pltpu.make_async_copy(wdt_hbm.at[:, ds(jnp.minimum(i - 1, NF - 1), FW)], wdst.at[slot],
                                         lsems.at[4, slot])

        def cp_x(j):
            return pltpu.make_async_copy(xt_hbm.at[:, ds(j, GW)], x_sc.at[:, ds(j, GW)], xsems.at[j])

        def cp_out(b):
            return pltpu.make_async_copy(out_sc.at[b + 1], out_hbm.at[:, ds(b, TQ)], osems.at[b])

        moe = [pltpu.make_async_copy(wg_hbm, wg_sc, sems.at[0]),
               pltpu.make_async_copy(wu_hbm, wu_sc, sems.at[1])]
        cp_m0 = pltpu.make_async_copy(wmod_hbm.at[:, 0:2 * D], wmod_sc.at[:, 0:2 * D], sems.at[3])
        cp_m1 = pltpu.make_async_copy(wmod_hbm.at[:, 2 * D:6 * D], wmod_sc.at[:, 2 * D:6 * D], sems.at[4])

        def ln1_pair(g):
            z = z_ref[0]
            piv = jnp.broadcast_to(x_sc[0:16, ds(g, GW)].astype(F32)[0:1], (8, GW))
            s1 = s2 = None
            for r0 in range(0, D, srow):
                pw = piv
                if s2 is not None:
                    b2 = pltpu.bitcast(s2, U32)
                    pw = jnp.concatenate([tie(piv[:, :TQ], b2[:, :TQ]), tie(piv[:, TQ:], b2[:, TQ:])], axis=1)
                xd = x_sc[r0:r0 + srow, ds(g, GW)].astype(F32) - jnp.concatenate([pw] * (srow // 8), axis=0)
                xq = xd * xd
                p1 = _tree([xd[j:j + 8] for j in range(0, srow, 8)], jnp.add)
                p2 = _tree([xq[j:j + 8] for j in range(0, srow, 8)], jnp.add)
                s1 = p1 if s1 is None else s1 + p1
                s2 = p2 if s2 is None else s2 + p2
            s1 = jnp.sum(s1, axis=0, keepdims=True) * (1.0 / D)
            s2 = jnp.sum(s2, axis=0, keepdims=True) * (1.0 / D)
            var = jnp.maximum(s2 - s1 * s1, 0.0)
            inv = 1.0 / _rb(jnp.sqrt(_rb(_rb(var) + EPS)))
            mu = _rb(piv + s1)
            dep = None
            for f0 in range(0, D, 128):
                fw = min(128, D - f0)
                x = x_sc[f0:f0 + fw, ds(g + z, GW)].astype(F32)
                m = mu if dep is None else jnp.concatenate([tie(mu[:, :TQ], dep), tie(mu[:, TQ:], dep)], axis=1)
                n = (x - jnp.concatenate([m] * (fw // 8), axis=0)) * inv
                h = n.T * mod_sc[1:2, f0:f0 + fw] + mod_sc[0:1, f0:f0 + fw]
                h_sc[ds(g, TQ), f0:f0 + fw] = _pk(h.astype(BF16))
                if fchain:
                    dep = h_sc[pl.ds(pl.multiple_of(z, 8), 8), 0:128]

        def qproj(c, h=None):
            if h is None:
                h = _upk(h_sc[ds(c, TQ // 2), :])
            q = jnp.dot(h, _upk(wq_sc[...]), preferred_element_type=F32)
            q = (q * qscale).astype(BF16)
            return jnp.concatenate([q[:, :Dh], q[:, Dh:]], axis=0)

        def qk(c, q, split=False):
            if split:
                st = jnp.concatenate([
                    lax.dot_general(_upk(k_sc[ds(j, Sk // 4), :]), q, NT, preferred_element_type=F32)
                    for j in range(2)], axis=0)
            else:
                st = lax.dot_general(_upk(k_sc[...]), q, NT, preferred_element_type=F32)
            s_sc[c, 0:Sk, :] = st
            s_sc[c, Sk:Sk + 8, :] = jnp.broadcast_to(_red0(st, jnp.maximum, jnp.max, gm), (8, 2 * TQ))

        def tie(v, dep):
            return pltpu.bitcast(pltpu.bitcast(v, U32) | (dep & zv_sc[...]), v.dtype)

        def pv(c):
            m = s_sc[c, Sk:Sk + 1, :]
            p = jnp.exp2(s_sc[c, 0:Sk, :] - m)
            l = _red0(p, jnp.add, jnp.sum, gs)
            ot = jnp.dot(_upk(vt_sc[...]), p.astype(BF16), preferred_element_type=F32)
            ot = (ot * (1.0 / l)).astype(BF16)
            return jnp.concatenate([ot[:, :TQ], ot[:, TQ:]], axis=0)

        def pvh(c, n):
            cols = slice(n * TQ, (n + 1) * TQ)
            m = s_sc[c, Sk:Sk + 1, cols]
            p = jnp.exp2(s_sc[c, 0:Sk, cols] - m)
            l = _red0(p, jnp.add, jnp.sum, gs)
            ot = jnp.dot(_upk(vt_sc[...]), p.astype(BF16), preferred_element_type=F32)
            return ot * (1.0 / l)

        def oproj(c, o2t, split=False, final=False):
            if split:
                d = jnp.concatenate([
                    jnp.dot(_upk(wot_sc[ds(j, D // 4), :]), o2t, preferred_element_type=F32)
                    for j in range(2)], axis=0)
            else:
                d = jnp.dot(_upk(wot_sc[...]), o2t, preferred_element_type=F32)
            if not final:
                acc_sc[c] += d
            else:
                x1 = _rb(x_sc[:, ds(c, TQ)].astype(F32) + modt_sc[0:D, :] * (acc_sc[c] + d))
                xb = x1_sc.at[final - 1]
                xb[0:D, :] = x1
                mu, inv, rw, piv = _stats_t(x1, modt_sc[3 * D:4 * D, :])
                xb[D:D + 8, :] = jnp.broadcast_to(mu, (8, TQ))
                xb[D + 8:D + 16, :] = jnp.broadcast_to(inv, (8, TQ))
                st_sc[0, pl.ds(c, 1), :] = mu
                st_sc[1, pl.ds(c, 1), :] = inv
                st_sc[2, pl.ds(c, 1), :] = (rw - (mu - piv) * mod_sc[5:6, 0:TQ]) * inv + mod_sc[6:7, 0:TQ]

        def post(v0, slots, ch, cw, prow, cd, pad=0):
            mu0 = [x1_sc[u, D:D + 8, :] for u in slots]
            inv0 = [x1_sc[u, D + 8:D + 16, :] for u in slots]
            for f0 in range(0, D, 128):
                fw = min(128, D - f0)
                words = []
                for r0 in range(f0, f0 + fw, prow):
                    pr = min(prow, f0 + fw - r0)
                    gc = modt_sc[D + r0:D + r0 + pr, :]
                    gs_ = modt_sc[2 * D + r0:2 * D + r0 + pr, :]
                    dep = ch[-cd] if len(ch) >= cd else None
                    if r0 == f0 and len(cw) >= cwd:
                        dep = cw[-cwd] if dep is None else dep | cw[-cwd]
                    xs = []
                    for u in range(len(slots)):
                        x1 = x1_sc[slots[u], r0:r0 + pr, :]
                        xs.append(x1)
                        mu = mu0[u] if dep is None else tie(mu0[u], dep)
                        mu = jnp.concatenate([mu] * (pr // 8), axis=0)
                        inv = jnp.concatenate([inv0[u]] * (pr // 8), axis=0)
                        o = x1 + ((x1 - mu) * inv * gc + gs_)
                        out_sc[v0 + u, r0:r0 + pr, :] = o.astype(BF16)
                    wd = pltpu.bitcast(xs[0], U32)
                    if len(xs) > 1:
                        wd = wd | (pltpu.bitcast(xs[1], U32) >> 16)
                    words.append(wd)
                    dd = _pk(out_sc[z_ref[0], 0:16, :])
                    for _ in range(pad):
                        dd = pltpu.roll(dd, 1, 1)
                    ch.append(dd)
                wt = pltpu.bitcast(jnp.concatenate(words, axis=0), F32).T
                w_sc[ds(v0 // 2, TQ), f0:f0 + fw] = wt
                cw.append(pltpu.bitcast(w_sc[pl.ds(pl.multiple_of(z_ref[0], 8), 8), 0:128], U32))

        cp_c = pltpu.make_async_copy(c_hbm, c_sc, sems.at[5])
        cp_wr = pltpu.make_async_copy(wr_hbm, wr_sc, sems.at[6])
        with scope("p0_start"):
            for cp in (cp_c, cp_x(0), cp_m0, cp_wq(0, 0), cp_k(0, 0), cp_x(1)):
                cp.start()
            if pv_:
                for jj in range(2, ngrp):
                    cp_x(jj).start()
        with scope("p0_zero"):
            acc_sc[...] = jnp.zeros(acc_sc.shape, F32)
            x1_sc[...] = jnp.zeros(x1_sc.shape, F32)
            o_sc[...] = jnp.zeros(o_sc.shape, U32)
            st_sc[...] = jnp.zeros(st_sc.shape, F32)
            zv_sc[...] = jnp.zeros(zv_sc.shape, U32)
            z_ref[0] = 0
            u_sc[...] = jnp.zeros(u_sc.shape, F32)
        with scope("p1_wait_x0"):
            cp_c.wait()
            cp_x(0).wait()
        with scope("p2_ln"):
            c = c_sc[...].astype(F32)
            sc8 = jnp.broadcast_to((c * jax.nn.sigmoid(c)).astype(BF16), (8, D))
            for cc in range(2):
                x = x_sc[:, ds(cc, TQ)].astype(F32)
                mu, inv = _stats_t(x)
                w_sc[ds(cc, TQ), :] = ((x - mu) * inv).T
        with scope("p3_wait_m0"):
            cp_m0.wait()
        with scope("p4_mod"):
            m = _rb(jnp.dot(sc8, wmod_sc[:, 0:2 * D], preferred_element_type=F32))
            sa = m[0:1, 0:D]
            ca1 = _rb(1.0 + m[0:1, D:2 * D])
            mod_sc[0:1, :] = sa
            mod_sc[1:2, :] = ca1
            h_sc[0:TQ, :] = _pk((w_sc[0:2 * TQ, :] * ca1 + sa).astype(BF16))
        with scope("p5_wait_wq"):
            cp_wq(0, 0).wait()
        with scope("p6_qp"):
            wq_sc[...] = _pk(wqst[0])
            q_sc[0] = _pk(qproj(0))
            q_sc[1] = _pk(qproj(1))
        with scope("p7_wait_k"):
            cp_k(0, 0).wait()
        with scope("p8"):
            k_sc[...] = _pk(kst[0])

        def fbody(j, _):
            cp_x(j + 1).wait()

            if not pv_:
                @pl.when(j == 0)
                def _():
                    for jj in range(2, ngrp):
                        cp_x(jj).start()

            @pl.when(j == 2)
            def _():
                for cp in (cp_v(0, 0), cp_m1, cp_wr, cp_k(1, 1), cp_wq(1, 1), cp_v(1, 1), cp_wo(0, 1), cp_wd(1, 1)):
                    cp.start()
            with scope("first"):
                qk(2 * j, _upk(q_sc[0]))
                qk(2 * j + 1, _upk(q_sc[1]))
                ln1_pair(j + 1)
                q_sc[0] = _pk(qproj(2 * j + 2 + z_ref[0]))
                q_sc[1] = _pk(qproj(2 * j + 3 + z_ref[0]))
            return 0
        lax.fori_loop(0, ngrp - 1, fbody, 0)

        with scope("mid"):
            cp_m1.wait()
            cp_wr.wait()
            cp_v(0, 0).wait()
            for cp in moe:
                cp.start()
            vt_sc[...] = _pk(vst[0].T)
            m = _rb(jnp.dot(sc8, wmod_sc[:, 2 * D:6 * D], preferred_element_type=F32))
            ga = m[0:1, 0:D]
            sb = m[0:1, D:2 * D]
            cb1 = _rb(1.0 + m[0:1, 2 * D:3 * D])
            gb = m[0:1, 3 * D:4 * D]
            wr = wr_sc[...].astype(F32).reshape(1, D)
            mod_sc[2:3, :] = gb
            mod_sc[3:4, :] = sb
            mod_sc[4:5, :] = cb1
            mod_sc[5:6, :] = jnp.broadcast_to(jnp.sum(wr * cb1, axis=1, keepdims=True), (1, D))
            mod_sc[6:7, :] = jnp.broadcast_to(jnp.sum(wr * sb, axis=1, keepdims=True), (1, D))
            for i, vec in enumerate((ga, gb * cb1, gb * sb, wr * cb1)):
                modt_sc[i * D:(i + 1) * D, :] = jnp.broadcast_to(vec, (128, D)).T
            qk(nblk - 2, _upk(q_sc[0]))
            qk(nblk - 1, _upk(q_sc[1]))

        def step(i, _):
            slot = i % 2
            for cp in (cp_k(i, slot), cp_wq(i, slot), cp_v(i, slot), cp_wo(i - 1, slot), cp_wd(i, slot)):
                cp.wait()

            @pl.when(i + 1 < Hkv)
            def _():
                for cp in (cp_k(i + 1, 1 - slot), cp_wq(i + 1, 1 - slot), cp_v(i + 1, 1 - slot), cp_wd(i + 1, 1 - slot)):
                    cp.start()
            cp_wo(i, 1 - slot).start()

            with scope("main"):
                wq_sc[...] = _pk(wqst[slot])
                k_sc[...] = _pk(kst[slot])
                wot_sc[...] = _pk(wost[slot])
                q = qproj(0) if qfirst else None
                for c in range(nblk):
                    last = c == nblk - 1
                    o = pv(c)
                    if c == 0 and not qfirst:
                        q = qproj(0)
                    qn = None if last else qproj(c + 1)
                    qk(c, q, split=last)
                    oproj(c, o, split=last)
                    q = qn
                vt_sc[...] = _pk(vst[slot].T)
                wd_sc[ds(jnp.minimum(i - 1, NF - 1), FW // 2), :] = _pk(wdst[slot].T)
            return 0
        lax.fori_loop(1, Hkv, step, 0)

        cp_wo(Hkv - 1, Hkv % 2).wait()
        wot_sc[...] = _pk(wost[Hkv % 2])

        def lbody(j, _):
            with scope("last"):
                ch, cw = [], []
                for u0 in range(0, lu, 2):
                    post(lu * jnp.maximum(j - 1, 0) + u0, (u0, u0 + 1), ch, cw, prow, cd, pad)
                o = _upk(o_sc[...])
                for u in range(lu):
                    c = lu * j + u - 1
                    if order == 0:
                        oproj(jnp.maximum(c, 0) if u == 0 else c, o, final=u + 1)
                        o = pv(c + 1)
                    elif order == 2:
                        if u == 0:
                            oproj(jnp.maximum(c, 0), o, final=u + 1)
                            o0 = pvh(c + 1, 0)
                        else:
                            o0 = pvh(c + 1, 0)
                            oproj(c, o, final=u + 1)
                        o1 = pvh(c + 1, 1)
                        o = jnp.concatenate([o0, o1], axis=0).astype(BF16)
                    else:
                        on = pv(c + 1)
                        oproj(jnp.maximum(c, 0) if u == 0 else c, o, final=u + 1, split=(u == lu - 1))
                        o = on
                o_sc[...] = _pk(o)
            return 0
        lax.fori_loop(0, nblk // lu, lbody, 0)

        with scope("tail"):
            oproj(nblk - 1, _upk(o_sc[...]), split=True, final=lu + 1)
            r = _rb(st_sc[2]) + 0.0
            b16 = pltpu.bitcast(r, U32) >> 16
            ordk = jnp.where(b16 >= 0x8000, 0xFFFF - b16, b16 + 0x8000)
            tok = (lax.broadcasted_iota(U32, r.shape, 0) * TQ + lax.broadcasted_iota(U32, r.shape, 1))
            key = pltpu.bitcast((ordk << 11) + (S - 1 - tok) + KEY_BIAS, F32)
            sub = lax.broadcasted_iota(I32, (TOPC, 128), 0)
            top = jnp.zeros((TOPC, 128), F32)
            idxs = []
            mus = jnp.zeros((TOPC, TQ), F32)
            invs = jnp.zeros((TOPC, TQ), F32)
            for t in range(TOPC):
                mx = jnp.max(jnp.max(key, axis=0, keepdims=True), axis=1, keepdims=True)
                sel = key == mx
                key = jnp.where(sel, 0.0, key)
                top = jnp.where(sub == t, mx, top)
                mus = jnp.where(sub == t, jnp.sum(jnp.where(sel, st_sc[0], 0.0), axis=0, keepdims=True), mus)
                invs = jnp.where(sub == t, jnp.sum(jnp.where(sel, st_sc[1], 0.0), axis=0, keepdims=True), invs)
            ch, cw = [], []
            for u0 in range(0, lu, 2):
                post(nblk - lu + u0, (u0, u0 + 1), ch, cw, tprow, tcd)
            post(nblk, (lu,), ch, cw, tprow, tcd)
            topi = S - 1 - (pltpu.bitcast(top, I32) & (S - 1))
            idxs = [topi[t, 0] for t in range(TOPC)]
            blks = [ix // TQ for ix in idxs]
            for t in range(TOPC):
                xs_sc[t:t + 1, :] = w_sc[pl.ds(((blks[t] + 1) // 2) * TQ + idxs[t] % TQ, 1), :]
            hmask = 0
            for t in range(TOPC):
                hmask = hmask | (1 << blks[t])
            hit = [((hmask >> b) & 1) == 1 for b in range(nblk)]
            for b in range(nblk):
                @pl.when(jnp.logical_not(hit[b]))
                def _():
                    cp_out(b).start()
            ordt = (pltpu.bitcast(top, U32) - KEY_BIAS) >> 11
            rsel = pltpu.bitcast(jnp.where(ordt >= 0x8000, ordt - 0x8000, 0xFFFF - ordt) << 16, F32)[:, 0:1]
            mus = jnp.sum(mus, axis=1, keepdims=True)
            invs = jnp.sum(invs, axis=1, keepdims=True)
            words = pltpu.bitcast(xs_sc[...], U32)
            odd = ((topi[:, 0:1] // TQ) % 2) == 0
            x1s = pltpu.bitcast(jnp.where(odd, words << 16, words & jnp.uint32(0xFFFF0000)), F32)
            h2s = _rb(_rb(_rb(_rb(x1s - mus) * invs) * mod_sc[4:5, :]) + mod_sc[3:4, :])
            xsel = h2s.astype(BF16)
            for cp in moe:
                cp.wait()
            gt = _rb(jnp.dot(xsel, wg_sc[...], preferred_element_type=F32))
            ut = _rb(jnp.dot(xsel, wu_sc[...], preferred_element_type=F32))
            a = (_rb(gt * jax.nn.sigmoid(gt)) * ut).astype(BF16)
            y = _rb(jnp.dot(a, _upk(wd_sc[...]), preferred_element_type=F32))
            y = _rb(y * _rb(jax.nn.sigmoid(rsel)))
            new = x1s + mod_sc[2:3, :] * _rb(h2s + y)
            lns = [ix % TQ for ix in idxs]
            color = []
            for t in range(TOPC):
                cl = 0
                for s_ in range(t):
                    cl = cl + (lns[s_] == lns[t]).astype(I32)
                color.append(cl)
            nround = color[TOPC - 1]
            for t in range(1, TOPC - 1):
                nround = jnp.maximum(nround, color[t])

            def scatter(rnd, new):
                for n, f0 in enumerate(range(0, D, 128)):
                    fw = min(128, D - f0)
                    for t in range(TOPC):
                        row = jnp.where(color[t] == rnd, lns[t], TQ)
                        u_sc[n, pl.ds(row, 1), 0:fw] = new[t:t + 1, f0:f0 + fw]
                    ut_ = _pk(u_sc[n, 0:TQ, 0:fw].T.astype(BF16))
                    lane = lax.broadcasted_iota(I32, ut_.shape, 1)
                    for t in range(TOPC):
                        row = jnp.where(color[t] == rnd, lns[t], TQ)
                        pltpu.store(out_sc.bitcast(U32).at[blks[t] + 1, f0 // 2:(f0 + fw) // 2, :], ut_,
                                    mask=lane == row)
                return new
            scatter(0, new)
            lax.fori_loop(1, nround + 1, scatter, new)
            for b in range(nblk):
                @pl.when(hit[b])
                def _():
                    cp_out(b).start()
            for b in range(nblk):
                cp_out(b).wait()

    def fn(A_x, A_k_cache, A_v_cache, A_wq, A_wo, B_x, B_w_r, B_w_gate, B_w_up, B_w_down, c, w_mod):
        B, S, D = A_x.shape
        _, Hkv, Sk, Dh = A_k_cache.shape
        G = A_wq.shape[1] // Hkv
        Fd = B_w_gate.shape[1]
        nblk = S // TQ
        xt = A_x.reshape(S, D).T
        k = A_k_cache.reshape(Hkv, Sk, Dh)
        v = A_v_cache.reshape(Hkv, Sk, Dh)
        anyspec = pl.BlockSpec(memory_space=pl.ANY)
        vm = pl.BlockSpec(memory_space=pltpu.VMEM)
        out = pl.pallas_call(
            kernel,
            in_specs=[anyspec] * 11,
            out_specs=anyspec,
            out_shape=jax.ShapeDtypeStruct((D, S), BF16),
            scratch_shapes=[
                pltpu.VMEM((D, S), BF16),
                pltpu.VMEM((D, 6 * D), BF16),
                pltpu.VMEM((2, Sk, Dh), BF16),
                pltpu.VMEM((2, Sk, Dh), BF16),
                pltpu.VMEM((2, D, G), BF16),
                pltpu.VMEM((2, D, G), BF16),
                pltpu.VMEM((Sk // 2, Dh), U32),
                pltpu.VMEM((Dh // 2, Sk), U32),
                pltpu.VMEM((D // 2, G), U32),
                pltpu.VMEM((D // 2, G), U32),
                pltpu.VMEM((S // 2, D), U32),
                pltpu.VMEM((2, TQ, Dh), U32),
                pltpu.VMEM((nblk, Sk + 8, 2 * TQ), F32),
                pltpu.VMEM((nblk, D, TQ), F32),
                pltpu.VMEM((8, D), F32),
                pltpu.VMEM((4 * D, 128), F32),
                pltpu.VMEM((S // 2 + TQ, D), F32),
                pltpu.VMEM((nblk + 1, D, TQ), BF16),
                pltpu.VMEM((lu + 1, D + 16, TQ), F32),
                pltpu.VMEM((TOPC, D), F32),
                pltpu.VMEM((3, nblk, TQ), F32),
                pltpu.VMEM((8, 128), U32),
                pltpu.SMEM((1,), I32),
                pltpu.VMEM((Dh, TQ), U32),
                pltpu.VMEM((1, D), BF16),
                pltpu.VMEM((D,), BF16),
                pltpu.VMEM((D, Fd), BF16),
                pltpu.VMEM((D, Fd), BF16),
                pltpu.VMEM((Fd // 2, D), U32),
                pltpu.VMEM((2, D, 3 * 128), BF16),
                pltpu.VMEM((5, TQ + 8, 128), F32),
                pltpu.SemaphoreType.DMA((7,)),
                pltpu.SemaphoreType.DMA((nblk // 2,)),
                pltpu.SemaphoreType.DMA((5, 2)),
                pltpu.SemaphoreType.DMA((nblk,)),
            ],
            compiler_params=pltpu.CompilerParams(vmem_limit_bytes=110 * 1024 * 1024,
                                                 disable_bounds_checks=bool(nochk),
                                                 disable_semaphore_checks=bool(nochk)),
        )(c, B_w_r, xt, k, v, A_wq, A_wo.T, w_mod, B_w_gate, B_w_up, B_w_down.T)
        return out.T.reshape(B, S, D)
    return fn


_impl = make()


@jax.jit
def pallas_adaLN_cond__gqa_block_cached__moe_arch_mod__prompt_kernel(
    A_x: jax.Array,
    A_k_cache: jax.Array,
    A_v_cache: jax.Array,
    A_wq: jax.Array,
    A_wo: jax.Array,
    B_x: jax.Array,
    B_w_r: jax.Array,
    B_w_gate: jax.Array,
    B_w_up: jax.Array,
    B_w_down: jax.Array,
    c: jax.Array,
    w_mod: jax.Array,
):
    return _impl(A_x, A_k_cache, A_v_cache, A_wq, A_wo, B_x, B_w_r, B_w_gate, B_w_up, B_w_down, c, w_mod)
```

```python
import math
import jax
import jax.numpy as jnp
from jax import lax
import jax.experimental.pallas as pl
import jax.experimental.pallas.tpu as pltpu

F32 = jnp.float32
BF16 = jnp.bfloat16
U32 = jnp.uint32
I32 = jnp.int32
EPS = 1e-05
TOPC = 8
NT = (((1,), (1,)), ((), ()))
TQ = 128
KEY_BIAS = 0x20000000


def _pk(x):
    return pltpu.bitcast(x, U32)


def _upk(x):
    return pltpu.bitcast(x, BF16)


def _rb(x):
    return x.astype(BF16).astype(F32)


def _tree(xs, op):
    while len(xs) > 1:
        xs = [op(xs[i], xs[i + 1]) if i + 1 < len(xs) else xs[i] for i in range(0, len(xs), 2)]
    return xs[0]


def _red0(x, op, red, grp):
    n = x.shape[0]
    acc = None
    for t in range(0, n, 8 * grp):
        part = _tree([x[j:j + 8, :] for j in range(t, min(t + 8 * grp, n), 8)], op)
        acc = part if acc is None else op(acc, part)
    return red(acc, axis=0, keepdims=True)


def _ln_t(x):
    d = x.shape[0]
    mu = _red0(x, jnp.add, jnp.sum, 8) * (1.0 / d)
    xc = x - mu
    var = _red0(xc * xc, jnp.add, jnp.sum, 8) * (1.0 / d)
    den = _rb(jnp.sqrt(_rb(_rb(var) + EPS)))
    return xc * (1.0 / den)


def _stats_t(x, w=None):
    d = x.shape[0]
    piv = x[0:1, :]
    xd = x - piv
    s1 = _red0(xd, jnp.add, jnp.sum, 8) * (1.0 / d)
    s2 = _red0(xd * xd, jnp.add, jnp.sum, 8) * (1.0 / d)
    var = jnp.maximum(s2 - s1 * s1, 0.0)
    den = _rb(jnp.sqrt(_rb(_rb(var) + EPS)))
    mu = _rb(piv + s1)
    if w is None:
        return mu, 1.0 / den
    return mu, 1.0 / den, _red0(xd * w, jnp.add, jnp.sum, 8), piv


def make(scopes=0, gm=4, gs=16, mimic=1, prow=32, chain=1, xin=0, inl=1, lu=4, nsplit=1, late=1, cd=1, cwd=2, tprow=32, tcd=2, pad=1, order=2, fchain=0, srow=16, pv_=0, qfirst=1, nochk=1, fd=2, kb=26, gsp=12):
    def scope(name):
        return jax.named_scope(name) if scopes else jax.named_scope("")

    def kernel(c_hbm, wr_hbm, xt_hbm, k_hbm, v_hbm, wq_hbm, wot_hbm, wmod_hbm,
               wg_hbm, wu_hbm, wdt_hbm, out_hbm,
               x_sc, wmod_sc, kst, vst, wqst, wost, k_sc, vt_sc, wq_sc, wot_sc,
               h_sc, q_sc, s_sc, acc_sc, mod_sc, modt_sc, w_sc, out_sc, x1_sc, xs_sc, st_sc, zv_sc, z_ref, o_sc, c_sc, wr_sc,
               wg_sc, wu_sc, wd_sc, wdst, u_sc, sems, xsems, lsems, osems, fsems):
        D, S = x_sc.shape
        Hkv, Sk, Dh = k_hbm.shape
        G = 2 * Dh
        nblk = S // TQ
        ngrp = nblk // 2
        GW = 2 * TQ
        qscale = (Dh ** -0.5) * math.log2(math.e)

        def ds(i, n):
            return slice(i * n, (i + 1) * n) if isinstance(i, int) else pl.ds(pl.multiple_of(i * n, n), n)

        def cp_k(g, slot):
            return pltpu.make_async_copy(k_hbm.at[g], kst.at[slot], lsems.at[0, slot])

        def cp_wq(g, slot):
            return pltpu.make_async_copy(wq_hbm.at[:, ds(g, G)], wqst.at[slot], lsems.at[1, slot])

        def cp_v(g, slot):
            return pltpu.make_async_copy(v_hbm.at[g], vst.at[slot], lsems.at[2, slot])

        def cp_wo(g, slot):
            return pltpu.make_async_copy(wot_hbm.at[:, ds(g, G)], wost.at[slot], lsems.at[3, slot])

        FW = 3 * 128
        NF = wdt_hbm.shape[1] // FW

        def cp_wd(i, slot):
            return pltpu.make_async_copy(wdt_hbm.at[:, ds(jnp.minimum(i - 1, NF - 1), FW)], wdst.at[slot],
                                         lsems.at[4, slot])

        def cp_x(j):
            return pltpu.make_async_copy(xt_hbm.at[:, ds(j, GW)], x_sc.at[:, ds(j, GW)], xsems.at[j])

        def cp_out(b):
            return pltpu.make_async_copy(out_sc.at[b + 1], out_hbm.at[:, ds(b, TQ)], osems.at[b])

        moe = [pltpu.make_async_copy(wg_hbm, wg_sc, sems.at[0]),
               pltpu.make_async_copy(wu_hbm, wu_sc, sems.at[1])]
        cp_m0 = pltpu.make_async_copy(wmod_hbm.at[:, 0:2 * D], wmod_sc.at[:, 0:2 * D], sems.at[3])
        cp_m1 = pltpu.make_async_copy(wmod_hbm.at[:, 2 * D:6 * D], wmod_sc.at[:, 2 * D:6 * D], sems.at[4])

        def ln1_pair(g):
            z = z_ref[0]
            piv = jnp.broadcast_to(x_sc[0:16, ds(g, GW)].astype(F32)[0:1], (8, GW))
            s1 = s2 = None
            for r0 in range(0, D, srow):
                pw = piv
                if s2 is not None:
                    b2 = pltpu.bitcast(s2, U32)
                    pw = jnp.concatenate([tie(piv[:, :TQ], b2[:, :TQ]), tie(piv[:, TQ:], b2[:, TQ:])], axis=1)
                xd = x_sc[r0:r0 + srow, ds(g, GW)].astype(F32) - jnp.concatenate([pw] * (srow // 8), axis=0)
                xq = xd * xd
                p1 = _tree([xd[j:j + 8] for j in range(0, srow, 8)], jnp.add)
                p2 = _tree([xq[j:j + 8] for j in range(0, srow, 8)], jnp.add)
                s1 = p1 if s1 is None else s1 + p1
                s2 = p2 if s2 is None else s2 + p2
            s1 = jnp.sum(s1, axis=0, keepdims=True) * (1.0 / D)
            s2 = jnp.sum(s2, axis=0, keepdims=True) * (1.0 / D)
            var = jnp.maximum(s2 - s1 * s1, 0.0)
            inv = 1.0 / _rb(jnp.sqrt(_rb(_rb(var) + EPS)))
            mu = _rb(piv + s1)
            dep = None
            for f0 in range(0, D, 128):
                fw = min(128, D - f0)
                x = x_sc[f0:f0 + fw, ds(g + z, GW)].astype(F32)
                m = mu if dep is None else jnp.concatenate([tie(mu[:, :TQ], dep), tie(mu[:, TQ:], dep)], axis=1)
                n = (x - jnp.concatenate([m] * (fw // 8), axis=0)) * inv
                h = n.T * mod_sc[1:2, f0:f0 + fw] + mod_sc[0:1, f0:f0 + fw]
                h_sc[ds(g, TQ), f0:f0 + fw] = _pk(h.astype(BF16))
                if fchain:
                    dep = h_sc[pl.ds(pl.multiple_of(z, 8), 8), 0:128]

        def qproj(c, h=None):
            if h is None:
                h = _upk(h_sc[ds(c, TQ // 2), :])
            q = jnp.dot(h, _upk(wq_sc[...]), preferred_element_type=F32)
            q = (q * qscale).astype(BF16)
            return jnp.concatenate([q[:, :Dh], q[:, Dh:]], axis=0)

        def qk(c, q, split=False):
            if split:
                st = jnp.concatenate([
                    lax.dot_general(_upk(k_sc[ds(j, Sk // 4), :]), q, NT, preferred_element_type=F32)
                    for j in range(2)], axis=0)
            else:
                st = lax.dot_general(_upk(k_sc[...]), q, NT, preferred_element_type=F32)
            s_sc[c, 0:Sk, :] = st
            s_sc[c, Sk:Sk + 8, :] = jnp.broadcast_to(_red0(st, jnp.maximum, jnp.max, gm), (8, 2 * TQ))

        def tie(v, dep):
            return pltpu.bitcast(pltpu.bitcast(v, U32) | (dep & zv_sc[...]), v.dtype)

        def pv(c):
            m = s_sc[c, Sk:Sk + 1, :]
            p = jnp.exp2(s_sc[c, 0:Sk, :] - m)
            l = _red0(p, jnp.add, jnp.sum, gs)
            ot = jnp.dot(_upk(vt_sc[...]), p.astype(BF16), preferred_element_type=F32)
            ot = (ot * (1.0 / l)).astype(BF16)
            return jnp.concatenate([ot[:, :TQ], ot[:, TQ:]], axis=0)

        def pvh(c, n):
            cols = slice(n * TQ, (n + 1) * TQ)
            m = s_sc[c, Sk:Sk + 1, cols]
            p = jnp.exp2(s_sc[c, 0:Sk, cols] - m)
            l = _red0(p, jnp.add, jnp.sum, gs)
            ot = jnp.dot(_upk(vt_sc[...]), p.astype(BF16), preferred_element_type=F32)
            return ot * (1.0 / l)

        def oproj(c, o2t, split=False, final=False):
            if split:
                d = jnp.concatenate([
                    jnp.dot(_upk(wot_sc[ds(j, D // 4), :]), o2t, preferred_element_type=F32)
                    for j in range(2)], axis=0)
            else:
                d = jnp.dot(_upk(wot_sc[...]), o2t, preferred_element_type=F32)
            if not final:
                acc_sc[c] += d
            else:
                x1 = _rb(x_sc[:, ds(c, TQ)].astype(F32) + modt_sc[0:D, :] * (acc_sc[c] + d))
                xb = x1_sc.at[final - 1]
                xb[0:D, :] = x1
                mu, inv, rw, piv = _stats_t(x1, modt_sc[3 * D:4 * D, :])
                xb[D:D + 8, :] = jnp.broadcast_to(mu, (8, TQ))
                xb[D + 8:D + 16, :] = jnp.broadcast_to(inv, (8, TQ))
                st_sc[0, pl.ds(c, 1), :] = mu
                st_sc[1, pl.ds(c, 1), :] = inv
                st_sc[2, pl.ds(c, 1), :] = (rw - (mu - piv) * mod_sc[5:6, 0:TQ]) * inv + mod_sc[6:7, 0:TQ]

        def post(v0, slots, ch, cw, prow, cd, pad=0):
            mu0 = [x1_sc[u, D:D + 8, :] for u in slots]
            inv0 = [x1_sc[u, D + 8:D + 16, :] for u in slots]
            for f0 in range(0, D, 128):
                fw = min(128, D - f0)
                words = []
                for r0 in range(f0, f0 + fw, prow):
                    pr = min(prow, f0 + fw - r0)
                    gc = modt_sc[D + r0:D + r0 + pr, :]
                    gs_ = modt_sc[2 * D + r0:2 * D + r0 + pr, :]
                    dep = ch[-cd] if len(ch) >= cd else None
                    if r0 == f0 and len(cw) >= cwd:
                        dep = cw[-cwd] if dep is None else dep | cw[-cwd]
                    xs = []
                    for u in range(len(slots)):
                        x1 = x1_sc[slots[u], r0:r0 + pr, :]
                        xs.append(x1)
                        mu = mu0[u] if dep is None else tie(mu0[u], dep)
                        mu = jnp.concatenate([mu] * (pr // 8), axis=0)
                        inv = jnp.concatenate([inv0[u]] * (pr // 8), axis=0)
                        o = x1 + ((x1 - mu) * inv * gc + gs_)
                        out_sc[v0 + u, r0:r0 + pr, :] = o.astype(BF16)
                    wd = pltpu.bitcast(xs[0], U32)
                    if len(xs) > 1:
                        wd = wd | (pltpu.bitcast(xs[1], U32) >> 16)
                    words.append(wd)
                    dd = _pk(out_sc[z_ref[0], 0:16, :])
                    for _ in range(pad):
                        dd = pltpu.roll(dd, 1, 1)
                    ch.append(dd)
                wt = pltpu.bitcast(jnp.concatenate(words, axis=0), F32).T
                w_sc[ds(v0 // 2, TQ), f0:f0 + fw] = wt
                cw.append(pltpu.bitcast(w_sc[pl.ds(pl.multiple_of(z_ref[0], 8), 8), 0:128], U32))

        cp_c = pltpu.make_async_copy(c_hbm, c_sc, sems.at[5])
        cp_wr = pltpu.make_async_copy(wr_hbm, wr_sc, sems.at[6])
        with scope("p0_start"):
            for cp in (cp_c, cp_x(0), cp_m0):
                cp.start()
            if pv_:
                for jj in range(2, ngrp):
                    cp_x(jj).start()
        with scope("p0_zero"):
            acc_sc[...] = jnp.zeros(acc_sc.shape, F32)
            x1_sc[...] = jnp.zeros(x1_sc.shape, F32)
            o_sc[...] = jnp.zeros(o_sc.shape, U32)
            st_sc[...] = jnp.zeros(st_sc.shape, F32)
            zv_sc[...] = jnp.zeros(zv_sc.shape, U32)
            z_ref[0] = 0
            z_ref[1] = 0
            u_sc[...] = jnp.zeros(u_sc.shape, F32)
        with scope("p1_wait_x0"):
            cp_c.wait()
            cp_wq(0, 0).start()
            cp_x(0).wait()
        with scope("p2_ln"):
            cp_k(0, 0).start()
            c = c_sc[...].astype(F32)
            sc8 = jnp.broadcast_to((c * jax.nn.sigmoid(c)).astype(BF16), (8, D))
            for cc in range(2):
                x = x_sc[:, ds(cc, TQ)].astype(F32)
                mu, inv = _stats_t(x)
                w_sc[ds(cc, TQ), :] = ((x - mu) * inv).T
        with scope("p3_wait_m0"):
            cp_m0.wait()
        with scope("p4_mod"):
            cp_x(1).start()
            m = _rb(jnp.dot(sc8, wmod_sc[:, 0:2 * D], preferred_element_type=F32))
            sa = m[0:1, 0:D]
            ca1 = _rb(1.0 + m[0:1, D:2 * D])
            mod_sc[0:1, :] = sa
            mod_sc[1:2, :] = ca1
            h_sc[0:TQ, :] = _pk((w_sc[0:2 * TQ, :] * ca1 + sa).astype(BF16))
        with scope("p5_wait_wq"):
            cp_wq(0, 0).wait()
        with scope("p6_qp"):
            wq_sc[...] = _pk(wqst[0])
            q_sc[0] = _pk(qproj(0))
            q_sc[1] = _pk(qproj(1))
        with scope("p7_wait_k"):
            cp_k(0, 0).wait()
        with scope("p8"):
            k_sc[...] = _pk(kst[0])

        def fbody(j, _):
            cp_x(j + 1).wait()

            if not pv_:
                @pl.when(j == 0)
                def _():
                    for jj in range(2, ngrp):
                        cp_x(jj).start()

            @pl.when(j == 2)
            def _():
                for cp in (cp_v(0, 0), cp_m1, cp_wr, cp_k(1, 1), cp_wq(1, 1), cp_v(1, 1), cp_wo(0, 1), cp_wd(1, 1)):
                    cp.start()
            with scope("first"):
                qk(2 * j, _upk(q_sc[0]))
                qk(2 * j + 1, _upk(q_sc[1]))
                ln1_pair(j + 1)
                q_sc[0] = _pk(qproj(2 * j + 2 + z_ref[0]))
                q_sc[1] = _pk(qproj(2 * j + 3 + z_ref[0]))
            return 0
        lax.fori_loop(0, ngrp - 1, fbody, 0)

        with scope("mid"):
            cp_m1.wait()
            cp_wr.wait()
            cp_v(0, 0).wait()
            for cp in moe:
                cp.start()
            vt_sc[...] = _pk(vst[0].T)
            m = _rb(jnp.dot(sc8, wmod_sc[:, 2 * D:6 * D], preferred_element_type=F32))
            ga = m[0:1, 0:D]
            sb = m[0:1, D:2 * D]
            cb1 = _rb(1.0 + m[0:1, 2 * D:3 * D])
            gb = m[0:1, 3 * D:4 * D]
            wr = wr_sc[...].astype(F32).reshape(1, D)
            mod_sc[2:3, :] = gb
            mod_sc[3:4, :] = sb
            mod_sc[4:5, :] = cb1
            mod_sc[5:6, :] = jnp.broadcast_to(jnp.sum(wr * cb1, axis=1, keepdims=True), (1, D))
            mod_sc[6:7, :] = jnp.broadcast_to(jnp.sum(wr * sb, axis=1, keepdims=True), (1, D))
            for i, vec in enumerate((ga, gb * cb1, gb * sb, wr * cb1)):
                modt_sc[i * D:(i + 1) * D, :] = jnp.broadcast_to(vec, (128, D)).T
            qk(nblk - 2, _upk(q_sc[0]))
            qk(nblk - 1, _upk(q_sc[1]))

        def step(i, _):
            slot = i & 1
            with scope("mw"):
                for cp in (cp_k(i, slot), cp_wq(i, slot), cp_v(i, slot), cp_wo(i - 1, slot), cp_wd(i, slot)):
                    cp.wait()

            @pl.when(i + 1 < Hkv)
            def _():
                for cp in (cp_k(i + 1, 1 - slot), cp_wq(i + 1, 1 - slot), cp_v(i + 1, 1 - slot), cp_wd(i + 1, 1 - slot)):
                    cp.start()
            cp_wo(i, 1 - slot).start()

            with scope("main"):
                wq_sc[...] = _pk(wqst[slot])
                k_sc[...] = _pk(kst[slot])
                wot_sc[...] = _pk(wost[slot])
                q = qproj(0) if qfirst else None
                for c in range(nblk):
                    last = c == nblk - 1
                    o = pv(c)
                    if c == 0 and not qfirst:
                        q = qproj(0)
                    qn = None if last else qproj(c + 1)
                    qk(c, q, split=last)
                    oproj(c, o, split=last)
                    q = qn
                vt_sc[...] = _pk(vst[slot].T)
                wd_sc[ds(jnp.minimum(i - 1, NF - 1), FW // 2), :] = _pk(wdst[slot].T)
            return 0
        lax.fori_loop(1, Hkv, step, 0)

        with scope("lw"):
            cp_wo(Hkv - 1, Hkv % 2).wait()
        with scope("lf"):
            wot_sc[...] = _pk(wost[Hkv % 2])

        def lbody(j, _):
            with scope("last"):
                ch, cw = [], []
                for u0 in range(0, lu, 2):
                    post(lu * jnp.maximum(j - 1, 0) + u0, (u0, u0 + 1), ch, cw, prow, cd, pad)
                o = _upk(o_sc[...])
                for u in range(lu):
                    c = lu * j + u - 1
                    if order == 0:
                        oproj(jnp.maximum(c, 0) if u == 0 else c, o, final=u + 1)
                        o = pv(c + 1)
                    elif order == 2:
                        if u == 0:
                            oproj(jnp.maximum(c, 0), o, final=u + 1)
                            o0 = pvh(c + 1, 0)
                        else:
                            o0 = pvh(c + 1, 0)
                            oproj(c, o, final=u + 1)
                        o1 = pvh(c + 1, 1)
                        o = jnp.concatenate([o0, o1], axis=0).astype(BF16)
                    else:
                        on = pv(c + 1)
                        oproj(jnp.maximum(c, 0) if u == 0 else c, o, final=u + 1, split=(u == lu - 1))
                        o = on
                o_sc[...] = _pk(o)
            return 0
        lax.fori_loop(0, nblk // lu, lbody, 0)

        with scope("tail"):
            oproj(nblk - 1, _upk(o_sc[...]), split=True, final=lu + 1)
            r = _rb(st_sc[2]) + 0.0
            b16 = pltpu.bitcast(r, U32) >> 16
            ordk = jnp.where(b16 >= 0x8000, 0xFFFF - b16, b16 + 0x8000)
            tok = (lax.broadcasted_iota(U32, r.shape, 0) * TQ + lax.broadcasted_iota(U32, r.shape, 1))
            key = pltpu.bitcast((ordk << 11) + (S - 1 - tok) + KEY_BIAS, F32)
            def rank(row, col):
                return _red0(jnp.where(col > row, 1.0, 0.0), jnp.add, jnp.sum, 16)

            lm = jnp.max(key, axis=0, keepdims=True)
            lrank = rank(lm, jnp.broadcast_to(lm, (TQ, TQ)).T)
            cand = jnp.concatenate([jnp.where(lrank == float(t), key, 0.0) for t in range(TOPC)], axis=0)
            cand = jnp.broadcast_to(jnp.max(cand, axis=1, keepdims=True), (TOPC * nblk, TQ))
            eye = (lax.broadcasted_iota(I32, cand.shape, 0) == lax.broadcasted_iota(I32, cand.shape, 1))
            crow = _red0(jnp.where(eye, cand, 0.0), jnp.maximum, jnp.max, 16)
            crank = rank(crow, cand)
            subf = lax.broadcasted_iota(I32, (TOPC, TQ), 0).astype(F32)
            top = jnp.max(jnp.where(crank == subf, crow, 0.0), axis=1, keepdims=True)
            top = jnp.broadcast_to(top, (TOPC, TQ))
            mus = jnp.zeros((TOPC, TQ), F32)
            invs = jnp.zeros((TOPC, TQ), F32)
            for cc in range(nblk):
                sel = key[cc:cc + 1, :] == top
                mus = jnp.where(sel, st_sc[0, cc:cc + 1, :], mus)
                invs = jnp.where(sel, st_sc[1, cc:cc + 1, :], invs)
            ch, cw = [], []
            for u0 in range(0, lu, 2):
                post(nblk - lu + u0, (u0, u0 + 1), ch, cw, tprow, tcd)
            post(nblk, (lu,), ch, cw, tprow, tcd)
            topi = S - 1 - (pltpu.bitcast(top, I32) & (S - 1))
            LG = TQ.bit_length() - 1
            rowi = ((((topi >> LG) + 1) >> 1) << LG) + (topi & (TQ - 1))
            for t in range(TOPC):
                xs_sc[t:t + 1, :] = w_sc[pl.ds(rowi[t, 0], 1), :]
            idxs = [topi[t, 0] for t in range(TOPC)]
            blks = [ix >> LG for ix in idxs]
            hmask = 0
            for t in range(TOPC):
                hmask = hmask | (1 << blks[t])
            hit = [((hmask >> b) & 1) == 1 for b in range(nblk)]
            for b in range(nblk):
                @pl.when(jnp.logical_not(hit[b]))
                def _():
                    cp_out(b).start()
            ordt = (pltpu.bitcast(top, U32) - KEY_BIAS) >> 11
            rsel = pltpu.bitcast(jnp.where(ordt >= 0x8000, ordt - 0x8000, 0xFFFF - ordt) << 16, F32)[:, 0:1]
            mus = jnp.sum(mus, axis=1, keepdims=True)
            invs = jnp.sum(invs, axis=1, keepdims=True)
            words = pltpu.bitcast(xs_sc[...], U32)
            odd = ((topi[:, 0:1] >> LG) & 1) == 0
            x1s = pltpu.bitcast(jnp.where(odd, words << 16, words & jnp.uint32(0xFFFF0000)), F32)
            h2s = _rb(_rb(_rb(_rb(x1s - mus) * invs) * mod_sc[4:5, :]) + mod_sc[3:4, :])
            xsel = h2s.astype(BF16)
            for cp in moe:
                cp.wait()
            gt = _rb(jnp.dot(xsel, wg_sc[...], preferred_element_type=F32))
            ut = _rb(jnp.dot(xsel, wu_sc[...], preferred_element_type=F32))
            af = _rb(gt * jax.nn.sigmoid(gt)) * ut
            a = af.astype(BF16)
            gate = _rb(jax.nn.sigmoid(rsel))
            lns = [ix & (TQ - 1) for ix in idxs]
            color, first = [], []
            for t in range(TOPC):
                cl, dup = 0, False
                for s_ in range(t):
                    cl = cl + (lns[s_] == lns[t]).astype(I32)
                    dup = jnp.logical_or(dup, blks[s_] == blks[t])
                color.append(cl)
                first.append(jnp.logical_not(dup))
            nround = color[TOPC - 1]
            for t in range(1, TOPC - 1):
                nround = jnp.maximum(nround, color[t])
            tiles = [(n, f0, min(128, D - f0)) for n, f0 in enumerate(range(0, D, 128))]

            def cp_fix(t, f0, fw, n):
                return pltpu.make_async_copy(out_sc.at[blks[t] + 1, f0:f0 + fw, :],
                                             out_hbm.at[f0:f0 + fw, ds(blks[t], TQ)], fsems.at[n])

            def scatter(rnd, n, f0, fw, new):
                rows = [jnp.where((color[t] >> 1) == rnd, lns[t] + (color[t] & 1) * TQ, 2 * TQ) for t in range(TOPC)]
                for t in range(TOPC):
                    u_sc[n, pl.ds(rows[t], 1), 0:fw] = new[t:t + 1, :]
                ut_ = _pk(u_sc[n, 0:2 * TQ, 0:fw].T.astype(BF16))
                lane = lax.broadcasted_iota(I32, (fw // 2, TQ), 1)
                for t in range(TOPC):
                    val = ut_[:, :TQ] if t == 0 else jnp.where((color[t] & 1) == 0, ut_[:, :TQ], ut_[:, TQ:])
                    ln = jnp.where((color[t] >> 1) == rnd, lns[t], TQ)
                    pltpu.store(out_sc.bitcast(U32).at[blks[t] + 1, f0 // 2:(f0 + fw) // 2, :], val,
                                mask=lane == ln)

            fence = []
            news = []
            for n, f0, fw in tiles:
                an = a
                if len(fence) >= fd:
                    an = jnp.concatenate([af[:, :kb * 128], tie(af[:, kb * 128:(kb + 1) * 128], fence[-fd]),
                                          af[:, (kb + 1) * 128:]], axis=1).astype(BF16)
                y = _rb(jnp.dot(an, _upk(wd_sc[:, f0:f0 + fw]), preferred_element_type=F32))
                y = _rb(y * gate)
                new = x1s[:, f0:f0 + fw] + mod_sc[2:3, f0:f0 + fw] * _rb(h2s[:, f0:f0 + fw] + y)
                news.append(new)
                scatter(0, n, f0, fw, new)
                fence.append(_pk(out_sc[z_ref[0], 0:16, :]))
                for t in range(TOPC):
                    @pl.when(first[t])
                    def _():
                        cp_fix(t, f0, fw, n).start()
            xs_sc[...] = jnp.concatenate(news, axis=1)
        with scope("fin_wait"):
            for b in range(nblk):
                @pl.when(jnp.logical_not(hit[b]))
                def _():
                    cp_out(b).wait()
            for n, f0, fw in tiles:
                for t in range(TOPC):
                    @pl.when(first[t])
                    def _():
                        cp_fix(t, f0, fw, n).wait()

            @pl.when(nround >= 2)
            def _():
                def extra(rnd, carry):
                    for n, f0, fw in tiles:
                        scatter(rnd, n, f0, fw, xs_sc[:, f0:f0 + fw])
                    return carry
                lax.fori_loop(1, (nround >> 1) + 1, extra, 0)
                for t in range(TOPC):
                    @pl.when(first[t])
                    def _():
                        cp_fix(t, 0, D, 0).start()
                for t in range(TOPC):
                    @pl.when(first[t])
                    def _():
                        cp_fix(t, 0, D, 0).wait()

    def fn(A_x, A_k_cache, A_v_cache, A_wq, A_wo, B_x, B_w_r, B_w_gate, B_w_up, B_w_down, c, w_mod):
        B, S, D = A_x.shape
        _, Hkv, Sk, Dh = A_k_cache.shape
        G = A_wq.shape[1] // Hkv
        Fd = B_w_gate.shape[1]
        nblk = S // TQ
        xt = A_x.reshape(S, D).T
        k = A_k_cache.reshape(Hkv, Sk, Dh)
        v = A_v_cache.reshape(Hkv, Sk, Dh)
        anyspec = pl.BlockSpec(memory_space=pl.ANY)
        vm = pl.BlockSpec(memory_space=pltpu.VMEM)
        out = pl.pallas_call(
            kernel,
            in_specs=[anyspec] * 11,
            out_specs=anyspec,
            out_shape=jax.ShapeDtypeStruct((D, S), BF16),
            scratch_shapes=[
                pltpu.VMEM((D, S), BF16),
                pltpu.VMEM((D, 6 * D), BF16),
                pltpu.VMEM((2, Sk, Dh), BF16),
                pltpu.VMEM((2, Sk, Dh), BF16),
                pltpu.VMEM((2, D, G), BF16),
                pltpu.VMEM((2, D, G), BF16),
                pltpu.VMEM((Sk // 2, Dh), U32),
                pltpu.VMEM((Dh // 2, Sk), U32),
                pltpu.VMEM((D // 2, G), U32),
                pltpu.VMEM((D // 2, G), U32),
                pltpu.VMEM((S // 2, D), U32),
                pltpu.VMEM((2, TQ, Dh), U32),
                pltpu.VMEM((nblk, Sk + 8, 2 * TQ), F32),
                pltpu.VMEM((nblk, D, TQ), F32),
                pltpu.VMEM((8, D), F32),
                pltpu.VMEM((4 * D, 128), F32),
                pltpu.VMEM((S // 2 + TQ, D), F32),
                pltpu.VMEM((nblk + 1, D, TQ), BF16),
                pltpu.VMEM((lu + 1, D + 16, TQ), F32),
                pltpu.VMEM((TOPC, D), F32),
                pltpu.VMEM((3, nblk, TQ), F32),
                pltpu.VMEM((8, 128), U32),
                pltpu.SMEM((2,), I32),
                pltpu.VMEM((Dh, TQ), U32),
                pltpu.VMEM((1, D), BF16),
                pltpu.VMEM((D,), BF16),
                pltpu.VMEM((D, Fd), BF16),
                pltpu.VMEM((D, Fd), BF16),
                pltpu.VMEM((Fd // 2, D), U32),
                pltpu.VMEM((2, D, 3 * 128), BF16),
                pltpu.VMEM((5, 2 * TQ + 8, 128), F32),
                pltpu.SemaphoreType.DMA((7,)),
                pltpu.SemaphoreType.DMA((nblk // 2,)),
                pltpu.SemaphoreType.DMA((5, 2)),
                pltpu.SemaphoreType.DMA((nblk,)),
                pltpu.SemaphoreType.DMA((5,)),
            ],
            compiler_params=pltpu.CompilerParams(vmem_limit_bytes=110 * 1024 * 1024,
                                                 disable_bounds_checks=bool(nochk),
                                                 disable_semaphore_checks=bool(nochk)),
        )(c, B_w_r, xt, k, v, A_wq, A_wo.T, w_mod, B_w_gate, B_w_up, B_w_down.T)
        return out.T.reshape(B, S, D)
    return fn


_impl = make()


@jax.jit
def pallas_adaLN_cond__gqa_block_cached__moe_arch_mod__prompt_kernel(
    A_x: jax.Array,
    A_k_cache: jax.Array,
    A_v_cache: jax.Array,
    A_wq: jax.Array,
    A_wo: jax.Array,
    B_x: jax.Array,
    B_w_r: jax.Array,
    B_w_gate: jax.Array,
    B_w_up: jax.Array,
    B_w_down: jax.Array,
    c: jax.Array,
    w_mod: jax.Array,
):
    return _impl(A_x, A_k_cache, A_v_cache, A_wq, A_wo, B_x, B_w_r, B_w_gate, B_w_up, B_w_down, c, w_mod)
```

```python
import math

import jax
import jax.numpy as jnp
from jax import lax
import jax.experimental.pallas as pl
import jax.experimental.pallas.tpu as pltpu

F32 = jnp.float32
BF16 = jnp.bfloat16
U32 = jnp.uint32
I32 = jnp.int32
EPS = 1e-05
TOPC = 8
NT = (((1,), (1,)), ((), ()))
TQ = 128
LG = 7
LU = 4
FW = 3 * 128
MT = 5
KEY_BIAS = 0x20000000


def _pk(x):
    return pltpu.bitcast(x, U32)


def _upk(x):
    return pltpu.bitcast(x, BF16)


def _rb(x):
    return x.astype(BF16).astype(F32)


def _tree(xs, op):
    while len(xs) > 1:
        xs = [op(xs[i], xs[i + 1]) if i + 1 < len(xs) else xs[i] for i in range(0, len(xs), 2)]
    return xs[0]


def _red0(x, op, red, grp):
    n = x.shape[0]
    acc = None
    for t in range(0, n, 8 * grp):
        part = _tree([x[j:j + 8, :] for j in range(t, min(t + 8 * grp, n), 8)], op)
        acc = part if acc is None else op(acc, part)
    return red(acc, axis=0, keepdims=True)


def _ln_finish(piv, s1, s2):
    var = jnp.maximum(s2 - s1 * s1, 0.0)
    return _rb(piv + s1), 1.0 / _rb(jnp.sqrt(_rb(_rb(var) + EPS)))


def _stats_t(x, w=None):
    d = x.shape[0]
    piv = x[0:1, :]
    xd = x - piv
    s1 = _red0(xd, jnp.add, jnp.sum, 8) * (1.0 / d)
    s2 = _red0(xd * xd, jnp.add, jnp.sum, 8) * (1.0 / d)
    mu, inv = _ln_finish(piv, s1, s2)
    if w is None:
        return mu, inv
    return mu, inv, _red0(xd * w, jnp.add, jnp.sum, 8), piv


def _kernel(c_hbm, wr_hbm, xt_hbm, k_hbm, v_hbm, wq_hbm, wot_hbm, wmod_hbm,
            wg_hbm, wu_hbm, wdt_hbm, out_hbm,
            x_sc, wmod_sc, kst, vst, wqst, wost, k_sc, vt_sc, wq_sc, wot_sc,
            h_sc, q_sc, s_sc, acc_sc, mod_sc, modt_sc, w_sc, out_sc, x1_sc, xs_sc, st_sc,
            zv_sc, z_ref, o_sc, c_sc, wr_sc, mrow_sc, wg_sc, wu_sc, wd_sc, wdst, u_sc,
            sems, xsems, lsems, osems, fsems):
    D, S = x_sc.shape
    Hkv, Sk, Dh = k_hbm.shape
    G = 2 * Dh
    nblk = S // TQ
    ngrp = nblk // 2
    GW = 2 * TQ
    NF = wdt_hbm.shape[1] // FW
    qscale = (Dh ** -0.5) * math.log2(math.e)
    ftiles = [(n, f0, min(128, D - f0)) for n, f0 in enumerate(range(0, D, 128))]

    def ds(i, n):
        return slice(i * n, (i + 1) * n) if isinstance(i, int) else pl.ds(pl.multiple_of(i * n, n), n)

    def cp_k(g, slot):
        return pltpu.make_async_copy(k_hbm.at[g], kst.at[slot], lsems.at[0, slot])

    def cp_wq(g, slot):
        return pltpu.make_async_copy(wq_hbm.at[:, ds(g, G)], wqst.at[slot], lsems.at[1, slot])

    def cp_v(g, slot):
        return pltpu.make_async_copy(v_hbm.at[g], vst.at[slot], lsems.at[2, slot])

    def cp_wo(g, slot):
        return pltpu.make_async_copy(wot_hbm.at[:, ds(g, G)], wost.at[slot], lsems.at[3, slot])

    def cp_wd(i, slot):
        return pltpu.make_async_copy(wdt_hbm.at[:, ds(jnp.minimum(i - 1, NF - 1), FW)], wdst.at[slot],
                                     lsems.at[4, slot])

    def cp_x(j):
        return pltpu.make_async_copy(xt_hbm.at[:, ds(j, GW)], x_sc.at[:, ds(j, GW)], xsems.at[j])

    def cp_out(b):
        return pltpu.make_async_copy(out_sc.at[b + 1], out_hbm.at[:, ds(b, TQ)], osems.at[b])

    moe = [pltpu.make_async_copy(wg_hbm, wg_sc, sems.at[0]),
           pltpu.make_async_copy(wu_hbm, wu_sc, sems.at[1])]
    cp_m0 = pltpu.make_async_copy(wmod_hbm.at[:, 0:2 * D], wmod_sc.at[:, 0:2 * D], sems.at[2])
    cp_m1 = pltpu.make_async_copy(wmod_hbm.at[:, 2 * D:6 * D], wmod_sc.at[:, 2 * D:6 * D], sems.at[3])
    cp_c = pltpu.make_async_copy(c_hbm, c_sc, sems.at[4])
    cp_wr = pltpu.make_async_copy(wr_hbm, wr_sc, sems.at[5])

    def tie(v, dep):
        return pltpu.bitcast(pltpu.bitcast(v, U32) | (dep & zv_sc[...]), v.dtype)

    def ln1_pair(g):
        piv = jnp.broadcast_to(x_sc[0:16, ds(g, GW)].astype(F32)[0:1], (8, GW))
        s1 = s2 = None
        for r0 in range(0, D, 16):
            pw = piv
            if s2 is not None:
                b2 = pltpu.bitcast(s2, U32)
                pw = jnp.concatenate([tie(piv[:, :TQ], b2[:, :TQ]), tie(piv[:, TQ:], b2[:, TQ:])], axis=1)
            xd = x_sc[r0:r0 + 16, ds(g, GW)].astype(F32) - jnp.concatenate([pw, pw], axis=0)
            xq = xd * xd
            p1 = xd[0:8] + xd[8:16]
            p2 = xq[0:8] + xq[8:16]
            s1 = p1 if s1 is None else s1 + p1
            s2 = p2 if s2 is None else s2 + p2
        mu, inv = _ln_finish(piv, jnp.sum(s1, axis=0, keepdims=True) * (1.0 / D),
                             jnp.sum(s2, axis=0, keepdims=True) * (1.0 / D))
        g2 = g + z_ref[0]
        for _, f0, fw in ftiles:
            x = x_sc[f0:f0 + fw, ds(g2, GW)].astype(F32)
            n = (x - jnp.concatenate([mu] * (fw // 8), axis=0)) * inv
            h = n.T * mod_sc[1:2, f0:f0 + fw] + mod_sc[0:1, f0:f0 + fw]
            h_sc[ds(g, TQ), f0:f0 + fw] = _pk(h.astype(BF16))
        return pltpu.bitcast(mu[:, 0:128], U32)

    def mod_part(j, dep):
        t0 = jnp.clip(2 * D // 128 + MT * (j - 3), 0, 6 * D // 128 - MT)
        cols = pl.ds(pl.multiple_of(t0 * 128, 128), MT * 128)
        acc = None
        for r0 in range(0, D, 16):
            sc = modt_sc[r0:r0 + 16, :]
            if acc is not None:
                dep = pltpu.bitcast(acc[:, 0:128], U32)
            sc = jnp.concatenate([tie(sc[0:8], dep), tie(sc[8:16], dep)], axis=0)
            pr = wmod_sc[r0:r0 + 16, cols].astype(F32) * jnp.concatenate([sc] * MT, axis=1)
            pr = pr[0:8] + pr[8:16]
            acc = pr if acc is None else acc + pr
        mrow_sc[:, cols] = jnp.sum(acc, axis=0, keepdims=True)

    def qproj(c):
        h = _upk(h_sc[ds(c, TQ // 2), :])
        q = jnp.dot(h, _upk(wq_sc[...]), preferred_element_type=F32)
        q = (q * qscale).astype(BF16)
        return jnp.concatenate([q[:, :Dh], q[:, Dh:]], axis=0)

    def qk(c, q, split=False):
        if split:
            st = jnp.concatenate([
                lax.dot_general(_upk(k_sc[ds(j, Sk // 4), :]), q, NT, preferred_element_type=F32)
                for j in range(2)], axis=0)
        else:
            st = lax.dot_general(_upk(k_sc[...]), q, NT, preferred_element_type=F32)
        s_sc[c, 0:Sk, :] = st
        s_sc[c, Sk:Sk + 8, :] = jnp.broadcast_to(_red0(st, jnp.maximum, jnp.max, 1), (8, 2 * TQ))

    def pv_cols(c, cols):
        p = jnp.exp2(s_sc[c, 0:Sk, cols] - s_sc[c, Sk:Sk + 1, cols])
        l = _red0(p, jnp.add, jnp.sum, 2)
        ot = jnp.dot(_upk(vt_sc[...]), p.astype(BF16), preferred_element_type=F32)
        return ot * (1.0 / l)

    def pv(c):
        ot = pv_cols(c, slice(0, 2 * TQ)).astype(BF16)
        return jnp.concatenate([ot[:, :TQ], ot[:, TQ:]], axis=0)

    def oproj(c, o2t, split=False, slot=None):
        if split:
            d = jnp.concatenate([
                jnp.dot(_upk(wot_sc[ds(j, D // 4), :]), o2t, preferred_element_type=F32)
                for j in range(2)], axis=0)
        else:
            d = jnp.dot(_upk(wot_sc[...]), o2t, preferred_element_type=F32)
        if slot is None:
            acc_sc[c] += d
        else:
            x1 = _rb(x_sc[:, ds(c, TQ)].astype(F32) + modt_sc[0:D, :] * (acc_sc[c] + d))
            xb = x1_sc.at[slot]
            xb[0:D, :] = x1
            mu, inv, rw, piv = _stats_t(x1, modt_sc[3 * D:4 * D, :])
            xb[D:D + 8, :] = jnp.broadcast_to(mu, (8, TQ))
            xb[D + 8:D + 16, :] = jnp.broadcast_to(inv, (8, TQ))
            st_sc[0, pl.ds(c, 1), :] = mu
            st_sc[1, pl.ds(c, 1), :] = inv
            st_sc[2, pl.ds(c, 1), :] = (rw - (mu - piv) * mod_sc[5:6, 0:TQ]) * inv + mod_sc[6:7, 0:TQ]

    def post(v0, slots, ch, cw, dist, slow):
        mu0 = [x1_sc[u, D:D + 8, :] for u in slots]
        inv0 = [x1_sc[u, D + 8:D + 16, :] for u in slots]
        for _, f0, fw in ftiles:
            words = []
            for r0 in range(f0, f0 + fw, 32):
                gc = modt_sc[D + r0:D + r0 + 32, :]
                gs = modt_sc[2 * D + r0:2 * D + r0 + 32, :]
                dep = ch[-dist] if len(ch) >= dist else None
                if r0 == f0 and len(cw) >= 3:
                    dep = dep | cw[-3]
                xs = []
                for u in range(len(slots)):
                    x1 = x1_sc[slots[u], r0:r0 + 32, :]
                    xs.append(x1)
                    mu = mu0[u] if dep is None else tie(mu0[u], dep)
                    mu = jnp.concatenate([mu] * 4, axis=0)
                    inv = jnp.concatenate([inv0[u]] * 4, axis=0)
                    o = x1 + ((x1 - mu) * inv * gc + gs)
                    out_sc[v0 + u, r0:r0 + 32, :] = o.astype(BF16)
                wd = pltpu.bitcast(xs[0], U32)
                if len(xs) > 1:
                    wd = wd | (pltpu.bitcast(xs[1], U32) >> 16)
                words.append(wd)
                dd = _pk(out_sc[z_ref[0], 0:16, :])
                ch.append(pltpu.roll(dd, 1, 1) if slow else dd)
            w_sc[ds(v0 // 2, TQ), f0:f0 + fw] = pltpu.bitcast(jnp.concatenate(words, axis=0), F32).T
            cw.append(pltpu.bitcast(w_sc[pl.ds(pl.multiple_of(z_ref[0], 8), 8), 0:128], U32))

    for cp in (cp_c, cp_x(0), cp_m0):
        cp.start()
    acc_sc[...] = jnp.zeros(acc_sc.shape, F32)
    x1_sc[...] = jnp.zeros(x1_sc.shape, F32)
    o_sc[...] = jnp.zeros(o_sc.shape, U32)
    st_sc[...] = jnp.zeros(st_sc.shape, F32)
    zv_sc[...] = jnp.zeros(zv_sc.shape, U32)
    z_ref[0] = 0
    u_sc[...] = jnp.zeros(u_sc.shape, F32)
    cp_c.wait()
    cp_wq(0, 0).start()
    cp_x(0).wait()
    cp_k(0, 0).start()
    c = c_sc[...].astype(F32)
    scb = (c * jax.nn.sigmoid(c)).astype(BF16)
    modt_sc[0:D, :] = jnp.broadcast_to(scb.astype(F32), (128, D)).T
    for cc in range(2):
        x = x_sc[:, ds(cc, TQ)].astype(F32)
        mu, inv = _stats_t(x)
        w_sc[ds(cc, TQ), :] = ((x - mu) * inv).T
    cp_m0.wait()
    cp_x(1).start()
    m = _rb(jnp.dot(jnp.broadcast_to(scb, (8, D)), wmod_sc[:, 0:2 * D], preferred_element_type=F32))
    sa = m[0:1, 0:D]
    ca1 = _rb(1.0 + m[0:1, D:2 * D])
    mod_sc[0:1, :] = sa
    mod_sc[1:2, :] = ca1
    h_sc[0:TQ, :] = _pk((w_sc[0:2 * TQ, :] * ca1 + sa).astype(BF16))
    cp_wq(0, 0).wait()
    wq_sc[...] = _pk(wqst[0])
    q_sc[0] = _pk(qproj(0))
    q_sc[1] = _pk(qproj(1))
    cp_k(0, 0).wait()
    cp_x(2).start()
    cp_x(3).start()
    k_sc[...] = _pk(kst[0])

    def first(j, carry):
        cp_x(j + 1).wait()

        @pl.when(j == 0)
        def _():
            cp_m1.start()

        @pl.when(j == 1)
        def _():
            for jj in range(4, ngrp):
                cp_x(jj).start()

        @pl.when(j == 3)
        def _():
            cp_m1.wait()

        @pl.when(j == 3)
        def _():
            for cp in (cp_v(0, 0), cp_wr, cp_k(1, 1), cp_wq(1, 1), cp_v(1, 1), cp_wo(0, 1), cp_wd(1, 1)):
                cp.start()
        qk(2 * j, _upk(q_sc[0]))
        qk(2 * j + 1, _upk(q_sc[1]))
        mod_part(j, ln1_pair(j + 1))
        q_sc[0] = _pk(qproj(2 * j + 2 + z_ref[0]))
        q_sc[1] = _pk(qproj(2 * j + 3 + z_ref[0]))
        return carry
    lax.fori_loop(0, ngrp - 1, first, 0)

    cp_wr.wait()
    cp_v(0, 0).wait()
    for cp in moe:
        cp.start()
    vt_sc[...] = _pk(vst[0].T)
    m = _rb(mrow_sc[:, 2 * D:6 * D])
    ga = m[0:1, 0:D]
    sb = m[0:1, D:2 * D]
    cb1 = _rb(1.0 + m[0:1, 2 * D:3 * D])
    gb = m[0:1, 3 * D:4 * D]
    wr = wr_sc[...].astype(F32).reshape(1, D)
    mod_sc[2:3, :] = gb
    mod_sc[3:4, :] = sb
    mod_sc[4:5, :] = cb1
    mod_sc[5:6, :] = jnp.broadcast_to(jnp.sum(wr * cb1, axis=1, keepdims=True), (1, D))
    mod_sc[6:7, :] = jnp.broadcast_to(jnp.sum(wr * sb, axis=1, keepdims=True), (1, D))
    for i, vec in enumerate((ga, gb * cb1, gb * sb, wr * cb1)):
        modt_sc[i * D:(i + 1) * D, :] = jnp.broadcast_to(vec, (128, D)).T
    qk(nblk - 2, _upk(q_sc[0]))
    qk(nblk - 1, _upk(q_sc[1]))

    def main(i, carry):
        slot = i & 1
        for cp in (cp_k(i, slot), cp_wq(i, slot), cp_v(i, slot), cp_wo(i - 1, slot), cp_wd(i, slot)):
            cp.wait()

        @pl.when(i + 1 < Hkv)
        def _():
            for cp in (cp_k(i + 1, 1 - slot), cp_wq(i + 1, 1 - slot), cp_v(i + 1, 1 - slot),
                       cp_wd(i + 1, 1 - slot)):
                cp.start()
        cp_wo(i, 1 - slot).start()

        wq_sc[...] = _pk(wqst[slot])
        k_sc[...] = _pk(kst[slot])
        wot_sc[...] = _pk(wost[slot])
        q = qproj(0)
        for c in range(nblk):
            end = c == nblk - 1
            o = pv(c)
            qn = None if end else qproj(c + 1)
            qk(c, q, split=end)
            oproj(c, o, split=end)
            q = qn
        vt_sc[...] = _pk(vst[slot].T)
        wd_sc[ds(jnp.minimum(i - 1, NF - 1), FW // 2), :] = _pk(wdst[slot].T)
        return carry
    lax.fori_loop(1, Hkv, main, 0)

    cp_wo(Hkv - 1, Hkv % 2).wait()
    wot_sc[...] = _pk(wost[Hkv % 2])

    def last(j, carry):
        ch, cw = [], []
        for u0 in range(0, LU, 2):
            post(LU * jnp.maximum(j - 1, 0) + u0, (u0, u0 + 1), ch, cw, 1, True)
        o = _upk(o_sc[...])
        for u in range(LU):
            c = LU * j + u - 1
            if u == 0:
                oproj(jnp.maximum(c, 0), o, slot=u)
                o0 = pv_cols(c + 1, slice(0, TQ))
            else:
                o0 = pv_cols(c + 1, slice(0, TQ))
                oproj(c, o, slot=u)
            o1 = pv_cols(c + 1, slice(TQ, 2 * TQ))
            o = jnp.concatenate([o0, o1], axis=0).astype(BF16)
        o_sc[...] = _pk(o)
        return carry
    lax.fori_loop(0, nblk // LU, last, 0)

    oproj(nblk - 1, _upk(o_sc[...]), split=True, slot=LU)

    r = _rb(st_sc[2]) + 0.0
    b16 = pltpu.bitcast(r, U32) >> 16
    ordk = jnp.where(b16 >= 0x8000, 0xFFFF - b16, b16 + 0x8000)
    tok = lax.broadcasted_iota(U32, r.shape, 0) * TQ + lax.broadcasted_iota(U32, r.shape, 1)
    key = pltpu.bitcast((ordk << 11) + (S - 1 - tok) + KEY_BIAS, F32)

    def rank(row, col):
        return _red0(jnp.where(col > row, 1.0, 0.0), jnp.add, jnp.sum, 16)

    lm = jnp.max(key, axis=0, keepdims=True)
    lrank = rank(lm, jnp.broadcast_to(lm, (TQ, TQ)).T)
    cand = jnp.concatenate([jnp.where(lrank == float(t), key, 0.0) for t in range(TOPC)], axis=0)
    cand = jnp.broadcast_to(jnp.max(cand, axis=1, keepdims=True), (TOPC * nblk, TQ))
    eye = lax.broadcasted_iota(I32, cand.shape, 0) == lax.broadcasted_iota(I32, cand.shape, 1)
    crow = _red0(jnp.where(eye, cand, 0.0), jnp.maximum, jnp.max, 16)
    crank = rank(crow, cand)
    subf = lax.broadcasted_iota(I32, (TOPC, TQ), 0).astype(F32)
    top = jnp.max(jnp.where(crank == subf, crow, 0.0), axis=1, keepdims=True)
    top = jnp.broadcast_to(top, (TOPC, TQ))
    mus = jnp.zeros((TOPC, TQ), F32)
    invs = jnp.zeros((TOPC, TQ), F32)
    for cc in range(nblk):
        sel = key[cc:cc + 1, :] == top
        mus = jnp.where(sel, st_sc[0, cc:cc + 1, :], mus)
        invs = jnp.where(sel, st_sc[1, cc:cc + 1, :], invs)
    ch, cw = [], []
    for u0 in range(0, LU, 2):
        post(nblk - LU + u0, (u0, u0 + 1), ch, cw, 2, False)
    post(nblk, (LU,), ch, cw, 2, False)
    topi = S - 1 - (pltpu.bitcast(top, I32) & (S - 1))
    rowi = ((((topi >> LG) + 1) >> 1) << LG) + (topi & (TQ - 1))
    for t in range(TOPC):
        xs_sc[t:t + 1, :] = w_sc[pl.ds(rowi[t, 0], 1), :]
    idxs = [topi[t, 0] for t in range(TOPC)]
    blks = [ix >> LG for ix in idxs]
    hmask = 0
    for t in range(TOPC):
        hmask = hmask | (1 << blks[t])
    clean = [((hmask >> b) & 1) == 0 for b in range(nblk)]
    for b in range(nblk):
        @pl.when(clean[b])
        def _():
            cp_out(b).start()
    ordt = (pltpu.bitcast(top, U32) - KEY_BIAS) >> 11
    rsel = pltpu.bitcast(jnp.where(ordt >= 0x8000, ordt - 0x8000, 0xFFFF - ordt) << 16, F32)[:, 0:1]
    mus = jnp.sum(mus, axis=1, keepdims=True)
    invs = jnp.sum(invs, axis=1, keepdims=True)
    words = pltpu.bitcast(xs_sc[...], U32)
    low = ((topi[:, 0:1] >> LG) & 1) == 0
    x1s = pltpu.bitcast(jnp.where(low, words << 16, words & jnp.uint32(0xFFFF0000)), F32)
    h2s = _rb(_rb(_rb(_rb(x1s - mus) * invs) * mod_sc[4:5, :]) + mod_sc[3:4, :])
    xsel = h2s.astype(BF16)

    for cp in moe:
        cp.wait()
    gt = _rb(jnp.dot(xsel, wg_sc[...], preferred_element_type=F32))
    ut = _rb(jnp.dot(xsel, wu_sc[...], preferred_element_type=F32))
    af = _rb(gt * jax.nn.sigmoid(gt)) * ut
    gate = _rb(jax.nn.sigmoid(rsel))
    lns = [ix & (TQ - 1) for ix in idxs]
    color, lead = [], []
    for t in range(TOPC):
        cl, dup = 0, False
        for s_ in range(t):
            cl = cl + (lns[s_] == lns[t]).astype(I32)
            dup = jnp.logical_or(dup, blks[s_] == blks[t])
        color.append(cl)
        lead.append(jnp.logical_not(dup))
    cmax = color[TOPC - 1]
    for t in range(1, TOPC - 1):
        cmax = jnp.maximum(cmax, color[t])

    def cp_fix(t, n, f0, fw):
        return pltpu.make_async_copy(out_sc.at[blks[t] + 1, f0:f0 + fw, :],
                                     out_hbm.at[f0:f0 + fw, ds(blks[t], TQ)], fsems.at[n])

    def scatter(rnd, n, f0, fw, new):
        now = [(color[t] >> 1) == rnd for t in range(TOPC)]
        for t in range(TOPC):
            row = jnp.where(now[t], lns[t] + (color[t] & 1) * TQ, 2 * TQ)
            u_sc[n, pl.ds(row, 1), 0:fw] = new[t:t + 1, :]
        ut_ = u_sc[n, 0:2 * TQ, 0:fw].T
        lane = lax.broadcasted_iota(I32, (fw, TQ), 1)
        for t in range(TOPC):
            val = ut_[:, :TQ] if t == 0 else jnp.where((color[t] & 1) == 0, ut_[:, :TQ], ut_[:, TQ:])
            cur = out_sc[blks[t] + 1, f0:f0 + fw, :].astype(F32)
            out_sc[blks[t] + 1, f0:f0 + fw, :] = jnp.where(
                lane == jnp.where(now[t], lns[t], TQ), val, cur).astype(BF16)

    kb = (af.shape[1] // 128) * 13 // 18 * 128
    fence, news = [], []
    for n, f0, fw in ftiles:
        an = af
        if n >= 2:
            an = jnp.concatenate([af[:, :kb], tie(af[:, kb:kb + 128], fence[n - 2]), af[:, kb + 128:]],
                                 axis=1)
        y = _rb(jnp.dot(an.astype(BF16), _upk(wd_sc[:, f0:f0 + fw]), preferred_element_type=F32))
        y = _rb(y * gate)
        new = x1s[:, f0:f0 + fw] + mod_sc[2:3, f0:f0 + fw] * _rb(h2s[:, f0:f0 + fw] + y)
        news.append(new)
        scatter(0, n, f0, fw, new)
        fence.append(_pk(out_sc[z_ref[0], 0:16, :]))
        for t in range(TOPC):
            @pl.when(lead[t])
            def _():
                cp_fix(t, n, f0, fw).start()
    xs_sc[...] = jnp.concatenate(news, axis=1)

    for b in range(nblk):
        @pl.when(clean[b])
        def _():
            cp_out(b).wait()
    for n, f0, fw in ftiles:
        for t in range(TOPC):
            @pl.when(lead[t])
            def _():
                cp_fix(t, n, f0, fw).wait()

    @pl.when(cmax >= 2)
    def _():
        def extra(rnd, carry):
            for n, f0, fw in ftiles:
                scatter(rnd, n, f0, fw, xs_sc[:, f0:f0 + fw])
            return carry
        lax.fori_loop(1, (cmax >> 1) + 1, extra, 0)
        for t in range(TOPC):
            @pl.when(lead[t])
            def _():
                cp_fix(t, 0, 0, D).start()
        for t in range(TOPC):
            @pl.when(lead[t])
            def _():
                cp_fix(t, 0, 0, D).wait()


@jax.jit
def pallas_adaLN_cond__gqa_block_cached__moe_arch_mod__prompt_kernel(
    A_x: jax.Array,
    A_k_cache: jax.Array,
    A_v_cache: jax.Array,
    A_wq: jax.Array,
    A_wo: jax.Array,
    B_x: jax.Array,
    B_w_r: jax.Array,
    B_w_gate: jax.Array,
    B_w_up: jax.Array,
    B_w_down: jax.Array,
    c: jax.Array,
    w_mod: jax.Array,
):
    del B_x
    B, S, D = A_x.shape
    _, Hkv, Sk, Dh = A_k_cache.shape
    G = A_wq.shape[1] // Hkv
    Fd = B_w_gate.shape[1]
    nblk = S // TQ
    assert B == 1 and G == 2 * Dh and TOPC * nblk == TQ and Fd % FW == 0 and Fd // FW < Hkv
    assert (2 * D) % 128 == 0 and 4 * D <= 4 * MT * 128 and MT * 128 <= 2 * D
    hbm = pl.BlockSpec(memory_space=pl.ANY)
    out_t = pl.pallas_call(
        _kernel,
        in_specs=[hbm] * 11,
        out_specs=hbm,
        out_shape=jax.ShapeDtypeStruct((D, S), BF16),
        scratch_shapes=[
            pltpu.VMEM((D, S), BF16),
            pltpu.VMEM((D, 6 * D), BF16),
            pltpu.VMEM((2, Sk, Dh), BF16),
            pltpu.VMEM((2, Sk, Dh), BF16),
            pltpu.VMEM((2, D, G), BF16),
            pltpu.VMEM((2, D, G), BF16),
            pltpu.VMEM((Sk // 2, Dh), U32),
            pltpu.VMEM((Dh // 2, Sk), U32),
            pltpu.VMEM((D // 2, G), U32),
            pltpu.VMEM((D // 2, G), U32),
            pltpu.VMEM((S // 2, D), U32),
            pltpu.VMEM((2, TQ, Dh), U32),
            pltpu.VMEM((nblk, Sk + 8, 2 * TQ), F32),
            pltpu.VMEM((nblk, D, TQ), F32),
            pltpu.VMEM((8, D), F32),
            pltpu.VMEM((4 * D, 128), F32),
            pltpu.VMEM((S // 2 + TQ, D), F32),
            pltpu.VMEM((nblk + 1, D, TQ), BF16),
            pltpu.VMEM((LU + 1, D + 16, TQ), F32),
            pltpu.VMEM((TOPC, D), F32),
            pltpu.VMEM((3, nblk, TQ), F32),
            pltpu.VMEM((8, 128), U32),
            pltpu.SMEM((1,), I32),
            pltpu.VMEM((Dh, TQ), U32),
            pltpu.VMEM((1, D), BF16),
            pltpu.VMEM((D,), BF16),
            pltpu.VMEM((1, 6 * D), F32),
            pltpu.VMEM((D, Fd), BF16),
            pltpu.VMEM((D, Fd), BF16),
            pltpu.VMEM((Fd // 2, D), U32),
            pltpu.VMEM((2, D, FW), BF16),
            pltpu.VMEM((pl.cdiv(D, 128), 2 * TQ + 8, 128), F32),
            pltpu.SemaphoreType.DMA((6,)),
            pltpu.SemaphoreType.DMA((nblk // 2,)),
            pltpu.SemaphoreType.DMA((5, 2)),
            pltpu.SemaphoreType.DMA((nblk,)),
            pltpu.SemaphoreType.DMA((pl.cdiv(D, 128),)),
        ],
        compiler_params=pltpu.CompilerParams(vmem_limit_bytes=110 * 1024 * 1024,
                                             disable_bounds_checks=True,
                                             disable_semaphore_checks=True),
    )(c, B_w_r, A_x.reshape(S, D).T, A_k_cache.reshape(Hkv, Sk, Dh), A_v_cache.reshape(Hkv, Sk, Dh),
      A_wq, A_wo.T, w_mod, B_w_gate, B_w_up, B_w_down.T)
    return out_t.T.reshape(B, S, D)
```

```python
import math

import jax
import jax.numpy as jnp
from jax import lax
import jax.experimental.pallas as pl
import jax.experimental.pallas.tpu as pltpu

F32 = jnp.float32
BF16 = jnp.bfloat16
U32 = jnp.uint32
I32 = jnp.int32
EPS = 1e-05
TOPC = 8
NT = (((1,), (1,)), ((), ()))
TQ = 128
LG = 7
LU = 4
FW = 3 * 128
MT = 5
KEY_BIAS = 0x20000000


def _pk(x):
    return pltpu.bitcast(x, U32)


def _upk(x):
    return pltpu.bitcast(x, BF16)


def _rb(x):
    return x.astype(BF16).astype(F32)


def _tree(xs, op):
    while len(xs) > 1:
        xs = [op(xs[i], xs[i + 1]) if i + 1 < len(xs) else xs[i] for i in range(0, len(xs), 2)]
    return xs[0]


def _red0(x, op, red, grp):
    n = x.shape[0]
    acc = None
    for t in range(0, n, 8 * grp):
        part = _tree([x[j:j + 8, :] for j in range(t, min(t + 8 * grp, n), 8)], op)
        acc = part if acc is None else op(acc, part)
    return red(acc, axis=0, keepdims=True)


def _ln_finish(piv, s1, s2):
    var = jnp.maximum(s2 - s1 * s1, 0.0)
    return _rb(piv + s1), 1.0 / _rb(jnp.sqrt(_rb(_rb(var) + EPS)))


def _stats_t(x, w=None):
    d = x.shape[0]
    piv = x[0:1, :]
    xd = x - piv
    s1 = _red0(xd, jnp.add, jnp.sum, 8) * (1.0 / d)
    s2 = _red0(xd * xd, jnp.add, jnp.sum, 8) * (1.0 / d)
    mu, inv = _ln_finish(piv, s1, s2)
    if w is None:
        return mu, inv
    return mu, inv, _red0(xd * w, jnp.add, jnp.sum, 8), piv


def _kernel(c_hbm, wr_hbm, xt_hbm, k_hbm, v_hbm, wq_hbm, wot_hbm, wmod_hbm,
            wg_hbm, wu_hbm, wdt_hbm, out_hbm,
            x_sc, wmod_sc, kvst, wst, k_sc, vt_sc, wq_sc, wot_sc,
            h_sc, q_sc, s_sc, acc_sc, mod_sc, modt_sc, w_sc, out_sc, x1_sc, xs_sc, st_sc,
            zv_sc, z_ref, o_sc, c_sc, wr_sc, mrow_sc, wg_sc, wu_sc, wd_sc, u_sc,
            sems, xsems, lsems, osems, fsems):
    D, S = x_sc.shape
    Hkv, Sk, Dh = k_hbm.shape
    G = 2 * Dh
    nblk = S // TQ
    ngrp = nblk // 2
    GW = 2 * TQ
    NF = wdt_hbm.shape[1] // FW
    qscale = (Dh ** -0.5) * math.log2(math.e)
    ftiles = [(n, f0, min(128, D - f0)) for n, f0 in enumerate(range(0, D, 128))]

    def ds(i, n):
        return slice(i * n, (i + 1) * n) if isinstance(i, int) else pl.ds(pl.multiple_of(i * n, n), n)

    def cp_k(g, slot, sem):
        return pltpu.make_async_copy(k_hbm.at[g], kvst.at[slot, 0:Sk, :], sem)

    def cp_v(g, slot, sem):
        return pltpu.make_async_copy(v_hbm.at[g], kvst.at[slot, Sk:2 * Sk, :], sem)

    def cp_wq(g, slot, sem):
        return pltpu.make_async_copy(wq_hbm.at[:, ds(g, G)], wst.at[slot, :, 0:G], sem)

    def cp_wo(g, slot, sem):
        return pltpu.make_async_copy(wot_hbm.at[:, ds(g, G)], wst.at[slot, :, G:2 * G], sem)

    def start_head(i, slot):
        cp_wq(i, slot, lsems.at[0]).start()
        cp_wo(i - 1, slot, lsems.at[0]).start()
        pltpu.make_async_copy(wdt_hbm.at[:, ds(jnp.minimum(i - 1, NF - 1), FW)],
                              wst.at[slot, :, 2 * G:2 * G + FW], lsems.at[0]).start()
        cp_k(i, slot, lsems.at[1]).start()
        cp_v(i, slot, lsems.at[1]).start()

    def wait_head(slot):
        pltpu.make_async_copy(wst.at[slot], wst.at[slot], lsems.at[0]).wait()
        pltpu.make_async_copy(kvst.at[slot], kvst.at[slot], lsems.at[1]).wait()

    def cp_x(j):
        return pltpu.make_async_copy(xt_hbm.at[:, ds(j, GW)], x_sc.at[:, ds(j, GW)], xsems.at[j])

    def cp_out(b):
        return pltpu.make_async_copy(out_sc.at[b + 1], out_hbm.at[:, ds(b, TQ)], osems.at[b])

    moe = [pltpu.make_async_copy(wg_hbm, wg_sc, sems.at[0]),
           pltpu.make_async_copy(wu_hbm, wu_sc, sems.at[1])]
    cp_m0 = pltpu.make_async_copy(wmod_hbm.at[:, 0:2 * D], wmod_sc.at[:, 0:2 * D], sems.at[2])
    cp_m1 = pltpu.make_async_copy(wmod_hbm.at[:, 2 * D:6 * D], wmod_sc.at[:, 2 * D:6 * D], sems.at[3])
    cp_c = pltpu.make_async_copy(c_hbm, c_sc, sems.at[4])
    cp_wr = pltpu.make_async_copy(wr_hbm, wr_sc, sems.at[5])
    cp_v0 = cp_v(0, 0, sems.at[6])
    cp_k0 = cp_k(0, 0, sems.at[7])
    cp_wq0 = cp_wq(0, 0, sems.at[8])
    cp_wol = cp_wo(Hkv - 1, Hkv % 2, sems.at[9])

    def tie(v, dep):
        return pltpu.bitcast(pltpu.bitcast(v, U32) | (dep & zv_sc[...]), v.dtype)

    def ln1_pair(g):
        piv = jnp.broadcast_to(x_sc[0:16, ds(g, GW)].astype(F32)[0:1], (8, GW))
        s1 = s2 = None
        for r0 in range(0, D, 16):
            pw = piv
            if s2 is not None:
                b2 = pltpu.bitcast(s2, U32)
                pw = jnp.concatenate([tie(piv[:, :TQ], b2[:, :TQ]), tie(piv[:, TQ:], b2[:, TQ:])], axis=1)
            xd = x_sc[r0:r0 + 16, ds(g, GW)].astype(F32) - jnp.concatenate([pw, pw], axis=0)
            xq = xd * xd
            p1 = xd[0:8] + xd[8:16]
            p2 = xq[0:8] + xq[8:16]
            s1 = p1 if s1 is None else s1 + p1
            s2 = p2 if s2 is None else s2 + p2
        mu, inv = _ln_finish(piv, jnp.sum(s1, axis=0, keepdims=True) * (1.0 / D),
                             jnp.sum(s2, axis=0, keepdims=True) * (1.0 / D))
        g2 = g + z_ref[0]
        for _, f0, fw in ftiles:
            x = x_sc[f0:f0 + fw, ds(g2, GW)].astype(F32)
            n = (x - jnp.concatenate([mu] * (fw // 8), axis=0)) * inv
            h = n.T * mod_sc[1:2, f0:f0 + fw] + mod_sc[0:1, f0:f0 + fw]
            h_sc[ds(g, TQ), f0:f0 + fw] = _pk(h.astype(BF16))
        return h_sc[pl.ds(pl.multiple_of(z_ref[0], 8), 8), 0:128]

    def mod_part(j, dep):
        t0 = jnp.clip(2 * D // 128 + MT * (j - 3), 0, 6 * D // 128 - MT)
        cols = pl.ds(pl.multiple_of(t0 * 128, 128), MT * 128)
        acc = None
        for r0 in range(0, D, 16):
            sc = modt_sc[r0:r0 + 16, :]
            if acc is not None:
                dep = pltpu.bitcast(acc[:, 0:128], U32)
            sc = jnp.concatenate([tie(sc[0:8], dep), tie(sc[8:16], dep)], axis=0)
            pr = wmod_sc[r0:r0 + 16, cols].astype(F32) * jnp.concatenate([sc] * MT, axis=1)
            pr = pr[0:8] + pr[8:16]
            acc = pr if acc is None else acc + pr
        mrow_sc[:, cols] = jnp.sum(acc, axis=0, keepdims=True)

    def qproj(c):
        h = _upk(h_sc[ds(c, TQ // 2), :])
        q = jnp.dot(h, _upk(wq_sc[...]), preferred_element_type=F32)
        q = (q * qscale).astype(BF16)
        return jnp.concatenate([q[:, :Dh], q[:, Dh:]], axis=0)

    def qk(c, q, split=False):
        if split:
            st = jnp.concatenate([
                lax.dot_general(_upk(k_sc[ds(j, Sk // 4), :]), q, NT, preferred_element_type=F32)
                for j in range(2)], axis=0)
        else:
            st = lax.dot_general(_upk(k_sc[...]), q, NT, preferred_element_type=F32)
        s_sc[c, 0:Sk, :] = st
        s_sc[c, Sk:Sk + 8, :] = jnp.broadcast_to(_red0(st, jnp.maximum, jnp.max, 1), (8, 2 * TQ))

    def pv_cols(c, cols):
        p = jnp.exp2(s_sc[c, 0:Sk, cols] - s_sc[c, Sk:Sk + 1, cols])
        l = _red0(p, jnp.add, jnp.sum, 2)
        ot = jnp.dot(_upk(vt_sc[...]), p.astype(BF16), preferred_element_type=F32)
        return ot * (1.0 / l)

    def pv(c):
        ot = pv_cols(c, slice(0, 2 * TQ)).astype(BF16)
        return jnp.concatenate([ot[:, :TQ], ot[:, TQ:]], axis=0)

    def oproj(c, o2t, split=False, slot=None):
        if split:
            d = jnp.concatenate([
                jnp.dot(_upk(wot_sc[ds(j, D // 4), :]), o2t, preferred_element_type=F32)
                for j in range(2)], axis=0)
        else:
            d = jnp.dot(_upk(wot_sc[...]), o2t, preferred_element_type=F32)
        if slot is None:
            acc_sc[c] += d
        else:
            x1 = _rb(x_sc[:, ds(c, TQ)].astype(F32) + modt_sc[0:D, :] * (acc_sc[c] + d))
            xb = x1_sc.at[slot]
            xb[0:D, :] = x1
            mu, inv, rw, piv = _stats_t(x1, modt_sc[3 * D:4 * D, :])
            xb[D:D + 8, :] = jnp.broadcast_to(mu, (8, TQ))
            xb[D + 8:D + 16, :] = jnp.broadcast_to(inv, (8, TQ))
            st_sc[0, pl.ds(c, 1), :] = mu
            st_sc[1, pl.ds(c, 1), :] = inv
            st_sc[2, pl.ds(c, 1), :] = (rw - (mu - piv) * mod_sc[5:6, 0:TQ]) * inv + mod_sc[6:7, 0:TQ]

    def post(v0, slots, ch, cw, dist, slow):
        mu0 = [x1_sc[u, D:D + 8, :] for u in slots]
        inv0 = [x1_sc[u, D + 8:D + 16, :] for u in slots]
        for _, f0, fw in ftiles:
            words = []
            for r0 in range(f0, f0 + fw, 32):
                gc = modt_sc[D + r0:D + r0 + 32, :]
                gs = modt_sc[2 * D + r0:2 * D + r0 + 32, :]
                dep = ch[-dist] if len(ch) >= dist else None
                if r0 == f0 and len(cw) >= 3:
                    dep = dep | cw[-3]
                xs = []
                for u in range(len(slots)):
                    x1 = x1_sc[slots[u], r0:r0 + 32, :]
                    xs.append(x1)
                    mu = mu0[u] if dep is None else tie(mu0[u], dep)
                    mu = jnp.concatenate([mu] * 4, axis=0)
                    inv = jnp.concatenate([inv0[u]] * 4, axis=0)
                    o = x1 + ((x1 - mu) * inv * gc + gs)
                    out_sc[v0 + u, r0:r0 + 32, :] = o.astype(BF16)
                wd = pltpu.bitcast(xs[0], U32)
                if len(xs) > 1:
                    wd = wd | (pltpu.bitcast(xs[1], U32) >> 16)
                words.append(wd)
                dd = _pk(out_sc[z_ref[0], 0:16, :])
                ch.append(pltpu.roll(dd, 1, 1) if slow else dd)
            w_sc[ds(v0 // 2, TQ), f0:f0 + fw] = pltpu.bitcast(jnp.concatenate(words, axis=0), F32).T
            cw.append(pltpu.bitcast(w_sc[pl.ds(pl.multiple_of(z_ref[0], 8), 8), 0:128], U32))

    for cp in (cp_c, cp_x(0), cp_m0):
        cp.start()
    acc_sc[...] = jnp.zeros(acc_sc.shape, F32)
    x1_sc[...] = jnp.zeros(x1_sc.shape, F32)
    o_sc[...] = jnp.zeros(o_sc.shape, U32)
    st_sc[...] = jnp.zeros(st_sc.shape, F32)
    zv_sc[...] = jnp.zeros(zv_sc.shape, U32)
    z_ref[0] = 0
    u_sc[...] = jnp.zeros(u_sc.shape, F32)
    cp_c.wait()
    cp_wq0.start()
    cp_x(0).wait()
    cp_k0.start()
    c = c_sc[...].astype(F32)
    scb = (c * jax.nn.sigmoid(c)).astype(BF16)
    modt_sc[0:D, :] = jnp.broadcast_to(scb.astype(F32), (128, D)).T
    for cc in range(2):
        x = x_sc[:, ds(cc, TQ)].astype(F32)
        mu, inv = _stats_t(x)
        w_sc[ds(cc, TQ), :] = ((x - mu) * inv).T
    cp_m0.wait()
    cp_x(1).start()
    m = _rb(jnp.dot(jnp.broadcast_to(scb, (8, D)), wmod_sc[:, 0:2 * D], preferred_element_type=F32))
    sa = m[0:1, 0:D]
    ca1 = _rb(1.0 + m[0:1, D:2 * D])
    mod_sc[0:1, :] = sa
    mod_sc[1:2, :] = ca1
    h_sc[0:TQ, :] = _pk((w_sc[0:2 * TQ, :] * ca1 + sa).astype(BF16))
    cp_wq0.wait()
    cp_x(2).start()
    cp_x(3).start()
    wq_sc[...] = _pk(wst[0, :, 0:G])
    q_sc[0] = _pk(qproj(0))
    q_sc[1] = _pk(qproj(1))
    cp_k0.wait()
    cp_m1.start()
    k_sc[...] = _pk(kvst[0, 0:Sk, :])

    def first(j, carry):
        cp_x(j + 1).wait()

        @pl.when(j == 3)
        def _():
            cp_m1.wait()

        @pl.when(j == 0)
        def _():
            for jj in range(4, ngrp):
                cp_x(jj).start()

        @pl.when(j == 2)
        def _():
            cp_v0.start()
            cp_wr.start()
            start_head(1, 1)
        qk(2 * j, _upk(q_sc[0]))
        qk(2 * j + 1, _upk(q_sc[1]))
        dep = ln1_pair(j + 1)
        q_sc[0] = _pk(qproj(2 * j + 2 + z_ref[0]))
        q_sc[1] = _pk(qproj(2 * j + 3 + z_ref[0]))
        mod_part(j, dep)
        return carry
    lax.fori_loop(0, ngrp - 1, first, 0)

    cp_wr.wait()
    cp_v0.wait()
    for cp in moe:
        cp.start()
    vt_sc[...] = _pk(kvst[0, Sk:2 * Sk, :].T)
    m = _rb(mrow_sc[:, 2 * D:6 * D])
    ga = m[0:1, 0:D]
    sb = m[0:1, D:2 * D]
    cb1 = _rb(1.0 + m[0:1, 2 * D:3 * D])
    gb = m[0:1, 3 * D:4 * D]
    wr = wr_sc[...].astype(F32).reshape(1, D)
    mod_sc[2:3, :] = gb
    mod_sc[3:4, :] = sb
    mod_sc[4:5, :] = cb1
    mod_sc[5:6, :] = jnp.broadcast_to(jnp.sum(wr * cb1, axis=1, keepdims=True), (1, D))
    mod_sc[6:7, :] = jnp.broadcast_to(jnp.sum(wr * sb, axis=1, keepdims=True), (1, D))
    for i, vec in enumerate((ga, gb * cb1, gb * sb, wr * cb1)):
        modt_sc[i * D:(i + 1) * D, :] = jnp.broadcast_to(vec, (128, D)).T
    qk(nblk - 2, _upk(q_sc[0]))
    qk(nblk - 1, _upk(q_sc[1]))

    def main(i, carry):
        slot = i & 1
        wait_head(slot)
        wq_sc[...] = _pk(wst[slot, :, 0:G])

        @pl.when(i + 1 < Hkv)
        def _():
            start_head(i + 1, 1 - slot)

        @pl.when(i + 1 == Hkv)
        def _():
            cp_wol.start()

        k_sc[...] = _pk(kvst[slot, 0:Sk, :])
        wot_sc[...] = _pk(wst[slot, :, G:2 * G])
        q = qproj(0)
        for c in range(nblk):
            end = c == nblk - 1
            o = pv(c)
            qn = None if end else qproj(c + 1)
            qk(c, q, split=end)
            oproj(c, o, split=end)
            q = qn
        vt_sc[...] = _pk(kvst[slot, Sk:2 * Sk, :].T)
        wd_sc[ds(jnp.minimum(i - 1, NF - 1), FW // 2), :] = _pk(wst[slot, :, 2 * G:2 * G + FW].T)
        return carry
    lax.fori_loop(1, Hkv, main, 0)

    cp_wol.wait()
    wot_sc[...] = _pk(wst[Hkv % 2, :, G:2 * G])

    def last(j, carry):
        ch, cw = [], []
        for u0 in range(0, LU, 2):
            post(LU * jnp.maximum(j - 1, 0) + u0, (u0, u0 + 1), ch, cw, 1, True)
        o = _upk(o_sc[...])
        for u in range(LU):
            c = LU * j + u - 1
            if u == 0:
                oproj(jnp.maximum(c, 0), o, slot=u)
                o0 = pv_cols(c + 1, slice(0, TQ))
            else:
                o0 = pv_cols(c + 1, slice(0, TQ))
                oproj(c, o, slot=u)
            o1 = pv_cols(c + 1, slice(TQ, 2 * TQ))
            o = jnp.concatenate([o0, o1], axis=0).astype(BF16)
        o_sc[...] = _pk(o)
        return carry
    lax.fori_loop(0, nblk // LU, last, 0)

    oproj(nblk - 1, _upk(o_sc[...]), split=True, slot=LU)

    r = _rb(st_sc[2]) + 0.0
    b16 = pltpu.bitcast(r, U32) >> 16
    ordk = jnp.where(b16 >= 0x8000, 0xFFFF - b16, b16 + 0x8000)
    tok = lax.broadcasted_iota(U32, r.shape, 0) * TQ + lax.broadcasted_iota(U32, r.shape, 1)
    key = pltpu.bitcast((ordk << 11) + (S - 1 - tok) + KEY_BIAS, F32)

    def rank(row, col):
        return _red0(jnp.where(col > row, 1.0, 0.0), jnp.add, jnp.sum, 16)

    lm = jnp.max(key, axis=0, keepdims=True)
    lrank = rank(lm, jnp.broadcast_to(lm, (TQ, TQ)).T)
    cand = jnp.concatenate([jnp.where(lrank == float(t), key, 0.0) for t in range(TOPC)], axis=0)
    cand = jnp.broadcast_to(jnp.max(cand, axis=1, keepdims=True), (TOPC * nblk, TQ))
    eye = lax.broadcasted_iota(I32, cand.shape, 0) == lax.broadcasted_iota(I32, cand.shape, 1)
    crow = _red0(jnp.where(eye, cand, 0.0), jnp.maximum, jnp.max, 16)
    crank = rank(crow, cand)
    subf = lax.broadcasted_iota(I32, (TOPC, TQ), 0).astype(F32)
    top = jnp.max(jnp.where(crank == subf, crow, 0.0), axis=1, keepdims=True)
    top = jnp.broadcast_to(top, (TOPC, TQ))
    mus = jnp.zeros((TOPC, TQ), F32)
    invs = jnp.zeros((TOPC, TQ), F32)
    for cc in range(nblk):
        sel = key[cc:cc + 1, :] == top
        mus = jnp.where(sel, st_sc[0, cc:cc + 1, :], mus)
        invs = jnp.where(sel, st_sc[1, cc:cc + 1, :], invs)
    ch, cw = [], []
    for u0 in range(0, LU, 2):
        post(nblk - LU + u0, (u0, u0 + 1), ch, cw, 2, False)
    post(nblk, (LU,), ch, cw, 2, False)
    topi = S - 1 - (pltpu.bitcast(top, I32) & (S - 1))
    rowi = ((((topi >> LG) + 1) >> 1) << LG) + (topi & (TQ - 1))
    for t in range(TOPC):
        xs_sc[t:t + 1, :] = w_sc[pl.ds(rowi[t, 0], 1), :]
    idxs = [topi[t, 0] for t in range(TOPC)]
    blks = [ix >> LG for ix in idxs]
    hmask = 0
    for t in range(TOPC):
        hmask = hmask | (1 << blks[t])
    clean = [((hmask >> b) & 1) == 0 for b in range(nblk)]
    for b in range(nblk):
        @pl.when(clean[b])
        def _():
            cp_out(b).start()
    ordt = (pltpu.bitcast(top, U32) - KEY_BIAS) >> 11
    rsel = pltpu.bitcast(jnp.where(ordt >= 0x8000, ordt - 0x8000, 0xFFFF - ordt) << 16, F32)[:, 0:1]
    mus = jnp.sum(mus, axis=1, keepdims=True)
    invs = jnp.sum(invs, axis=1, keepdims=True)
    words = pltpu.bitcast(xs_sc[...], U32)
    low = ((topi[:, 0:1] >> LG) & 1) == 0
    x1s = pltpu.bitcast(jnp.where(low, words << 16, words & jnp.uint32(0xFFFF0000)), F32)
    h2s = _rb(_rb(_rb(_rb(x1s - mus) * invs) * mod_sc[4:5, :]) + mod_sc[3:4, :])
    xsel = h2s.astype(BF16)

    for cp in moe:
        cp.wait()
    gt = _rb(jnp.dot(xsel, wg_sc[...], preferred_element_type=F32))
    ut = _rb(jnp.dot(xsel, wu_sc[...], preferred_element_type=F32))
    af = _rb(gt * jax.nn.sigmoid(gt)) * ut
    gate = _rb(jax.nn.sigmoid(rsel))
    lns = [ix & (TQ - 1) for ix in idxs]
    color, lead = [], []
    for t in range(TOPC):
        cl, dup = 0, False
        for s_ in range(t):
            cl = cl + (lns[s_] == lns[t]).astype(I32)
            dup = jnp.logical_or(dup, blks[s_] == blks[t])
        color.append(cl)
        lead.append(jnp.logical_not(dup))
    cmax = color[TOPC - 1]
    for t in range(1, TOPC - 1):
        cmax = jnp.maximum(cmax, color[t])

    def cp_fix(t, n, f0, fw):
        return pltpu.make_async_copy(out_sc.at[blks[t] + 1, f0:f0 + fw, :],
                                     out_hbm.at[f0:f0 + fw, ds(blks[t], TQ)], fsems.at[n])

    def scatter(rnd, n, f0, fw, new):
        now = [(color[t] >> 1) == rnd for t in range(TOPC)]
        for t in range(TOPC):
            row = jnp.where(now[t], lns[t] + (color[t] & 1) * TQ, 2 * TQ)
            u_sc[n, pl.ds(row, 1), 0:fw] = new[t:t + 1, :]
        ut_ = u_sc[n, 0:2 * TQ, 0:fw].T
        lane = lax.broadcasted_iota(I32, (fw, TQ), 1)
        for t in range(TOPC):
            val = ut_[:, :TQ] if t == 0 else jnp.where((color[t] & 1) == 0, ut_[:, :TQ], ut_[:, TQ:])
            cur = out_sc[blks[t] + 1, f0:f0 + fw, :].astype(F32)
            out_sc[blks[t] + 1, f0:f0 + fw, :] = jnp.where(
                lane == jnp.where(now[t], lns[t], TQ), val, cur).astype(BF16)

    kb = (af.shape[1] // 128) * 13 // 18 * 128
    fence, news = [], []
    for n, f0, fw in ftiles:
        an = af
        if n >= 2:
            an = jnp.concatenate([af[:, :kb], tie(af[:, kb:kb + 128], fence[n - 2]), af[:, kb + 128:]],
                                 axis=1)
        y = _rb(jnp.dot(an.astype(BF16), _upk(wd_sc[:, f0:f0 + fw]), preferred_element_type=F32))
        y = _rb(y * gate)
        new = x1s[:, f0:f0 + fw] + mod_sc[2:3, f0:f0 + fw] * _rb(h2s[:, f0:f0 + fw] + y)
        news.append(new)
        scatter(0, n, f0, fw, new)
        fence.append(_pk(out_sc[z_ref[0], 0:16, :]))
        for t in range(TOPC):
            @pl.when(lead[t])
            def _():
                cp_fix(t, n, f0, fw).start()
    xs_sc[...] = jnp.concatenate(news, axis=1)

    for b in range(nblk):
        @pl.when(clean[b])
        def _():
            cp_out(b).wait()
    for n, f0, fw in ftiles:
        for t in range(TOPC):
            @pl.when(lead[t])
            def _():
                cp_fix(t, n, f0, fw).wait()

    @pl.when(cmax >= 2)
    def _():
        def extra(rnd, carry):
            for n, f0, fw in ftiles:
                scatter(rnd, n, f0, fw, xs_sc[:, f0:f0 + fw])
            return carry
        lax.fori_loop(1, (cmax >> 1) + 1, extra, 0)
        for t in range(TOPC):
            @pl.when(lead[t])
            def _():
                cp_fix(t, 0, 0, D).start()
        for t in range(TOPC):
            @pl.when(lead[t])
            def _():
                cp_fix(t, 0, 0, D).wait()


@jax.jit
def pallas_adaLN_cond__gqa_block_cached__moe_arch_mod__prompt_kernel(
    A_x: jax.Array,
    A_k_cache: jax.Array,
    A_v_cache: jax.Array,
    A_wq: jax.Array,
    A_wo: jax.Array,
    B_x: jax.Array,
    B_w_r: jax.Array,
    B_w_gate: jax.Array,
    B_w_up: jax.Array,
    B_w_down: jax.Array,
    c: jax.Array,
    w_mod: jax.Array,
):
    del B_x
    B, S, D = A_x.shape
    _, Hkv, Sk, Dh = A_k_cache.shape
    G = A_wq.shape[1] // Hkv
    Fd = B_w_gate.shape[1]
    nblk = S // TQ
    assert B == 1 and G == 2 * Dh and TOPC * nblk == TQ and Fd % FW == 0 and Fd // FW < Hkv
    assert (2 * D) % 128 == 0 and 4 * D <= 4 * MT * 128 and MT * 128 <= 2 * D
    hbm = pl.BlockSpec(memory_space=pl.ANY)
    out_t = pl.pallas_call(
        _kernel,
        in_specs=[hbm] * 11,
        out_specs=hbm,
        out_shape=jax.ShapeDtypeStruct((D, S), BF16),
        scratch_shapes=[
            pltpu.VMEM((D, S), BF16),
            pltpu.VMEM((D, 6 * D), BF16),
            pltpu.VMEM((2, 2 * Sk, Dh), BF16),
            pltpu.VMEM((2, D, 2 * G + FW), BF16),
            pltpu.VMEM((Sk // 2, Dh), U32),
            pltpu.VMEM((Dh // 2, Sk), U32),
            pltpu.VMEM((D // 2, G), U32),
            pltpu.VMEM((D // 2, G), U32),
            pltpu.VMEM((S // 2, D), U32),
            pltpu.VMEM((2, TQ, Dh), U32),
            pltpu.VMEM((nblk, Sk + 8, 2 * TQ), F32),
            pltpu.VMEM((nblk, D, TQ), F32),
            pltpu.VMEM((8, D), F32),
            pltpu.VMEM((4 * D, 128), F32),
            pltpu.VMEM((S // 2 + TQ, D), F32),
            pltpu.VMEM((nblk + 1, D, TQ), BF16),
            pltpu.VMEM((LU + 1, D + 16, TQ), F32),
            pltpu.VMEM((TOPC, D), F32),
            pltpu.VMEM((3, nblk, TQ), F32),
            pltpu.VMEM((8, 128), U32),
            pltpu.SMEM((1,), I32),
            pltpu.VMEM((Dh, TQ), U32),
            pltpu.VMEM((1, D), BF16),
            pltpu.VMEM((D,), BF16),
            pltpu.VMEM((1, 6 * D), F32),
            pltpu.VMEM((D, Fd), BF16),
            pltpu.VMEM((D, Fd), BF16),
            pltpu.VMEM((Fd // 2, D), U32),
            pltpu.VMEM((pl.cdiv(D, 128), 2 * TQ + 8, 128), F32),
            pltpu.SemaphoreType.DMA((10,)),
            pltpu.SemaphoreType.DMA((nblk // 2,)),
            pltpu.SemaphoreType.DMA((2,)),
            pltpu.SemaphoreType.DMA((nblk,)),
            pltpu.SemaphoreType.DMA((pl.cdiv(D, 128),)),
        ],
        compiler_params=pltpu.CompilerParams(vmem_limit_bytes=110 * 1024 * 1024,
                                             disable_bounds_checks=True,
                                             disable_semaphore_checks=True),
    )(c, B_w_r, A_x.reshape(S, D).T, A_k_cache.reshape(Hkv, Sk, Dh), A_v_cache.reshape(Hkv, Sk, Dh),
      A_wq, A_wo.T, w_mod, B_w_gate, B_w_up, B_w_down.T)
    return out_t.T.reshape(B, S, D)
```

```python
import math

import jax
import jax.numpy as jnp
from jax import lax
import jax.experimental.pallas as pl
import jax.experimental.pallas.tpu as pltpu

F32 = jnp.float32
BF16 = jnp.bfloat16
U32 = jnp.uint32
I32 = jnp.int32
EPS = 1e-05
TOPC = 8
NT = (((1,), (1,)), ((), ()))
TQ = 128
LG = 7
LU = 4
FW = 3 * 128
MT = 3
KEY_BIAS = 0x20000000


def _pk(x):
    return pltpu.bitcast(x, U32)


def _upk(x):
    return pltpu.bitcast(x, BF16)


def _rb(x):
    return x.astype(BF16).astype(F32)


def _tree(xs, op):
    while len(xs) > 1:
        xs = [op(xs[i], xs[i + 1]) if i + 1 < len(xs) else xs[i] for i in range(0, len(xs), 2)]
    return xs[0]


def _red0(x, op, red, grp):
    n = x.shape[0]
    acc = None
    for t in range(0, n, 8 * grp):
        part = _tree([x[j:j + 8, :] for j in range(t, min(t + 8 * grp, n), 8)], op)
        acc = part if acc is None else op(acc, part)
    return red(acc, axis=0, keepdims=True)


def _ln_finish(piv, s1, s2):
    var = jnp.maximum(s2 - s1 * s1, 0.0)
    return _rb(piv + s1), 1.0 / _rb(jnp.sqrt(_rb(_rb(var) + EPS)))


def _stats_t(x, w=None):
    d = x.shape[0]
    piv = x[0:1, :]
    xd = x - piv
    s1 = _red0(xd, jnp.add, jnp.sum, 8) * (1.0 / d)
    s2 = _red0(xd * xd, jnp.add, jnp.sum, 8) * (1.0 / d)
    mu, inv = _ln_finish(piv, s1, s2)
    if w is None:
        return mu, inv
    return mu, inv, _red0(xd * w, jnp.add, jnp.sum, 8), piv


def _kernel(c_hbm, wr_hbm, xt_hbm, k_hbm, v_hbm, wq_hbm, wot_hbm, wmod_hbm,
            wg_hbm, wu_hbm, wdt_hbm, out_hbm,
            x_sc, wmod_sc, kvst, wst, k_sc, vt_sc, wq_sc, wot_sc,
            h_sc, q_sc, s_sc, acc_sc, mod_sc, modt_sc, w_sc, out_sc, x1_sc, xs_sc, st_sc,
            zv_sc, z_ref, ix_ref, o_sc, c_sc, wr_sc, mrow_sc, wg_sc, wu_sc, wd_sc, u_sc,
            sems, xsems, lsems, osems, fsems):
    D, S = x_sc.shape
    Hkv, Sk, Dh = k_hbm.shape
    G = 2 * Dh
    nblk = S // TQ
    ngrp = nblk // 2
    GW = 2 * TQ
    NF = wdt_hbm.shape[1] // FW
    qscale = (Dh ** -0.5) * math.log2(math.e)
    ftiles = [(n, f0, min(128, D - f0)) for n, f0 in enumerate(range(0, D, 128))]

    def ds(i, n):
        return slice(i * n, (i + 1) * n) if isinstance(i, int) else pl.ds(pl.multiple_of(i * n, n), n)

    def cp_k(g, slot, sem):
        return pltpu.make_async_copy(k_hbm.at[g], kvst.at[slot, 0:Sk, :], sem)

    def cp_v(g, slot, sem):
        return pltpu.make_async_copy(v_hbm.at[g], kvst.at[slot, Sk:2 * Sk, :], sem)

    def cp_wq(g, slot, sem):
        return pltpu.make_async_copy(wq_hbm.at[:, ds(g, G)], wst.at[slot, :, 0:G], sem)

    def cp_wo(g, slot, sem):
        return pltpu.make_async_copy(wot_hbm.at[:, ds(g, G)], wst.at[slot, :, G:2 * G], sem)

    def start_head(i, slot):
        cp_wq(i, slot, lsems.at[0]).start()
        cp_wo(i - 1, slot, lsems.at[0]).start()
        pltpu.make_async_copy(wdt_hbm.at[:, ds(jnp.minimum(i - 1, NF - 1), FW)],
                              wst.at[slot, :, 2 * G:2 * G + FW], lsems.at[0]).start()
        cp_k(i, slot, lsems.at[1]).start()
        cp_v(i, slot, lsems.at[1]).start()

    def wait_head(slot):
        pltpu.make_async_copy(wst.at[slot], wst.at[slot], lsems.at[0]).wait()
        pltpu.make_async_copy(kvst.at[slot], kvst.at[slot], lsems.at[1]).wait()

    def cp_x(j):
        return pltpu.make_async_copy(xt_hbm.at[:, ds(j, GW)], x_sc.at[:, ds(j, GW)], xsems.at[j])

    def cp_out(b):
        return pltpu.make_async_copy(out_sc.at[b + 1], out_hbm.at[:, ds(b, TQ)], osems.at[b])

    moe = [pltpu.make_async_copy(wg_hbm, wg_sc, sems.at[0]),
           pltpu.make_async_copy(wu_hbm, wu_sc, sems.at[1])]
    MA = 6 * 128
    cp_m0a = pltpu.make_async_copy(wmod_hbm.at[:, 0:MA], wmod_sc.at[:, 0:MA], sems.at[2])
    cp_m0b = pltpu.make_async_copy(wmod_hbm.at[:, MA:2 * D], wmod_sc.at[:, MA:2 * D], sems.at[11])
    cp_m1 = pltpu.make_async_copy(wmod_hbm.at[:, 2 * D:6 * D], wmod_sc.at[:, 2 * D:6 * D], sems.at[3])
    cp_c = pltpu.make_async_copy(c_hbm, c_sc, sems.at[4])
    cp_wr = pltpu.make_async_copy(wr_hbm, wr_sc, sems.at[5])
    cp_v0 = cp_v(0, 0, sems.at[6])
    KA = 3 * Sk // 8
    cp_k0a = pltpu.make_async_copy(k_hbm.at[0, 0:KA, :], kvst.at[0, 0:KA, :], sems.at[7])
    cp_k0b = pltpu.make_async_copy(k_hbm.at[0, KA:Sk, :], kvst.at[0, KA:Sk, :], sems.at[10])
    cp_wq0 = cp_wq(0, 0, sems.at[8])
    cp_wol = cp_wo(Hkv - 1, Hkv % 2, sems.at[9])

    def tie(v, dep):
        return pltpu.bitcast(pltpu.bitcast(v, U32) | (dep & zv_sc[...]), v.dtype)

    def ln1_pair(g, after=None):
        piv = jnp.broadcast_to(x_sc[0:16, ds(g, GW)].astype(F32)[0:1], (8, GW))
        if after is not None:
            piv = jnp.concatenate([tie(piv[:, :TQ], after), tie(piv[:, TQ:], after)], axis=1)
        s1 = s2 = None
        for r0 in range(0, D, 16):
            pw = piv
            if s2 is not None:
                b2 = pltpu.bitcast(s2, U32)
                pw = jnp.concatenate([tie(piv[:, :TQ], b2[:, :TQ]), tie(piv[:, TQ:], b2[:, TQ:])], axis=1)
            xd = x_sc[r0:r0 + 16, ds(g, GW)].astype(F32) - jnp.concatenate([pw, pw], axis=0)
            xq = xd * xd
            p1 = xd[0:8] + xd[8:16]
            p2 = xq[0:8] + xq[8:16]
            s1 = p1 if s1 is None else s1 + p1
            s2 = p2 if s2 is None else s2 + p2
        mu, inv = _ln_finish(piv, jnp.sum(s1, axis=0, keepdims=True) * (1.0 / D),
                             jnp.sum(s2, axis=0, keepdims=True) * (1.0 / D))
        g2 = g + z_ref[0]
        for _, f0, fw in ftiles:
            x = x_sc[f0:f0 + fw, ds(g2, GW)].astype(F32)
            n = (x - jnp.concatenate([mu] * (fw // 8), axis=0)) * inv
            h = n.T * mod_sc[1:2, f0:f0 + fw] + mod_sc[0:1, f0:f0 + fw]
            h_sc[ds(g, TQ), f0:f0 + fw] = _pk(h.astype(BF16))

    def mod_rest():
        dep = zv_sc[...]
        for c0 in range(2 * D, 6 * D, MT * 128):
            acc = None
            for r0 in range(0, D, 16):
                sc = modt_sc[r0:r0 + 16, :]
                sc = jnp.concatenate([tie(sc[0:8], dep), tie(sc[8:16], dep)], axis=0)
                pr = wmod_sc[r0:r0 + 16, c0:c0 + MT * 128].astype(F32) * jnp.concatenate([sc] * MT, axis=1)
                pr = pr[0:8] + pr[8:16]
                acc = pr if acc is None else acc + pr
                dep = pltpu.bitcast(acc[:, 0:128], U32)
            mrow_sc[:, c0:c0 + MT * 128] = acc

    def mod_finish():
        m = _rb(jnp.sum(mrow_sc[:, 2 * D:6 * D], axis=0, keepdims=True))
        ga = m[0:1, 0:D]
        sb = m[0:1, D:2 * D]
        cb1 = _rb(1.0 + m[0:1, 2 * D:3 * D])
        gb = m[0:1, 3 * D:4 * D]
        wr = wr_sc[...].astype(F32).reshape(1, D)
        mod_sc[2:3, :] = gb
        mod_sc[3:4, :] = sb
        mod_sc[4:5, :] = cb1
        mod_sc[5:6, :] = jnp.broadcast_to(jnp.sum(wr * cb1, axis=1, keepdims=True), (1, D))
        mod_sc[6:7, :] = jnp.broadcast_to(jnp.sum(wr * sb, axis=1, keepdims=True), (1, D))
        for i, vec in enumerate((ga, gb * cb1, gb * sb, wr * cb1)):
            modt_sc[i * D:(i + 1) * D, :] = jnp.broadcast_to(vec, (128, D)).T

    def qproj(c):
        h = _upk(h_sc[ds(c, TQ // 2), :])
        q = jnp.dot(h, _upk(wq_sc[...]), preferred_element_type=F32)
        q = (q * qscale).astype(BF16)
        return jnp.concatenate([q[:, :Dh], q[:, Dh:]], axis=0)

    def qk(c, q, split=False):
        if split:
            st = jnp.concatenate([
                lax.dot_general(_upk(k_sc[ds(j, Sk // 4), :]), q, NT, preferred_element_type=F32)
                for j in range(2)], axis=0)
        else:
            st = lax.dot_general(_upk(k_sc[...]), q, NT, preferred_element_type=F32)
        s_sc[c, 0:Sk, :] = st
        s_sc[c, Sk:Sk + 8, :] = jnp.broadcast_to(_red0(st, jnp.maximum, jnp.max, 1), (8, 2 * TQ))
        return pltpu.bitcast(st[0:8, 0:128], U32)

    def qk_rows(c, q, r0, r1):
        st = lax.dot_general(_upk(k_sc[r0 // 2:r1 // 2, :]), q, NT, preferred_element_type=F32)
        s_sc[c, r0:r1, :] = st
        m = jnp.broadcast_to(_red0(st, jnp.maximum, jnp.max, 1), (8, 2 * TQ))
        s_sc[c, Sk:Sk + 8, :] = m if r0 == 0 else jnp.maximum(m, s_sc[c, Sk:Sk + 8, :])

    def pv_cols(c, cols):
        p = jnp.exp2(s_sc[c, 0:Sk, cols] - s_sc[c, Sk:Sk + 1, cols])
        l = _red0(p, jnp.add, jnp.sum, 2)
        ot = jnp.dot(_upk(vt_sc[...]), p.astype(BF16), preferred_element_type=F32)
        return ot * (1.0 / l)

    def pv(c):
        ot = pv_cols(c, slice(0, 2 * TQ)).astype(BF16)
        return jnp.concatenate([ot[:, :TQ], ot[:, TQ:]], axis=0)

    def oproj(c, o2t, split=False, slot=None):
        if split:
            d = jnp.concatenate([
                jnp.dot(_upk(wot_sc[ds(j, D // 4), :]), o2t, preferred_element_type=F32)
                for j in range(2)], axis=0)
        else:
            d = jnp.dot(_upk(wot_sc[...]), o2t, preferred_element_type=F32)
        if slot is None:
            acc_sc[c] += d
        else:
            x1 = _rb(x_sc[:, ds(c, TQ)].astype(F32) + modt_sc[0:D, :] * (acc_sc[c] + d))
            xb = x1_sc.at[slot]
            xb[0:D, :] = x1
            mu, inv, rw, piv = _stats_t(x1, modt_sc[3 * D:4 * D, :])
            xb[D:D + 8, :] = jnp.broadcast_to(mu, (8, TQ))
            xb[D + 8:D + 16, :] = jnp.broadcast_to(inv, (8, TQ))
            st_sc[0, pl.ds(c, 1), :] = mu
            st_sc[1, pl.ds(c, 1), :] = inv
            st_sc[2, pl.ds(c, 1), :] = (rw - (mu - piv) * mod_sc[5:6, 0:TQ]) * inv + mod_sc[6:7, 0:TQ]

    def post(v0, slots, ch, cw, dist, slow):
        mu0 = [x1_sc[u, D:D + 8, :] for u in slots]
        inv0 = [x1_sc[u, D + 8:D + 16, :] for u in slots]
        for _, f0, fw in ftiles:
            words = []
            for r0 in range(f0, f0 + fw, 32):
                gc = modt_sc[D + r0:D + r0 + 32, :]
                gs = modt_sc[2 * D + r0:2 * D + r0 + 32, :]
                dep = ch[-dist] if len(ch) >= dist else None
                if r0 == f0 and len(cw) >= 3:
                    dep = dep | cw[-3]
                xs = []
                for u in range(len(slots)):
                    x1 = x1_sc[slots[u], r0:r0 + 32, :]
                    xs.append(x1)
                    mu = mu0[u] if dep is None else tie(mu0[u], dep)
                    mu = jnp.concatenate([mu] * 4, axis=0)
                    inv = jnp.concatenate([inv0[u]] * 4, axis=0)
                    o = x1 + ((x1 - mu) * inv * gc + gs)
                    out_sc[v0 + u, r0:r0 + 32, :] = o.astype(BF16)
                wd = pltpu.bitcast(xs[0], U32)
                if len(xs) > 1:
                    wd = wd | (pltpu.bitcast(xs[1], U32) >> 16)
                words.append(wd)
                dd = _pk(out_sc[z_ref[0], 0:16, :])
                ch.append(pltpu.roll(dd, 1, 1) if slow else dd)
            w_sc[ds(v0 // 2, TQ), f0:f0 + fw] = pltpu.bitcast(jnp.concatenate(words, axis=0), F32).T
            cw.append(pltpu.bitcast(w_sc[pl.ds(pl.multiple_of(z_ref[0], 8), 8), 0:128], U32))

    for cp in (cp_c, cp_x(0), cp_m0a):
        cp.start()

    def zero(i, carry):
        acc_sc[i] = jnp.zeros(acc_sc.shape[1:], F32)
        return carry
    lax.fori_loop(0, nblk, zero, 0)
    cp_m0b.start()

    def zero2(i, carry):
        x1_sc[i] = jnp.zeros(x1_sc.shape[1:], F32)
        u_sc[i] = jnp.zeros(u_sc.shape[1:], F32)
        return carry
    lax.fori_loop(0, LU + 1, zero2, 0)
    o_sc[...] = jnp.zeros(o_sc.shape, U32)
    st_sc[...] = jnp.zeros(st_sc.shape, F32)
    zv_sc[...] = jnp.zeros(zv_sc.shape, U32)
    z_ref[0] = 0
    cp_c.wait()
    cp_wq0.start()
    cp_x(0).wait()
    cp_k0a.start()
    c = c_sc[...].astype(F32)
    scb = (c * jax.nn.sigmoid(c)).astype(BF16)
    modt_sc[0:D, :] = jnp.broadcast_to(scb.astype(F32), (128, D)).T
    for cc in range(2):
        x = x_sc[:, ds(cc, TQ)].astype(F32)
        mu, inv = _stats_t(x)
        w_sc[ds(cc, TQ), :] = ((x - mu) * inv).T
    sc8 = jnp.broadcast_to(scb, (8, D))
    cp_m0a.wait()
    cp_x(1).start()
    mrow_sc[:, 0:MA] = jnp.dot(sc8, wmod_sc[:, 0:MA], preferred_element_type=F32)
    cp_m0b.wait()
    cp_k0b.start()
    mrow_sc[:, MA:2 * D] = jnp.dot(sc8, wmod_sc[:, MA:2 * D], preferred_element_type=F32)
    m = _rb(mrow_sc[:, 0:2 * D])
    sa = m[0:1, 0:D]
    ca1 = _rb(1.0 + m[0:1, D:2 * D])
    mod_sc[0:1, :] = sa
    mod_sc[1:2, :] = ca1
    h_sc[0:TQ, :] = _pk((w_sc[0:2 * TQ, :] * ca1 + sa).astype(BF16))
    cp_wq0.wait()
    cp_x(2).start()
    cp_x(3).start()
    wq_sc[...] = _pk(wst[0, :, 0:G])
    q_sc[0] = _pk(qproj(0))
    q_sc[1] = _pk(qproj(1))
    cp_k0a.wait()
    k_sc[0:KA // 2, :] = _pk(kvst[0, 0:KA, :])
    qk_rows(0, _upk(q_sc[0]), 0, KA)
    qk_rows(1, _upk(q_sc[1]), 0, KA)
    cp_x(1).wait()
    cp_k0b.wait()
    for jj in range(4, ngrp):
        cp_x(jj).start()
    k_sc[KA // 2:Sk // 2, :] = _pk(kvst[0, KA:Sk, :])
    qk_rows(0, _upk(q_sc[0]), KA, Sk)
    qk_rows(1, _upk(q_sc[1]), KA, Sk)
    ln1_pair(1)
    q_sc[0] = _pk(qproj(2 + z_ref[0]))
    q_sc[1] = _pk(qproj(3 + z_ref[0]))

    def group(g, q0, q1, split):
        after = qk(2 * g, q0, split)
        qk(2 * g + 1, q1, split)
        ln1_pair(g + 1, after if split else None)
        return qproj(2 * g + 2 + z_ref[0]), qproj(2 * g + 3 + z_ref[0])

    def first(j, carry):
        cp_x(2 * j + 2).wait()
        cp_x(2 * j + 3).wait()

        @pl.when(j == 0)
        def _():
            cp_m1.start()
            cp_v0.start()
            cp_wr.start()
            start_head(1, 1)
        q0, q1 = group(2 * j + 1, _upk(q_sc[0]), _upk(q_sc[1]), False)
        q0, q1 = group(2 * j + 2, q0, q1, True)
        q_sc[0] = _pk(q0)
        q_sc[1] = _pk(q1)
        return carry
    lax.fori_loop(0, ngrp // 2 - 1, first, 0)

    cp_wr.wait()
    cp_m1.wait()
    cp_v0.wait()
    for cp in moe:
        cp.start()
    vt_sc[...] = _pk(kvst[0, Sk:2 * Sk, :].T)
    mod_rest()
    qk(nblk - 2, _upk(q_sc[0]))
    qk(nblk - 1, _upk(q_sc[1]))

    def main(i, carry):
        slot = i & 1
        wait_head(slot)
        wq_sc[...] = _pk(wst[slot, :, 0:G])

        @pl.when(i + 1 < Hkv)
        def _():
            start_head(i + 1, 1 - slot)

        @pl.when(i + 1 == Hkv)
        def _():
            cp_wol.start()

        k_sc[...] = _pk(kvst[slot, 0:Sk, :])
        wot_sc[...] = _pk(wst[slot, :, G:2 * G])
        q = qproj(0)
        for c in range(nblk):
            end = c == nblk - 1
            o = pv(c)
            qn = None if end else qproj(c + 1)
            qk(c, q, split=end)
            oproj(c, o, split=end)
            q = qn
        vt_sc[...] = _pk(kvst[slot, Sk:2 * Sk, :].T)
        mod_finish()
        wd_sc[ds(jnp.minimum(i - 1, NF - 1), FW // 2), :] = _pk(wst[slot, :, 2 * G:2 * G + FW].T)
        return carry
    lax.fori_loop(1, Hkv, main, 0)

    cp_wol.wait()
    wot_sc[...] = _pk(wst[Hkv % 2, :, G:2 * G])

    def last(j, carry):
        ch, cw = [], []
        for u0 in range(0, LU, 2):
            post(LU * jnp.maximum(j - 1, 0) + u0, (u0, u0 + 1), ch, cw, 1, True)
        o = _upk(o_sc[...])
        for u in range(LU):
            c = LU * j + u - 1
            if u == 0:
                oproj(jnp.maximum(c, 0), o, slot=u)
                o0 = pv_cols(c + 1, slice(0, TQ))
            else:
                o0 = pv_cols(c + 1, slice(0, TQ))
                oproj(c, o, slot=u)
            o1 = pv_cols(c + 1, slice(TQ, 2 * TQ))
            o = jnp.concatenate([o0, o1], axis=0).astype(BF16)
        o_sc[...] = _pk(o)
        return carry
    lax.fori_loop(0, nblk // LU, last, 0)

    oproj(nblk - 1, _upk(o_sc[...]), split=True, slot=LU)

    r = _rb(st_sc[2]) + 0.0
    b16 = pltpu.bitcast(r, U32) >> 16
    ordk = jnp.where(b16 >= 0x8000, 0xFFFF - b16, b16 + 0x8000)
    tok = lax.broadcasted_iota(U32, r.shape, 0) * TQ + lax.broadcasted_iota(U32, r.shape, 1)
    key = pltpu.bitcast((ordk << 11) + (S - 1 - tok) + KEY_BIAS, F32)

    def rank(row, col):
        return _red0(jnp.where(col > row, 1.0, 0.0), jnp.add, jnp.sum, 16)

    lm = jnp.max(key, axis=0, keepdims=True)
    lrank = rank(lm, jnp.broadcast_to(lm, (TQ, TQ)).T)
    cand = jnp.concatenate([jnp.where(lrank == float(t), key, 0.0) for t in range(TOPC)], axis=0)
    cand = jnp.broadcast_to(jnp.max(cand, axis=1, keepdims=True), (TOPC * nblk, TQ))
    eye = lax.broadcasted_iota(I32, cand.shape, 0) == lax.broadcasted_iota(I32, cand.shape, 1)
    crow = _red0(jnp.where(eye, cand, 0.0), jnp.maximum, jnp.max, 16)
    crank = rank(crow, cand)
    subf = lax.broadcasted_iota(I32, (TOPC, TQ), 0).astype(F32)
    top = jnp.max(jnp.where(crank == subf, crow, 0.0), axis=1, keepdims=True)
    top = jnp.broadcast_to(top, (TOPC, TQ))
    mus = jnp.zeros((TOPC, TQ), F32)
    invs = jnp.zeros((TOPC, TQ), F32)
    for cc in range(nblk):
        sel = key[cc:cc + 1, :] == top
        mus = jnp.where(sel, st_sc[0, cc:cc + 1, :], mus)
        invs = jnp.where(sel, st_sc[1, cc:cc + 1, :], invs)
    ch, cw = [], []
    for u0 in range(0, LU, 2):
        post(nblk - LU + u0, (u0, u0 + 1), ch, cw, 2, False)
    post(nblk, (LU,), ch, cw, 2, False)
    topi = S - 1 - (pltpu.bitcast(top, I32) & (S - 1))
    rowi = ((((topi >> LG) + 1) >> 1) << LG) + (topi & (TQ - 1))
    for t in range(TOPC):
        xs_sc[t:t + 1, :] = w_sc[pl.ds(rowi[t, 0], 1), :]
    idxs = [topi[t, 0] for t in range(TOPC)]
    blks = [ix >> LG for ix in idxs]
    hmask = 0
    for t in range(TOPC):
        hmask = hmask | (1 << blks[t])
    clean = [((hmask >> b) & 1) == 0 for b in range(nblk)]
    for b in range(nblk):
        @pl.when(clean[b])
        def _():
            cp_out(b).start()
    ordt = (pltpu.bitcast(top, U32) - KEY_BIAS) >> 11
    rsel = pltpu.bitcast(jnp.where(ordt >= 0x8000, ordt - 0x8000, 0xFFFF - ordt) << 16, F32)[:, 0:1]
    mus = jnp.sum(mus, axis=1, keepdims=True)
    invs = jnp.sum(invs, axis=1, keepdims=True)
    words = pltpu.bitcast(xs_sc[...], U32)
    low = ((topi[:, 0:1] >> LG) & 1) == 0
    x1s = pltpu.bitcast(jnp.where(low, words << 16, words & jnp.uint32(0xFFFF0000)), F32)
    h2s = _rb(_rb(_rb(_rb(x1s - mus) * invs) * mod_sc[4:5, :]) + mod_sc[3:4, :])
    xsel = h2s.astype(BF16)

    for cp in moe:
        cp.wait()
    gt = _rb(jnp.dot(xsel, wg_sc[...], preferred_element_type=F32))
    ut = _rb(jnp.dot(xsel, wu_sc[...], preferred_element_type=F32))
    af = _rb(gt * jax.nn.sigmoid(gt)) * ut
    gate = _rb(jax.nn.sigmoid(rsel))
    lns = [ix & (TQ - 1) for ix in idxs]
    color, lead = [], []
    for t in range(TOPC):
        cl, dup = 0, False
        for s_ in range(t):
            cl = cl + (lns[s_] == lns[t]).astype(I32)
            dup = jnp.logical_or(dup, blks[s_] == blks[t])
        color.append(cl)
        lead.append(jnp.logical_not(dup))
    cmax = color[TOPC - 1]
    for t in range(1, TOPC - 1):
        cmax = jnp.maximum(cmax, color[t])

    def cp_fix(t, n, f0, fw):
        return pltpu.make_async_copy(out_sc.at[blks[t] + 1, f0:f0 + fw, :],
                                     out_hbm.at[f0:f0 + fw, ds(blks[t], TQ)], fsems.at[n])

    def merge(blk, ln, f0, fw, val):
        cur = out_sc[blk + 1, f0:f0 + fw, :].astype(F32)
        lane = lax.broadcasted_iota(I32, (fw, TQ), 1)
        out_sc[blk + 1, f0:f0 + fw, :] = jnp.where(lane == ln, val, cur).astype(BF16)

    def scatter(n, f0, fw, new):
        now = [(color[t] >> 1) == 0 for t in range(TOPC)]
        for t in range(TOPC):
            row = jnp.where(now[t], lns[t] + (color[t] & 1) * TQ, 2 * TQ)
            u_sc[n, pl.ds(row, 1), 0:fw] = new[t:t + 1, :]
        ut_ = u_sc[n, 0:2 * TQ, 0:fw].T
        for t in range(TOPC):
            val = ut_[:, :TQ] if t == 0 else jnp.where((color[t] & 1) == 0, ut_[:, :TQ], ut_[:, TQ:])
            merge(blks[t], jnp.where(now[t], lns[t], TQ), f0, fw, val)

    kb = (af.shape[1] // 128) * 8 // 9 * 128
    fence, news = [], []
    for n, f0, fw in ftiles:
        an = af
        if n >= 2:
            an = jnp.concatenate([af[:, :kb], tie(af[:, kb:kb + 128], fence[n - 2]), af[:, kb + 128:]],
                                 axis=1)
        y = _rb(jnp.dot(an.astype(BF16), _upk(wd_sc[:, f0:f0 + fw]), preferred_element_type=F32))
        y = _rb(y * gate)
        new = x1s[:, f0:f0 + fw] + mod_sc[2:3, f0:f0 + fw] * _rb(h2s[:, f0:f0 + fw] + y)
        news.append(new)
        scatter(n, f0, fw, new)
        fence.append(_pk(out_sc[z_ref[0], 0:16, :]))
        for t in range(TOPC):
            @pl.when(lead[t])
            def _():
                cp_fix(t, n, f0, fw).start()
    xs_sc[...] = jnp.concatenate(news, axis=1)

    for b in range(nblk):
        @pl.when(clean[b])
        def _():
            cp_out(b).wait()
    for n, f0, fw in ftiles:
        for t in range(TOPC):
            @pl.when(lead[t])
            def _():
                cp_fix(t, n, f0, fw).wait()

    @pl.when(cmax >= 2)
    def _():
        for t in range(TOPC):
            ix_ref[t] = idxs[t]

        def redo(t, carry):
            ln = ix_ref[t] & (TQ - 1)
            row = xs_sc[pl.ds(t, 1), :]
            for n, f0, fw in ftiles:
                u_sc[n, pl.ds(ln, 1), 0:fw] = row[:, f0:f0 + fw]
                merge(ix_ref[t] >> LG, ln, f0, fw, u_sc[n, 0:TQ, 0:fw].T)
            return carry
        lax.fori_loop(2, TOPC, redo, 0)
        for t in range(TOPC):
            @pl.when(lead[t])
            def _():
                cp_fix(t, 0, 0, D).start()
        for t in range(TOPC):
            @pl.when(lead[t])
            def _():
                cp_fix(t, 0, 0, D).wait()


@jax.jit
def pallas_adaLN_cond__gqa_block_cached__moe_arch_mod__prompt_kernel(
    A_x: jax.Array,
    A_k_cache: jax.Array,
    A_v_cache: jax.Array,
    A_wq: jax.Array,
    A_wo: jax.Array,
    B_x: jax.Array,
    B_w_r: jax.Array,
    B_w_gate: jax.Array,
    B_w_up: jax.Array,
    B_w_down: jax.Array,
    c: jax.Array,
    w_mod: jax.Array,
):
    del B_x
    B, S, D = A_x.shape
    _, Hkv, Sk, Dh = A_k_cache.shape
    G = A_wq.shape[1] // Hkv
    Fd = B_w_gate.shape[1]
    nblk = S // TQ
    assert B == 1 and G == 2 * Dh and TOPC * nblk == TQ and Fd % FW == 0 and Fd // FW < Hkv
    assert pl.cdiv(D, 128) == LU + 1 and (2 * D) % 128 == 0 and 6 * 128 < 2 * D and (4 * D) % (MT * 128) == 0
    hbm = pl.BlockSpec(memory_space=pl.ANY)
    out_t = pl.pallas_call(
        _kernel,
        in_specs=[hbm] * 11,
        out_specs=hbm,
        out_shape=jax.ShapeDtypeStruct((D, S), BF16),
        scratch_shapes=[
            pltpu.VMEM((D, S), BF16),
            pltpu.VMEM((D, 6 * D), BF16),
            pltpu.VMEM((2, 2 * Sk, Dh), BF16),
            pltpu.VMEM((2, D, 2 * G + FW), BF16),
            pltpu.VMEM((Sk // 2, Dh), U32),
            pltpu.VMEM((Dh // 2, Sk), U32),
            pltpu.VMEM((D // 2, G), U32),
            pltpu.VMEM((D // 2, G), U32),
            pltpu.VMEM((S // 2, D), U32),
            pltpu.VMEM((2, TQ, Dh), U32),
            pltpu.VMEM((nblk, Sk + 8, 2 * TQ), F32),
            pltpu.VMEM((nblk, D, TQ), F32),
            pltpu.VMEM((8, D), F32),
            pltpu.VMEM((4 * D, 128), F32),
            pltpu.VMEM((S // 2 + TQ, D), F32),
            pltpu.VMEM((nblk + 1, D, TQ), BF16),
            pltpu.VMEM((LU + 1, D + 16, TQ), F32),
            pltpu.VMEM((TOPC, D), F32),
            pltpu.VMEM((3, nblk, TQ), F32),
            pltpu.VMEM((8, 128), U32),
            pltpu.SMEM((1,), I32),
            pltpu.SMEM((TOPC,), I32),
            pltpu.VMEM((Dh, TQ), U32),
            pltpu.VMEM((1, D), BF16),
            pltpu.VMEM((D,), BF16),
            pltpu.VMEM((8, 6 * D), F32),
            pltpu.VMEM((D, Fd), BF16),
            pltpu.VMEM((D, Fd), BF16),
            pltpu.VMEM((Fd // 2, D), U32),
            pltpu.VMEM((pl.cdiv(D, 128), 2 * TQ + 8, 128), F32),
            pltpu.SemaphoreType.DMA((12,)),
            pltpu.SemaphoreType.DMA((nblk // 2,)),
            pltpu.SemaphoreType.DMA((2,)),
            pltpu.SemaphoreType.DMA((nblk,)),
            pltpu.SemaphoreType.DMA((pl.cdiv(D, 128),)),
        ],
        compiler_params=pltpu.CompilerParams(vmem_limit_bytes=110 * 1024 * 1024,
                                             disable_bounds_checks=True,
                                             disable_semaphore_checks=True),
    )(c, B_w_r, A_x.reshape(S, D).T, A_k_cache.reshape(Hkv, Sk, Dh), A_v_cache.reshape(Hkv, Sk, Dh),
      A_wq, A_wo.T, w_mod, B_w_gate, B_w_up, B_w_down.T)
    return out_t.T.reshape(B, S, D)
```

```python
import math

import jax
import jax.numpy as jnp
from jax import lax
import jax.experimental.pallas as pl
import jax.experimental.pallas.tpu as pltpu

F32 = jnp.float32
BF16 = jnp.bfloat16
U32 = jnp.uint32
I32 = jnp.int32
EPS = 1e-05
TOPC = 8
NT = (((1,), (1,)), ((), ()))
TQ = 128
LG = 7
LU = 4
FW = 3 * 128
MT = 3
KEY_BIAS = 0x20000000


def _pk(x):
    return pltpu.bitcast(x, U32)


def _upk(x):
    return pltpu.bitcast(x, BF16)


def _rb(x):
    return x.astype(BF16).astype(F32)


def _tree(xs, op):
    while len(xs) > 1:
        xs = [op(xs[i], xs[i + 1]) if i + 1 < len(xs) else xs[i] for i in range(0, len(xs), 2)]
    return xs[0]


def _red0(x, op, red, grp):
    n = x.shape[0]
    acc = None
    for t in range(0, n, 8 * grp):
        part = _tree([x[j:j + 8, :] for j in range(t, min(t + 8 * grp, n), 8)], op)
        acc = part if acc is None else op(acc, part)
    return red(acc, axis=0, keepdims=True)


def _ln_finish(piv, s1, s2):
    var = jnp.maximum(s2 - s1 * s1, 0.0)
    return _rb(piv + s1), 1.0 / _rb(jnp.sqrt(_rb(_rb(var) + EPS)))


def _stats_t(x, w=None):
    d = x.shape[0]
    piv = x[0:1, :]
    xd = x - piv
    s1 = _red0(xd, jnp.add, jnp.sum, 8) * (1.0 / d)
    s2 = _red0(xd * xd, jnp.add, jnp.sum, 8) * (1.0 / d)
    mu, inv = _ln_finish(piv, s1, s2)
    if w is None:
        return mu, inv
    return mu, inv, _red0(xd * w, jnp.add, jnp.sum, 8), piv


def _kernel(c_hbm, wr_hbm, xt_hbm, k_hbm, v_hbm, wq_hbm, wot_hbm, wmod_hbm,
            wg_hbm, wu_hbm, wdt_hbm, out_hbm,
            x_sc, wmod_sc, kvst, wst, k_sc, vt_sc, wq_sc, wot_sc,
            h_sc, q_sc, s_sc, acc_sc, mod_sc, modt_sc, w_sc, out_sc, x1_sc, xs_sc, st_sc,
            zv_sc, z_ref, ix_ref, o_sc, c_sc, wr_sc, mrow_sc, wg_sc, wu_sc, wd_sc, u_sc,
            sems, xsems, lsems, osems, fsems):
    D, S = x_sc.shape
    Hkv, Sk, Dh = k_hbm.shape
    G = 2 * Dh
    nblk = S // TQ
    ngrp = nblk // 2
    GW = 2 * TQ
    NF = wdt_hbm.shape[1] // FW
    qscale = (Dh ** -0.5) * math.log2(math.e)
    ftiles = [(n, f0, min(128, D - f0)) for n, f0 in enumerate(range(0, D, 128))]

    def ds(i, n):
        return slice(i * n, (i + 1) * n) if isinstance(i, int) else pl.ds(pl.multiple_of(i * n, n), n)

    def cp_k(g, slot, sem):
        return pltpu.make_async_copy(k_hbm.at[g], kvst.at[slot, 0:Sk, :], sem)

    def cp_v(g, slot, sem):
        return pltpu.make_async_copy(v_hbm.at[g], kvst.at[slot, Sk:2 * Sk, :], sem)

    def cp_wq(g, slot, sem):
        return pltpu.make_async_copy(wq_hbm.at[:, ds(g, G)], wst.at[slot, :, 0:G], sem)

    def cp_wo(g, slot, sem):
        return pltpu.make_async_copy(wot_hbm.at[:, ds(g, G)], wst.at[slot, :, G:2 * G], sem)

    def start_head(i, slot):
        cp_wq(i, slot, lsems.at[0]).start()
        cp_wo(i - 1, slot, lsems.at[0]).start()
        pltpu.make_async_copy(wdt_hbm.at[:, ds(jnp.minimum(i - 1, NF - 1), FW)],
                              wst.at[slot, :, 2 * G:2 * G + FW], lsems.at[0]).start()
        cp_k(i, slot, lsems.at[1]).start()
        cp_v(i, slot, lsems.at[1]).start()

    def wait_head(slot):
        pltpu.make_async_copy(wst.at[slot], wst.at[slot], lsems.at[0]).wait()
        pltpu.make_async_copy(kvst.at[slot], kvst.at[slot], lsems.at[1]).wait()

    def cp_x(j):
        return pltpu.make_async_copy(xt_hbm.at[:, ds(j, GW)], x_sc.at[:, ds(j, GW)], xsems.at[j])

    def cp_out(b):
        return pltpu.make_async_copy(out_sc.at[b + 1], out_hbm.at[:, ds(b, TQ)], osems.at[b])

    moe = [pltpu.make_async_copy(wg_hbm, wg_sc, sems.at[0]),
           pltpu.make_async_copy(wu_hbm, wu_sc, sems.at[1])]
    MA = 6 * 128
    cp_m0a = pltpu.make_async_copy(wmod_hbm.at[:, 0:MA], wmod_sc.at[:, 0:MA], sems.at[2])
    cp_m0b = pltpu.make_async_copy(wmod_hbm.at[:, MA:2 * D], wmod_sc.at[:, MA:2 * D], sems.at[11])
    cp_m1 = pltpu.make_async_copy(wmod_hbm.at[:, 2 * D:6 * D], wmod_sc.at[:, 2 * D:6 * D], sems.at[3])
    cp_c = pltpu.make_async_copy(c_hbm, c_sc, sems.at[4])
    cp_wr = pltpu.make_async_copy(wr_hbm, wr_sc, sems.at[5])
    cp_v0 = cp_v(0, 0, sems.at[6])
    KA = 3 * Sk // 8
    cp_k0a = pltpu.make_async_copy(k_hbm.at[0, 0:KA, :], kvst.at[0, 0:KA, :], sems.at[7])
    cp_k0b = pltpu.make_async_copy(k_hbm.at[0, KA:Sk, :], kvst.at[0, KA:Sk, :], sems.at[10])
    cp_wq0 = cp_wq(0, 0, sems.at[8])
    cp_wol = cp_wo(Hkv - 1, Hkv % 2, sems.at[9])

    def tie(v, dep):
        return pltpu.bitcast(pltpu.bitcast(v, U32) | (dep & zv_sc[...]), v.dtype)

    def ln1_pair(g, after=None):
        piv = jnp.broadcast_to(x_sc[0:16, ds(g, GW)].astype(F32)[0:1], (8, GW))
        if after is not None:
            piv = jnp.concatenate([tie(piv[:, :TQ], after), tie(piv[:, TQ:], after)], axis=1)
        s1 = s2 = None
        for r0 in range(0, D, 16):
            pw = piv
            if s2 is not None:
                b2 = pltpu.bitcast(s2, U32)
                pw = jnp.concatenate([tie(piv[:, :TQ], b2[:, :TQ]), tie(piv[:, TQ:], b2[:, TQ:])], axis=1)
            xd = x_sc[r0:r0 + 16, ds(g, GW)].astype(F32) - jnp.concatenate([pw, pw], axis=0)
            xq = xd * xd
            p1 = xd[0:8] + xd[8:16]
            p2 = xq[0:8] + xq[8:16]
            s1 = p1 if s1 is None else s1 + p1
            s2 = p2 if s2 is None else s2 + p2
        mu, inv = _ln_finish(piv, jnp.sum(s1, axis=0, keepdims=True) * (1.0 / D),
                             jnp.sum(s2, axis=0, keepdims=True) * (1.0 / D))
        g2 = g + z_ref[0]
        for _, f0, fw in ftiles:
            x = x_sc[f0:f0 + fw, ds(g2, GW)].astype(F32)
            n = (x - jnp.concatenate([mu] * (fw // 8), axis=0)) * inv
            h = n.T * mod_sc[1:2, f0:f0 + fw] + mod_sc[0:1, f0:f0 + fw]
            h_sc[ds(g, TQ), f0:f0 + fw] = _pk(h.astype(BF16))

    def mod_rest():
        dep = zv_sc[...]
        for c0 in range(2 * D, 6 * D, MT * 128):
            acc = None
            for r0 in range(0, D, 16):
                sc = modt_sc[r0:r0 + 16, :]
                sc = jnp.concatenate([tie(sc[0:8], dep), tie(sc[8:16], dep)], axis=0)
                pr = wmod_sc[r0:r0 + 16, c0:c0 + MT * 128].astype(F32) * jnp.concatenate([sc] * MT, axis=1)
                pr = pr[0:8] + pr[8:16]
                acc = pr if acc is None else acc + pr
                dep = pltpu.bitcast(acc[:, 0:128], U32)
            mrow_sc[:, c0:c0 + MT * 128] = acc

    def mod_finish():
        m = _rb(jnp.sum(mrow_sc[:, 2 * D:6 * D], axis=0, keepdims=True))
        ga = m[0:1, 0:D]
        sb = m[0:1, D:2 * D]
        cb1 = _rb(1.0 + m[0:1, 2 * D:3 * D])
        gb = m[0:1, 3 * D:4 * D]
        wr = wr_sc[...].astype(F32).reshape(1, D)
        mod_sc[2:3, :] = gb
        mod_sc[3:4, :] = sb
        mod_sc[4:5, :] = cb1
        mod_sc[5:6, :] = jnp.broadcast_to(jnp.sum(wr * cb1, axis=1, keepdims=True), (1, D))
        mod_sc[6:7, :] = jnp.broadcast_to(jnp.sum(wr * sb, axis=1, keepdims=True), (1, D))
        for i, vec in enumerate((ga, gb * cb1, gb * sb, wr * cb1)):
            modt_sc[i * D:(i + 1) * D, :] = jnp.broadcast_to(vec, (128, D)).T

    def qproj(c):
        h = _upk(h_sc[ds(c, TQ // 2), :])
        q = jnp.dot(h, _upk(wq_sc[...]), preferred_element_type=F32)
        q = (q * qscale).astype(BF16)
        return jnp.concatenate([q[:, :Dh], q[:, Dh:]], axis=0)

    def qk(c, q, split=False):
        if split:
            st = jnp.concatenate([
                lax.dot_general(_upk(k_sc[ds(j, Sk // 4), :]), q, NT, preferred_element_type=F32)
                for j in range(2)], axis=0)
        else:
            st = lax.dot_general(_upk(k_sc[...]), q, NT, preferred_element_type=F32)
        s_sc[c, 0:Sk, :] = st
        s_sc[c, Sk:Sk + 8, :] = jnp.broadcast_to(_red0(st, jnp.maximum, jnp.max, 1), (8, 2 * TQ))
        return pltpu.bitcast(st[0:8, 0:128], U32)

    def qk_rows(c, q, r0, r1):
        st = lax.dot_general(_upk(k_sc[r0 // 2:r1 // 2, :]), q, NT, preferred_element_type=F32)
        s_sc[c, r0:r1, :] = st
        m = jnp.broadcast_to(_red0(st, jnp.maximum, jnp.max, 1), (8, 2 * TQ))
        s_sc[c, Sk:Sk + 8, :] = m if r0 == 0 else jnp.maximum(m, s_sc[c, Sk:Sk + 8, :])

    def pv_cols(c, cols):
        p = jnp.exp2(s_sc[c, 0:Sk, cols] - s_sc[c, Sk:Sk + 1, cols])
        l = _red0(p, jnp.add, jnp.sum, 2)
        ot = jnp.dot(_upk(vt_sc[...]), p.astype(BF16), preferred_element_type=F32)
        return ot * (1.0 / l)

    def pv(c):
        ot = pv_cols(c, slice(0, 2 * TQ)).astype(BF16)
        return jnp.concatenate([ot[:, :TQ], ot[:, TQ:]], axis=0)

    def oproj(c, o2t, split=False, slot=None):
        if split:
            d = jnp.concatenate([
                jnp.dot(_upk(wot_sc[ds(j, D // 4), :]), o2t, preferred_element_type=F32)
                for j in range(2)], axis=0)
        else:
            d = jnp.dot(_upk(wot_sc[...]), o2t, preferred_element_type=F32)
        if slot is None:
            acc_sc[c] += d
        else:
            x1 = _rb(x_sc[:, ds(c, TQ)].astype(F32) + modt_sc[0:D, :] * (acc_sc[c] + d))
            xb = x1_sc.at[slot]
            xb[0:D, :] = x1
            mu, inv, rw, piv = _stats_t(x1, modt_sc[3 * D:4 * D, :])
            xb[D:D + 8, :] = jnp.broadcast_to(mu, (8, TQ))
            xb[D + 8:D + 16, :] = jnp.broadcast_to(inv, (8, TQ))
            st_sc[0, pl.ds(c, 1), :] = mu
            st_sc[1, pl.ds(c, 1), :] = inv
            st_sc[2, pl.ds(c, 1), :] = (rw - (mu - piv) * mod_sc[5:6, 0:TQ]) * inv + mod_sc[6:7, 0:TQ]

    def post(v0, slots, ch, cw, dist, slow):
        mu0 = [x1_sc[u, D:D + 8, :] for u in slots]
        inv0 = [x1_sc[u, D + 8:D + 16, :] for u in slots]
        for _, f0, fw in ftiles:
            words = []
            for r0 in range(f0, f0 + fw, 32):
                gc = modt_sc[D + r0:D + r0 + 32, :]
                gs = modt_sc[2 * D + r0:2 * D + r0 + 32, :]
                dep = ch[-dist] if len(ch) >= dist else None
                if r0 == f0 and len(cw) >= 3:
                    dep = dep | cw[-3]
                xs = []
                for u in range(len(slots)):
                    x1 = x1_sc[slots[u], r0:r0 + 32, :]
                    xs.append(x1)
                    mu = mu0[u] if dep is None else tie(mu0[u], dep)
                    mu = jnp.concatenate([mu] * 4, axis=0)
                    inv = jnp.concatenate([inv0[u]] * 4, axis=0)
                    o = x1 + ((x1 - mu) * inv * gc + gs)
                    out_sc[v0 + u, r0:r0 + 32, :] = o.astype(BF16)
                wd = pltpu.bitcast(xs[0], U32)
                if len(xs) > 1:
                    wd = wd | (pltpu.bitcast(xs[1], U32) >> 16)
                words.append(wd)
                dd = _pk(out_sc[z_ref[0], 0:16, :])
                ch.append(pltpu.roll(dd, 1, 1) if slow else dd)
            w_sc[ds(v0 // 2, TQ), f0:f0 + fw] = pltpu.bitcast(jnp.concatenate(words, axis=0), F32).T
            cw.append(pltpu.bitcast(w_sc[pl.ds(pl.multiple_of(z_ref[0], 8), 8), 0:128], U32))

    @pl.when(pl.program_id(0) == 0)
    def _():
        for cp in (cp_c, cp_x(0), cp_m0a):
            cp.start()

        def zero(i, carry):
            acc_sc[i] = jnp.zeros(acc_sc.shape[1:], F32)
            return carry
        lax.fori_loop(0, nblk, zero, 0)
        cp_m0b.start()

        def zero2(i, carry):
            x1_sc[i] = jnp.zeros(x1_sc.shape[1:], F32)
            u_sc[i] = jnp.zeros(u_sc.shape[1:], F32)
            return carry
        lax.fori_loop(0, LU + 1, zero2, 0)
        o_sc[...] = jnp.zeros(o_sc.shape, U32)
        st_sc[...] = jnp.zeros(st_sc.shape, F32)
        zv_sc[...] = jnp.zeros(zv_sc.shape, U32)
        z_ref[0] = 0
        cp_c.wait()
        cp_wq0.start()
        cp_x(0).wait()
        cp_k0a.start()
        c = c_sc[...].astype(F32)
        scb = (c * jax.nn.sigmoid(c)).astype(BF16)
        modt_sc[0:D, :] = jnp.broadcast_to(scb.astype(F32), (128, D)).T
        for cc in range(2):
            x = x_sc[:, ds(cc, TQ)].astype(F32)
            mu, inv = _stats_t(x)
            w_sc[ds(cc, TQ), :] = ((x - mu) * inv).T
        sc8 = jnp.broadcast_to(scb, (8, D))
        cp_m0a.wait()
        cp_x(1).start()
        mrow_sc[:, 0:MA] = jnp.dot(sc8, wmod_sc[:, 0:MA], preferred_element_type=F32)
        cp_m0b.wait()
        cp_k0b.start()
        mrow_sc[:, MA:2 * D] = jnp.dot(sc8, wmod_sc[:, MA:2 * D], preferred_element_type=F32)
        m = _rb(mrow_sc[:, 0:2 * D])
        sa = m[0:1, 0:D]
        ca1 = _rb(1.0 + m[0:1, D:2 * D])
        mod_sc[0:1, :] = sa
        mod_sc[1:2, :] = ca1
        h_sc[0:TQ, :] = _pk((w_sc[0:2 * TQ, :] * ca1 + sa).astype(BF16))
        cp_wq0.wait()
        cp_x(2).start()
        cp_x(3).start()
        wq_sc[...] = _pk(wst[0, :, 0:G])
        q_sc[0] = _pk(qproj(0))
        q_sc[1] = _pk(qproj(1))
        cp_k0a.wait()
        k_sc[0:KA // 2, :] = _pk(kvst[0, 0:KA, :])
        qk_rows(0, _upk(q_sc[0]), 0, KA)
        qk_rows(1, _upk(q_sc[1]), 0, KA)
        cp_x(1).wait()
        cp_k0b.wait()
        for jj in range(4, ngrp):
            cp_x(jj).start()
        k_sc[KA // 2:Sk // 2, :] = _pk(kvst[0, KA:Sk, :])
        qk_rows(0, _upk(q_sc[0]), KA, Sk)
        qk_rows(1, _upk(q_sc[1]), KA, Sk)
        ln1_pair(1)
        q_sc[0] = _pk(qproj(2 + z_ref[0]))
        q_sc[1] = _pk(qproj(3 + z_ref[0]))

        def group(g, q0, q1, split):
            after = qk(2 * g, q0, split)
            qk(2 * g + 1, q1, split)
            ln1_pair(g + 1, after if split else None)
            return qproj(2 * g + 2 + z_ref[0]), qproj(2 * g + 3 + z_ref[0])

        def first(j, carry):
            cp_x(2 * j + 2).wait()
            cp_x(2 * j + 3).wait()

            @pl.when(j == 0)
            def _():
                cp_m1.start()
                cp_v0.start()
                cp_wr.start()
                start_head(1, 1)
            q0, q1 = group(2 * j + 1, _upk(q_sc[0]), _upk(q_sc[1]), False)
            q0, q1 = group(2 * j + 2, q0, q1, True)
            q_sc[0] = _pk(q0)
            q_sc[1] = _pk(q1)
            return carry
        lax.fori_loop(0, ngrp // 2 - 1, first, 0)

        cp_wr.wait()
        cp_m1.wait()
        cp_v0.wait()
        for cp in moe:
            cp.start()
        vt_sc[...] = _pk(kvst[0, Sk:2 * Sk, :].T)
        mod_rest()
        qk(nblk - 2, _upk(q_sc[0]))
        qk(nblk - 1, _upk(q_sc[1]))

        def main(i, carry):
            slot = i & 1
            wait_head(slot)
            wq_sc[...] = _pk(wst[slot, :, 0:G])

            @pl.when(i + 1 < Hkv)
            def _():
                start_head(i + 1, 1 - slot)

            @pl.when(i + 1 == Hkv)
            def _():
                cp_wol.start()

            k_sc[...] = _pk(kvst[slot, 0:Sk, :])
            wot_sc[...] = _pk(wst[slot, :, G:2 * G])
            q = qproj(0)
            for c in range(nblk):
                end = c == nblk - 1
                o = pv(c)
                qn = None if end else qproj(c + 1)
                qk(c, q, split=end)
                oproj(c, o, split=end)
                q = qn
            vt_sc[...] = _pk(kvst[slot, Sk:2 * Sk, :].T)
            mod_finish()
            wd_sc[ds(jnp.minimum(i - 1, NF - 1), FW // 2), :] = _pk(wst[slot, :, 2 * G:2 * G + FW].T)
            return carry
        lax.fori_loop(1, Hkv, main, 0)

    @pl.when(pl.program_id(0) == 1)
    def _():
        cp_wol.wait()
        wot_sc[...] = _pk(wst[Hkv % 2, :, G:2 * G])

        def last(j, carry):
            ch, cw = [], []
            for u0 in range(0, LU, 2):
                post(LU * jnp.maximum(j - 1, 0) + u0, (u0, u0 + 1), ch, cw, 1, True)
            o = _upk(o_sc[...])
            for u in range(LU):
                c = LU * j + u - 1
                if u == 0:
                    oproj(jnp.maximum(c, 0), o, slot=u)
                    o0 = pv_cols(c + 1, slice(0, TQ))
                else:
                    o0 = pv_cols(c + 1, slice(0, TQ))
                    oproj(c, o, slot=u)
                o1 = pv_cols(c + 1, slice(TQ, 2 * TQ))
                o = jnp.concatenate([o0, o1], axis=0).astype(BF16)
            o_sc[...] = _pk(o)
            return carry
        lax.fori_loop(0, nblk // LU, last, 0)

        oproj(nblk - 1, _upk(o_sc[...]), split=True, slot=LU)

        r = _rb(st_sc[2]) + 0.0
        b16 = pltpu.bitcast(r, U32) >> 16
        ordk = jnp.where(b16 >= 0x8000, 0xFFFF - b16, b16 + 0x8000)
        tok = lax.broadcasted_iota(U32, r.shape, 0) * TQ + lax.broadcasted_iota(U32, r.shape, 1)
        key = pltpu.bitcast((ordk << 11) + (S - 1 - tok) + KEY_BIAS, F32)

        def rank(row, col):
            return _red0(jnp.where(col > row, 1.0, 0.0), jnp.add, jnp.sum, 16)

        lm = jnp.max(key, axis=0, keepdims=True)
        lrank = rank(lm, jnp.broadcast_to(lm, (TQ, TQ)).T)
        cand = jnp.concatenate([jnp.where(lrank == float(t), key, 0.0) for t in range(TOPC)], axis=0)
        cand = jnp.broadcast_to(jnp.max(cand, axis=1, keepdims=True), (TOPC * nblk, TQ))
        eye = lax.broadcasted_iota(I32, cand.shape, 0) == lax.broadcasted_iota(I32, cand.shape, 1)
        crow = _red0(jnp.where(eye, cand, 0.0), jnp.maximum, jnp.max, 16)
        crank = rank(crow, cand)
        subf = lax.broadcasted_iota(I32, (TOPC, TQ), 0).astype(F32)
        top = jnp.max(jnp.where(crank == subf, crow, 0.0), axis=1, keepdims=True)
        top = jnp.broadcast_to(top, (TOPC, TQ))
        mus = jnp.zeros((TOPC, TQ), F32)
        invs = jnp.zeros((TOPC, TQ), F32)
        for cc in range(nblk):
            sel = key[cc:cc + 1, :] == top
            mus = jnp.where(sel, st_sc[0, cc:cc + 1, :], mus)
            invs = jnp.where(sel, st_sc[1, cc:cc + 1, :], invs)
        ch, cw = [], []
        for u0 in range(0, LU, 2):
            post(nblk - LU + u0, (u0, u0 + 1), ch, cw, 2, False)
        post(nblk, (LU,), ch, cw, 2, False)
        topi = S - 1 - (pltpu.bitcast(top, I32) & (S - 1))
        rowi = ((((topi >> LG) + 1) >> 1) << LG) + (topi & (TQ - 1))
        for t in range(TOPC):
            xs_sc[t:t + 1, :] = w_sc[pl.ds(jnp.clip(rowi[t, 0], 0, w_sc.shape[0] - 1), 1), :]
        idxs = [jnp.clip(topi[t, 0], 0, S - 1) for t in range(TOPC)]
        blks = [ix >> LG for ix in idxs]
        hmask = 0
        for t in range(TOPC):
            hmask = hmask | (1 << blks[t])
        clean = [((hmask >> b) & 1) == 0 for b in range(nblk)]
        for b in range(nblk):
            @pl.when(clean[b])
            def _():
                cp_out(b).start()
        ordt = (pltpu.bitcast(top, U32) - KEY_BIAS) >> 11
        rsel = pltpu.bitcast(jnp.where(ordt >= 0x8000, ordt - 0x8000, 0xFFFF - ordt) << 16, F32)[:, 0:1]
        mus = jnp.sum(mus, axis=1, keepdims=True)
        invs = jnp.sum(invs, axis=1, keepdims=True)
        words = pltpu.bitcast(xs_sc[...], U32)
        low = ((topi[:, 0:1] >> LG) & 1) == 0
        x1s = pltpu.bitcast(jnp.where(low, words << 16, words & jnp.uint32(0xFFFF0000)), F32)
        h2s = _rb(_rb(_rb(_rb(x1s - mus) * invs) * mod_sc[4:5, :]) + mod_sc[3:4, :])
        xsel = h2s.astype(BF16)

        for cp in moe:
            cp.wait()
        gt = _rb(jnp.dot(xsel, wg_sc[...], preferred_element_type=F32))
        ut = _rb(jnp.dot(xsel, wu_sc[...], preferred_element_type=F32))
        af = _rb(gt * jax.nn.sigmoid(gt)) * ut
        gate = _rb(jax.nn.sigmoid(rsel))
        lns = [ix & (TQ - 1) for ix in idxs]
        color, lead = [], []
        for t in range(TOPC):
            cl, dup = 0, False
            for s_ in range(t):
                cl = cl + (lns[s_] == lns[t]).astype(I32)
                dup = jnp.logical_or(dup, blks[s_] == blks[t])
            color.append(cl)
            lead.append(jnp.logical_not(dup))
        cmax = color[TOPC - 1]
        for t in range(1, TOPC - 1):
            cmax = jnp.maximum(cmax, color[t])

        def cp_fix(t, n, f0, fw):
            return pltpu.make_async_copy(out_sc.at[blks[t] + 1, f0:f0 + fw, :],
                                         out_hbm.at[f0:f0 + fw, ds(blks[t], TQ)], fsems.at[n])

        def merge(blk, ln, f0, fw, val):
            cur = out_sc[blk + 1, f0:f0 + fw, :].astype(F32)
            lane = lax.broadcasted_iota(I32, (fw, TQ), 1)
            out_sc[blk + 1, f0:f0 + fw, :] = jnp.where(lane == ln, val, cur).astype(BF16)

        def scatter(n, f0, fw, new):
            now = [(color[t] >> 1) == 0 for t in range(TOPC)]
            for t in range(TOPC):
                row = jnp.where(now[t], lns[t] + (color[t] & 1) * TQ, 2 * TQ)
                u_sc[n, pl.ds(row, 1), 0:fw] = new[t:t + 1, :]
            ut_ = u_sc[n, 0:2 * TQ, 0:fw].T
            for t in range(TOPC):
                val = ut_[:, :TQ] if t == 0 else jnp.where((color[t] & 1) == 0, ut_[:, :TQ], ut_[:, TQ:])
                merge(blks[t], jnp.where(now[t], lns[t], TQ), f0, fw, val)

        kb = (af.shape[1] // 128) * 8 // 9 * 128
        fence, news = [], []
        for n, f0, fw in ftiles:
            an = af
            if n >= 2:
                an = jnp.concatenate([af[:, :kb], tie(af[:, kb:kb + 128], fence[n - 2]), af[:, kb + 128:]],
                                     axis=1)
            y = _rb(jnp.dot(an.astype(BF16), _upk(wd_sc[:, f0:f0 + fw]), preferred_element_type=F32))
            y = _rb(y * gate)
            new = x1s[:, f0:f0 + fw] + mod_sc[2:3, f0:f0 + fw] * _rb(h2s[:, f0:f0 + fw] + y)
            news.append(new)
            scatter(n, f0, fw, new)
            fence.append(_pk(out_sc[z_ref[0], 0:16, :]))
            for t in range(TOPC):
                @pl.when(lead[t])
                def _():
                    cp_fix(t, n, f0, fw).start()
        xs_sc[...] = jnp.concatenate(news, axis=1)

        for b in range(nblk):
            @pl.when(clean[b])
            def _():
                cp_out(b).wait()
        for n, f0, fw in ftiles:
            for t in range(TOPC):
                @pl.when(lead[t])
                def _():
                    cp_fix(t, n, f0, fw).wait()

        @pl.when(cmax >= 2)
        def _():
            for t in range(TOPC):
                ix_ref[t] = idxs[t]

            def redo(t, carry):
                ln = ix_ref[t] & (TQ - 1)
                row = xs_sc[pl.ds(t, 1), :]
                for n, f0, fw in ftiles:
                    u_sc[n, pl.ds(ln, 1), 0:fw] = row[:, f0:f0 + fw]
                    merge(ix_ref[t] >> LG, ln, f0, fw, u_sc[n, 0:TQ, 0:fw].T)
                return carry
            lax.fori_loop(2, TOPC, redo, 0)
            for t in range(TOPC):
                @pl.when(lead[t])
                def _():
                    cp_fix(t, 0, 0, D).start()
            for t in range(TOPC):
                @pl.when(lead[t])
                def _():
                    cp_fix(t, 0, 0, D).wait()


@jax.jit
def pallas_adaLN_cond__gqa_block_cached__moe_arch_mod__prompt_kernel(
    A_x: jax.Array,
    A_k_cache: jax.Array,
    A_v_cache: jax.Array,
    A_wq: jax.Array,
    A_wo: jax.Array,
    B_x: jax.Array,
    B_w_r: jax.Array,
    B_w_gate: jax.Array,
    B_w_up: jax.Array,
    B_w_down: jax.Array,
    c: jax.Array,
    w_mod: jax.Array,
):
    del B_x
    B, S, D = A_x.shape
    _, Hkv, Sk, Dh = A_k_cache.shape
    G = A_wq.shape[1] // Hkv
    Fd = B_w_gate.shape[1]
    nblk = S // TQ
    assert B == 1 and G == 2 * Dh and TOPC * nblk == TQ and Fd % FW == 0 and Fd // FW < Hkv
    assert pl.cdiv(D, 128) == LU + 1 and (2 * D) % 128 == 0 and 6 * 128 < 2 * D and (4 * D) % (MT * 128) == 0
    hbm = pl.BlockSpec(memory_space=pl.ANY)
    out_t = pl.pallas_call(
        _kernel,
        grid=(2,),
        in_specs=[hbm] * 11,
        out_specs=hbm,
        out_shape=jax.ShapeDtypeStruct((D, S), BF16),
        scratch_shapes=[
            pltpu.VMEM((D, S), BF16),
            pltpu.VMEM((D, 6 * D), BF16),
            pltpu.VMEM((2, 2 * Sk, Dh), BF16),
            pltpu.VMEM((2, D, 2 * G + FW), BF16),
            pltpu.VMEM((Sk // 2, Dh), U32),
            pltpu.VMEM((Dh // 2, Sk), U32),
            pltpu.VMEM((D // 2, G), U32),
            pltpu.VMEM((D // 2, G), U32),
            pltpu.VMEM((S // 2, D), U32),
            pltpu.VMEM((2, TQ, Dh), U32),
            pltpu.VMEM((nblk, Sk + 8, 2 * TQ), F32),
            pltpu.VMEM((nblk, D, TQ), F32),
            pltpu.VMEM((8, D), F32),
            pltpu.VMEM((4 * D, 128), F32),
            pltpu.VMEM((S // 2 + TQ, D), F32),
            pltpu.VMEM((nblk + 1, D, TQ), BF16),
            pltpu.VMEM((LU + 1, D + 16, TQ), F32),
            pltpu.VMEM((TOPC, D), F32),
            pltpu.VMEM((3, nblk, TQ), F32),
            pltpu.VMEM((8, 128), U32),
            pltpu.SMEM((1,), I32),
            pltpu.SMEM((TOPC,), I32),
            pltpu.VMEM((Dh, TQ), U32),
            pltpu.VMEM((1, D), BF16),
            pltpu.VMEM((D,), BF16),
            pltpu.VMEM((8, 6 * D), F32),
            pltpu.VMEM((D, Fd), BF16),
            pltpu.VMEM((D, Fd), BF16),
            pltpu.VMEM((Fd // 2, D), U32),
            pltpu.VMEM((pl.cdiv(D, 128), 2 * TQ + 8, 128), F32),
            pltpu.SemaphoreType.DMA((12,)),
            pltpu.SemaphoreType.DMA((nblk // 2,)),
            pltpu.SemaphoreType.DMA((2,)),
            pltpu.SemaphoreType.DMA((nblk,)),
            pltpu.SemaphoreType.DMA((pl.cdiv(D, 128),)),
        ],
        compiler_params=pltpu.CompilerParams(dimension_semantics=("arbitrary",),
                                             vmem_limit_bytes=110 * 1024 * 1024,
                                             disable_bounds_checks=True,
                                             disable_semaphore_checks=True),
    )(c, B_w_r, A_x.reshape(S, D).T, A_k_cache.reshape(Hkv, Sk, Dh), A_v_cache.reshape(Hkv, Sk, Dh),
      A_wq, A_wo.T, w_mod, B_w_gate, B_w_up, B_w_down.T)
    return out_t.T.reshape(B, S, D)
```

```python
import math

import jax
import jax.numpy as jnp
from jax import lax
import jax.experimental.pallas as pl
import jax.experimental.pallas.tpu as pltpu

F32 = jnp.float32
BF16 = jnp.bfloat16
U32 = jnp.uint32
I32 = jnp.int32
EPS = 1e-05
TOPC = 8
NT = (((1,), (1,)), ((), ()))
TQ = 128
LG = 7
LU = 4
FW = 3 * 128
MT = 3
KEY_BIAS = 0x20000000


def _pk(x):
    return pltpu.bitcast(x, U32)


def _upk(x):
    return pltpu.bitcast(x, BF16)


def _rb(x):
    return x.astype(BF16).astype(F32)


def _tree(xs, op):
    while len(xs) > 1:
        xs = [op(xs[i], xs[i + 1]) if i + 1 < len(xs) else xs[i] for i in range(0, len(xs), 2)]
    return xs[0]


def _red0(x, op, red, grp):
    n = x.shape[0]
    acc = None
    for t in range(0, n, 8 * grp):
        part = _tree([x[j:j + 8, :] for j in range(t, min(t + 8 * grp, n), 8)], op)
        acc = part if acc is None else op(acc, part)
    return red(acc, axis=0, keepdims=True)


def _ln_finish(piv, s1, s2):
    var = jnp.maximum(s2 - s1 * s1, 0.0)
    return _rb(piv + s1), 1.0 / _rb(jnp.sqrt(_rb(_rb(var) + EPS)))


def _stats_t(x, w=None):
    d = x.shape[0]
    piv = x[0:1, :]
    xd = x - piv
    s1 = _red0(xd, jnp.add, jnp.sum, 8) * (1.0 / d)
    s2 = _red0(xd * xd, jnp.add, jnp.sum, 8) * (1.0 / d)
    mu, inv = _ln_finish(piv, s1, s2)
    if w is None:
        return mu, inv
    return mu, inv, _red0(xd * w, jnp.add, jnp.sum, 8), piv


def _kernel(c_hbm, wr_hbm, xt_hbm, k_hbm, v_hbm, wq_hbm, wot_hbm, wmod_hbm,
            wg_hbm, wu_hbm, wdt_hbm, out_hbm,
            x_sc, wmod_sc, kvst, wst, k_sc, vt_sc, wq_sc, wot_sc,
            h_sc, q_sc, s_sc, acc_sc, mod_sc, modt_sc, w_sc, out_sc, x1a_sc, x1b_sc, x1c_sc, xs_sc, st_sc,
            zv_sc, z_ref, ix_ref, o_sc, c_sc, wr_sc, mrow_sc, wg_sc, wu_sc, wd_sc, u_sc,
            sems, xsems, lsems, osems, fsems):
    D, S = x_sc.shape
    Hkv, Sk, Dh = k_hbm.shape
    G = 2 * Dh
    nblk = S // TQ
    ngrp = nblk // 2
    GW = 2 * TQ
    NF = wdt_hbm.shape[1] // FW
    qscale = (Dh ** -0.5) * math.log2(math.e)
    ftiles = [(n, f0, min(128, D - f0)) for n, f0 in enumerate(range(0, D, 128))]

    def ds(i, n):
        return slice(i * n, (i + 1) * n) if isinstance(i, int) else pl.ds(pl.multiple_of(i * n, n), n)

    def cp_k(g, slot, sem):
        return pltpu.make_async_copy(k_hbm.at[g], kvst.at[slot, 0:Sk, :], sem)

    def cp_v(g, slot, sem):
        return pltpu.make_async_copy(v_hbm.at[g], kvst.at[slot, Sk:2 * Sk, :], sem)

    def cp_wq(g, slot, sem):
        return pltpu.make_async_copy(wq_hbm.at[:, ds(g, G)], wst.at[slot, :, 0:G], sem)

    def cp_wo(g, slot, sem):
        return pltpu.make_async_copy(wot_hbm.at[:, ds(g, G)], wst.at[slot, :, G:2 * G], sem)

    def start_head(i, slot):
        cp_wq(i, slot, lsems.at[0]).start()
        cp_wo(i - 1, slot, lsems.at[0]).start()
        pltpu.make_async_copy(wdt_hbm.at[:, ds(jnp.minimum(i - 1, NF - 1), FW)],
                              wst.at[slot, :, 2 * G:2 * G + FW], lsems.at[0]).start()
        cp_k(i, slot, lsems.at[1]).start()
        cp_v(i, slot, lsems.at[1]).start()

    def wait_head(slot):
        pltpu.make_async_copy(wst.at[slot], wst.at[slot], lsems.at[0]).wait()
        pltpu.make_async_copy(kvst.at[slot], kvst.at[slot], lsems.at[1]).wait()

    def cp_x(j):
        return pltpu.make_async_copy(xt_hbm.at[:, ds(j, GW)], x_sc.at[:, ds(j, GW)], xsems.at[j])

    def cp_out(b):
        return pltpu.make_async_copy(out_sc.at[b + 1], out_hbm.at[:, ds(b, TQ)], osems.at[b])

    moe = [pltpu.make_async_copy(wg_hbm, wg_sc, sems.at[0]),
           pltpu.make_async_copy(wu_hbm, wu_sc, sems.at[1])]
    MA = 6 * 128
    cp_m0a = pltpu.make_async_copy(wmod_hbm.at[:, 0:MA], wmod_sc.at[:, 0:MA], sems.at[2])
    cp_m0b = pltpu.make_async_copy(wmod_hbm.at[:, MA:2 * D], wmod_sc.at[:, MA:2 * D], sems.at[11])
    cp_m1 = pltpu.make_async_copy(wmod_hbm.at[:, 2 * D:6 * D], wmod_sc.at[:, 2 * D:6 * D], sems.at[3])
    cp_c = pltpu.make_async_copy(c_hbm, c_sc, sems.at[4])
    cp_wr = pltpu.make_async_copy(wr_hbm, wr_sc, sems.at[5])
    cp_v0 = cp_v(0, 0, sems.at[6])
    KA = 3 * Sk // 8
    cp_k0a = pltpu.make_async_copy(k_hbm.at[0, 0:KA, :], kvst.at[0, 0:KA, :], sems.at[7])
    cp_k0b = pltpu.make_async_copy(k_hbm.at[0, KA:Sk, :], kvst.at[0, KA:Sk, :], sems.at[10])
    cp_wq0 = cp_wq(0, 0, sems.at[8])
    cp_wol = cp_wo(Hkv - 1, Hkv % 2, sems.at[9])

    def tie(v, dep):
        return pltpu.bitcast(pltpu.bitcast(v, U32) | (dep & zv_sc[...]), v.dtype)

    def ln1_pair(g, after=None):
        piv = jnp.broadcast_to(x_sc[0:16, ds(g, GW)].astype(F32)[0:1], (8, GW))
        if after is not None:
            piv = jnp.concatenate([tie(piv[:, :TQ], after), tie(piv[:, TQ:], after)], axis=1)
        s1 = s2 = None
        for r0 in range(0, D, 16):
            pw = piv
            if s2 is not None:
                b2 = pltpu.bitcast(s2, U32)
                pw = jnp.concatenate([tie(piv[:, :TQ], b2[:, :TQ]), tie(piv[:, TQ:], b2[:, TQ:])], axis=1)
            xd = x_sc[r0:r0 + 16, ds(g, GW)].astype(F32) - jnp.concatenate([pw, pw], axis=0)
            xq = xd * xd
            p1 = xd[0:8] + xd[8:16]
            p2 = xq[0:8] + xq[8:16]
            s1 = p1 if s1 is None else s1 + p1
            s2 = p2 if s2 is None else s2 + p2
        mu, inv = _ln_finish(piv, jnp.sum(s1, axis=0, keepdims=True) * (1.0 / D),
                             jnp.sum(s2, axis=0, keepdims=True) * (1.0 / D))
        g2 = g + z_ref[0]
        for _, f0, fw in ftiles:
            x = x_sc[f0:f0 + fw, ds(g2, GW)].astype(F32)
            n = (x - jnp.concatenate([mu] * (fw // 8), axis=0)) * inv
            h = n.T * mod_sc[1:2, f0:f0 + fw] + mod_sc[0:1, f0:f0 + fw]
            h_sc[ds(g, TQ), f0:f0 + fw] = _pk(h.astype(BF16))

    def mod_rest():
        dep = zv_sc[...]
        for c0 in range(2 * D, 6 * D, MT * 128):
            acc = None
            for r0 in range(0, D, 16):
                sc = modt_sc[r0:r0 + 16, :]
                sc = jnp.concatenate([tie(sc[0:8], dep), tie(sc[8:16], dep)], axis=0)
                pr = wmod_sc[r0:r0 + 16, c0:c0 + MT * 128].astype(F32) * jnp.concatenate([sc] * MT, axis=1)
                pr = pr[0:8] + pr[8:16]
                acc = pr if acc is None else acc + pr
                dep = pltpu.bitcast(acc[:, 0:128], U32)
            mrow_sc[:, c0:c0 + MT * 128] = acc

    def mod_finish():
        m = _rb(jnp.sum(mrow_sc[:, 2 * D:6 * D], axis=0, keepdims=True))
        ga = m[0:1, 0:D]
        sb = m[0:1, D:2 * D]
        cb1 = _rb(1.0 + m[0:1, 2 * D:3 * D])
        gb = m[0:1, 3 * D:4 * D]
        wr = wr_sc[...].astype(F32).reshape(1, D)
        mod_sc[2:3, :] = gb
        mod_sc[3:4, :] = sb
        mod_sc[4:5, :] = cb1
        mod_sc[5:6, :] = jnp.broadcast_to(jnp.sum(wr * cb1, axis=1, keepdims=True), (1, D))
        mod_sc[6:7, :] = jnp.broadcast_to(jnp.sum(wr * sb, axis=1, keepdims=True), (1, D))
        for i, vec in enumerate((ga, gb * cb1, gb * sb, wr * cb1)):
            modt_sc[i * D:(i + 1) * D, :] = jnp.broadcast_to(vec, (128, D)).T

    def qproj(c):
        h = _upk(h_sc[ds(c, TQ // 2), :])
        q = jnp.dot(h, _upk(wq_sc[...]), preferred_element_type=F32)
        q = (q * qscale).astype(BF16)
        return jnp.concatenate([q[:, :Dh], q[:, Dh:]], axis=0)

    def qk(c, q, split=False):
        if split:
            st = jnp.concatenate([
                lax.dot_general(_upk(k_sc[ds(j, Sk // 4), :]), q, NT, preferred_element_type=F32)
                for j in range(2)], axis=0)
        else:
            st = lax.dot_general(_upk(k_sc[...]), q, NT, preferred_element_type=F32)
        s_sc[c, 0:Sk, :] = st
        s_sc[c, Sk:Sk + 8, :] = jnp.broadcast_to(_red0(st, jnp.maximum, jnp.max, 1), (8, 2 * TQ))
        return pltpu.bitcast(st[0:8, 0:128], U32)

    def qk_rows(c, q, r0, r1):
        st = lax.dot_general(_upk(k_sc[r0 // 2:r1 // 2, :]), q, NT, preferred_element_type=F32)
        s_sc[c, r0:r1, :] = st
        m = jnp.broadcast_to(_red0(st, jnp.maximum, jnp.max, 1), (8, 2 * TQ))
        s_sc[c, Sk:Sk + 8, :] = m if r0 == 0 else jnp.maximum(m, s_sc[c, Sk:Sk + 8, :])

    def pv_cols(c, cols, ticks=None):
        p = jnp.exp2(s_sc[c, 0:Sk, cols] - s_sc[c, Sk:Sk + 1, cols])
        l = _red0(p, jnp.add, jnp.sum, 2)
        if ticks is None:
            ot = jnp.dot(_upk(vt_sc[...]), p.astype(BF16), preferred_element_type=F32)
        else:
            ot = None
            for r in range(0, Sk, Sk // 4):
                d = jnp.dot(_upk(vt_sc[:, r:r + Sk // 4]), p[r:r + Sk // 4].astype(BF16),
                            preferred_element_type=F32)
                ticks.extend(pltpu.bitcast(d[i:i + 8, 0:128], U32) for i in range(0, Dh, Dh // 4))
                ot = d if ot is None else ot + d
        return ot * (1.0 / l)

    def pv(c):
        ot = pv_cols(c, slice(0, 2 * TQ)).astype(BF16)
        return jnp.concatenate([ot[:, :TQ], ot[:, TQ:]], axis=0)

    def oproj(c, o2t, split=False, slot=None):
        if split:
            d = jnp.concatenate([
                jnp.dot(_upk(wot_sc[ds(j, D // 4), :]), o2t, preferred_element_type=F32)
                for j in range(2)], axis=0)
        else:
            d = jnp.dot(_upk(wot_sc[...]), o2t, preferred_element_type=F32)
        if slot is None:
            acc_sc[c] += d
        else:
            x1 = _rb(x_sc[:, ds(c, TQ)].astype(F32) + modt_sc[0:D, :] * (acc_sc[c] + d))
            xb = (x1a_sc, x1b_sc, x1c_sc)[slot // 2].at[slot % 2]
            xb[0:D, :] = x1
            mu, inv, rw, piv = _stats_t(x1, modt_sc[3 * D:4 * D, :])
            xb[D:D + 8, :] = jnp.broadcast_to(mu, (8, TQ))
            xb[D + 8:D + 16, :] = jnp.broadcast_to(inv, (8, TQ))
            st_sc[0, pl.ds(c, 1), :] = mu
            st_sc[1, pl.ds(c, 1), :] = inv
            st_sc[2, pl.ds(c, 1), :] = (rw - (mu - piv) * mod_sc[5:6, 0:TQ]) * inv + mod_sc[6:7, 0:TQ]

    def post(v0, xb, ticks=None, ch=None, cw=None, fresh=False):
        slots = [u + z_ref[0] if fresh else u for u in range(xb.shape[0])]
        mu0 = [xb[u, D:D + 8, :] for u in slots]
        inv0 = [xb[u, D + 8:D + 16, :] for u in slots]
        for _, f0, fw in ftiles:
            words = []
            for r0 in range(f0, f0 + fw, 32):
                gc = modt_sc[D + r0:D + r0 + 32, :]
                gs = modt_sc[2 * D + r0:2 * D + r0 + 32, :]
                if ticks is not None:
                    dep = ticks[r0 * len(ticks) // D]
                else:
                    dep = ch[-2] if len(ch) >= 2 else None
                    if r0 == f0 and len(cw) >= 3:
                        dep = dep | cw[-3]
                xs = []
                for u in range(len(slots)):
                    x1 = xb[slots[u], r0:r0 + 32, :]
                    xs.append(x1)
                    mu = mu0[u] if dep is None else tie(mu0[u], dep)
                    mu = jnp.concatenate([mu] * 4, axis=0)
                    inv = jnp.concatenate([inv0[u]] * 4, axis=0)
                    o = x1 + ((x1 - mu) * inv * gc + gs)
                    out_sc[v0 + u, r0:r0 + 32, :] = o.astype(BF16)
                wd = pltpu.bitcast(xs[0], U32)
                if ticks is not None:
                    wd = jnp.concatenate([tie(wd[0:8], dep), wd[8:]], axis=0)
                if len(xs) > 1:
                    wd = wd | (pltpu.bitcast(xs[1], U32) >> 16)
                words.append(wd)
                if ticks is None:
                    ch.append(_pk(out_sc[z_ref[0], 0:16, :]))
            w_sc[ds(v0 // 2, TQ), f0:f0 + fw] = pltpu.bitcast(jnp.concatenate(words, axis=0), F32).T
            if ticks is None:
                cw.append(pltpu.bitcast(w_sc[pl.ds(pl.multiple_of(z_ref[0], 8), 8), 0:128], U32))

    @pl.when(pl.program_id(0) == 0)
    def _():
        for cp in (cp_c, cp_x(0), cp_m0a):
            cp.start()

        def zero(i, carry):
            acc_sc[i] = jnp.zeros(acc_sc.shape[1:], F32)
            return carry
        lax.fori_loop(0, nblk, zero, 0)
        cp_m0b.start()

        def zero2(i, carry):
            x1b_sc[i & 1] = jnp.zeros(x1b_sc.shape[1:], F32)
            u_sc[i] = jnp.zeros(u_sc.shape[1:], F32)
            return carry
        lax.fori_loop(0, LU + 1, zero2, 0)
        o_sc[...] = jnp.zeros(o_sc.shape, U32)
        st_sc[...] = jnp.zeros(st_sc.shape, F32)
        zv_sc[...] = jnp.zeros(zv_sc.shape, U32)
        z_ref[0] = 0
        cp_c.wait()
        cp_wq0.start()
        cp_x(0).wait()
        cp_k0a.start()
        c = c_sc[...].astype(F32)
        scb = (c * jax.nn.sigmoid(c)).astype(BF16)
        modt_sc[0:D, :] = jnp.broadcast_to(scb.astype(F32), (128, D)).T
        for cc in range(2):
            x = x_sc[:, ds(cc, TQ)].astype(F32)
            mu, inv = _stats_t(x)
            w_sc[ds(cc, TQ), :] = ((x - mu) * inv).T
        sc8 = jnp.broadcast_to(scb, (8, D))
        cp_m0a.wait()
        cp_x(1).start()
        mrow_sc[:, 0:MA] = jnp.dot(sc8, wmod_sc[:, 0:MA], preferred_element_type=F32)
        cp_m0b.wait()
        cp_k0b.start()
        mrow_sc[:, MA:2 * D] = jnp.dot(sc8, wmod_sc[:, MA:2 * D], preferred_element_type=F32)
        m = _rb(mrow_sc[:, 0:2 * D])
        sa = m[0:1, 0:D]
        ca1 = _rb(1.0 + m[0:1, D:2 * D])
        mod_sc[0:1, :] = sa
        mod_sc[1:2, :] = ca1
        h_sc[0:TQ, :] = _pk((w_sc[0:2 * TQ, :] * ca1 + sa).astype(BF16))
        cp_wq0.wait()
        cp_x(2).start()
        cp_x(3).start()
        wq_sc[...] = _pk(wst[0, :, 0:G])
        q_sc[0] = _pk(qproj(0))
        q_sc[1] = _pk(qproj(1))
        cp_k0a.wait()
        k_sc[0:KA // 2, :] = _pk(kvst[0, 0:KA, :])
        qk_rows(0, _upk(q_sc[0]), 0, KA)
        qk_rows(1, _upk(q_sc[1]), 0, KA)
        cp_x(1).wait()
        cp_k0b.wait()
        for jj in range(4, ngrp):
            cp_x(jj).start()
        k_sc[KA // 2:Sk // 2, :] = _pk(kvst[0, KA:Sk, :])
        qk_rows(0, _upk(q_sc[0]), KA, Sk)
        qk_rows(1, _upk(q_sc[1]), KA, Sk)
        ln1_pair(1)
        q_sc[0] = _pk(qproj(2 + z_ref[0]))
        q_sc[1] = _pk(qproj(3 + z_ref[0]))

        def group(g, q0, q1, split):
            after = qk(2 * g, q0, split)
            qk(2 * g + 1, q1, split)
            ln1_pair(g + 1, after if split else None)
            return qproj(2 * g + 2 + z_ref[0]), qproj(2 * g + 3 + z_ref[0])

        def first(j, carry):
            cp_x(2 * j + 2).wait()
            cp_x(2 * j + 3).wait()

            @pl.when(j == 0)
            def _():
                cp_m1.start()
                cp_v0.start()
                cp_wr.start()
                start_head(1, 1)
            q0, q1 = group(2 * j + 1, _upk(q_sc[0]), _upk(q_sc[1]), False)
            q0, q1 = group(2 * j + 2, q0, q1, True)
            q_sc[0] = _pk(q0)
            q_sc[1] = _pk(q1)
            return carry
        lax.fori_loop(0, ngrp // 2 - 1, first, 0)

        cp_wr.wait()
        cp_m1.wait()
        cp_v0.wait()
        for cp in moe:
            cp.start()
        vt_sc[...] = _pk(kvst[0, Sk:2 * Sk, :].T)
        mod_rest()
        qk(nblk - 2, _upk(q_sc[0]))
        qk(nblk - 1, _upk(q_sc[1]))

        def main(i, carry):
            slot = i & 1
            wait_head(slot)
            wq_sc[...] = _pk(wst[slot, :, 0:G])

            @pl.when(i + 1 < Hkv)
            def _():
                start_head(i + 1, 1 - slot)

            @pl.when(i + 1 == Hkv)
            def _():
                cp_wol.start()

            k_sc[...] = _pk(kvst[slot, 0:Sk, :])
            wot_sc[...] = _pk(wst[slot, :, G:2 * G])
            q = qproj(0)
            for c in range(nblk):
                end = c == nblk - 1
                o = pv(c)
                qn = None if end else qproj(c + 1)
                qk(c, q, split=end)
                oproj(c, o, split=end)
                q = qn
            vt_sc[...] = _pk(kvst[slot, Sk:2 * Sk, :].T)
            mod_finish()
            wd_sc[ds(jnp.minimum(i - 1, NF - 1), FW // 2), :] = _pk(wst[slot, :, 2 * G:2 * G + FW].T)
            return carry
        lax.fori_loop(1, Hkv, main, 0)

    @pl.when(pl.program_id(0) == 1)
    def _():
        cp_wol.wait()
        wot_sc[...] = _pk(wst[Hkv % 2, :, G:2 * G])

        def last(j, carry):
            ticks = []
            o = _upk(o_sc[...])
            for u in range(LU):
                c = LU * j + u - 1
                if u == 0:
                    oproj(jnp.maximum(c, 0), o, slot=u)
                    o0 = pv_cols(c + 1, slice(0, TQ), ticks)
                else:
                    o0 = pv_cols(c + 1, slice(0, TQ), ticks)
                    if u == 2:
                        post(LU * jnp.maximum(j - 1, 0) + 2, x1b_sc, ticks[8:48])
                    oproj(c, o, slot=u)
                o1 = pv_cols(c + 1, slice(TQ, 2 * TQ), ticks)
                o = jnp.concatenate([o0, o1], axis=0).astype(BF16)
            post(LU * j, x1a_sc, ticks[68:104], fresh=True)
            o_sc[...] = _pk(o)
            return carry
        lax.fori_loop(0, nblk // LU, last, 0)

        oproj(nblk - 1, _upk(o_sc[...]), split=True, slot=LU)

        r = _rb(st_sc[2]) + 0.0
        b16 = pltpu.bitcast(r, U32) >> 16
        ordk = jnp.where(b16 >= 0x8000, 0xFFFF - b16, b16 + 0x8000)
        tok = lax.broadcasted_iota(U32, r.shape, 0) * TQ + lax.broadcasted_iota(U32, r.shape, 1)
        key = pltpu.bitcast((ordk << 11) + (S - 1 - tok) + KEY_BIAS, F32)

        def rank(row, col):
            return _red0(jnp.where(col > row, 1.0, 0.0), jnp.add, jnp.sum, 16)

        lm = jnp.max(key, axis=0, keepdims=True)
        lrank = rank(lm, jnp.broadcast_to(lm, (TQ, TQ)).T)
        cand = jnp.concatenate([jnp.where(lrank == float(t), key, 0.0) for t in range(TOPC)], axis=0)
        cand = jnp.broadcast_to(jnp.max(cand, axis=1, keepdims=True), (TOPC * nblk, TQ))
        eye = lax.broadcasted_iota(I32, cand.shape, 0) == lax.broadcasted_iota(I32, cand.shape, 1)
        crow = _red0(jnp.where(eye, cand, 0.0), jnp.maximum, jnp.max, 16)
        crank = rank(crow, cand)
        subf = lax.broadcasted_iota(I32, (TOPC, TQ), 0).astype(F32)
        top = jnp.max(jnp.where(crank == subf, crow, 0.0), axis=1, keepdims=True)
        top = jnp.broadcast_to(top, (TOPC, TQ))
        mus = jnp.zeros((TOPC, TQ), F32)
        invs = jnp.zeros((TOPC, TQ), F32)
        for cc in range(nblk):
            sel = key[cc:cc + 1, :] == top
            mus = jnp.where(sel, st_sc[0, cc:cc + 1, :], mus)
            invs = jnp.where(sel, st_sc[1, cc:cc + 1, :], invs)
        ch, cw = [], []
        post(nblk - 2, x1b_sc, ch=ch, cw=cw)
        post(nblk, x1c_sc, ch=ch, cw=cw)
        topi = S - 1 - (pltpu.bitcast(top, I32) & (S - 1))
        rowi = ((((topi >> LG) + 1) >> 1) << LG) + (topi & (TQ - 1))
        for t in range(TOPC):
            xs_sc[t:t + 1, :] = w_sc[pl.ds(jnp.clip(rowi[t, 0], 0, w_sc.shape[0] - 1), 1), :]
        idxs = [jnp.clip(topi[t, 0], 0, S - 1) for t in range(TOPC)]
        blks = [ix >> LG for ix in idxs]
        hmask = 0
        for t in range(TOPC):
            hmask = hmask | (1 << blks[t])
        clean = [((hmask >> b) & 1) == 0 for b in range(nblk)]
        for b in range(nblk):
            @pl.when(clean[b])
            def _():
                cp_out(b).start()
        ordt = (pltpu.bitcast(top, U32) - KEY_BIAS) >> 11
        rsel = pltpu.bitcast(jnp.where(ordt >= 0x8000, ordt - 0x8000, 0xFFFF - ordt) << 16, F32)[:, 0:1]
        mus = jnp.sum(mus, axis=1, keepdims=True)
        invs = jnp.sum(invs, axis=1, keepdims=True)
        words = pltpu.bitcast(xs_sc[...], U32)
        low = ((topi[:, 0:1] >> LG) & 1) == 0
        x1s = pltpu.bitcast(jnp.where(low, words << 16, words & jnp.uint32(0xFFFF0000)), F32)
        h2s = _rb(_rb(_rb(_rb(x1s - mus) * invs) * mod_sc[4:5, :]) + mod_sc[3:4, :])
        xsel = h2s.astype(BF16)

        for cp in moe:
            cp.wait()
        gt = _rb(jnp.dot(xsel, wg_sc[...], preferred_element_type=F32))
        ut = _rb(jnp.dot(xsel, wu_sc[...], preferred_element_type=F32))
        af = _rb(gt * jax.nn.sigmoid(gt)) * ut
        gate = _rb(jax.nn.sigmoid(rsel))
        lns = [ix & (TQ - 1) for ix in idxs]
        color, lead = [], []
        for t in range(TOPC):
            cl, dup = 0, False
            for s_ in range(t):
                cl = cl + (lns[s_] == lns[t]).astype(I32)
                dup = jnp.logical_or(dup, blks[s_] == blks[t])
            color.append(cl)
            lead.append(jnp.logical_not(dup))
        cmax = color[TOPC - 1]
        for t in range(1, TOPC - 1):
            cmax = jnp.maximum(cmax, color[t])

        def cp_fix(t, n, f0, fw):
            return pltpu.make_async_copy(out_sc.at[blks[t] + 1, f0:f0 + fw, :],
                                         out_hbm.at[f0:f0 + fw, ds(blks[t], TQ)], fsems.at[n])

        def merge(blk, ln, f0, fw, val):
            cur = out_sc[blk + 1, f0:f0 + fw, :].astype(F32)
            lane = lax.broadcasted_iota(I32, (fw, TQ), 1)
            out_sc[blk + 1, f0:f0 + fw, :] = jnp.where(lane == ln, val, cur).astype(BF16)

        def scatter(n, f0, fw, new):
            now = [(color[t] >> 1) == 0 for t in range(TOPC)]
            for t in range(TOPC):
                row = jnp.where(now[t], lns[t] + (color[t] & 1) * TQ, 2 * TQ)
                u_sc[n, pl.ds(row, 1), 0:fw] = new[t:t + 1, :]
            ut_ = u_sc[n, 0:2 * TQ, 0:fw].T
            for t in range(TOPC):
                val = ut_[:, :TQ] if t == 0 else jnp.where((color[t] & 1) == 0, ut_[:, :TQ], ut_[:, TQ:])
                merge(blks[t], jnp.where(now[t], lns[t], TQ), f0, fw, val)

        kb = (af.shape[1] // 128) * 8 // 9 * 128
        fence, news = [], []
        for n, f0, fw in ftiles:
            an = af
            if n >= 2:
                an = jnp.concatenate([af[:, :kb], tie(af[:, kb:kb + 128], fence[n - 2]), af[:, kb + 128:]],
                                     axis=1)
            y = _rb(jnp.dot(an.astype(BF16), _upk(wd_sc[:, f0:f0 + fw]), preferred_element_type=F32))
            y = _rb(y * gate)
            new = x1s[:, f0:f0 + fw] + mod_sc[2:3, f0:f0 + fw] * _rb(h2s[:, f0:f0 + fw] + y)
            news.append(new)
            scatter(n, f0, fw, new)
            fence.append(_pk(out_sc[z_ref[0], 0:16, :]))
            for t in range(TOPC):
                @pl.when(lead[t])
                def _():
                    cp_fix(t, n, f0, fw).start()
        xs_sc[...] = jnp.concatenate(news, axis=1)

        for b in range(nblk):
            @pl.when(clean[b])
            def _():
                cp_out(b).wait()
        for n, f0, fw in ftiles:
            for t in range(TOPC):
                @pl.when(lead[t])
                def _():
                    cp_fix(t, n, f0, fw).wait()

        @pl.when(cmax >= 2)
        def _():
            for t in range(TOPC):
                ix_ref[t] = idxs[t]

            def redo(t, carry):
                ln = ix_ref[t] & (TQ - 1)
                row = xs_sc[pl.ds(t, 1), :]
                for n, f0, fw in ftiles:
                    u_sc[n, pl.ds(ln, 1), 0:fw] = row[:, f0:f0 + fw]
                    merge(ix_ref[t] >> LG, ln, f0, fw, u_sc[n, 0:TQ, 0:fw].T)
                return carry
            lax.fori_loop(2, TOPC, redo, 0)
            for t in range(TOPC):
                @pl.when(lead[t])
                def _():
                    cp_fix(t, 0, 0, D).start()
            for t in range(TOPC):
                @pl.when(lead[t])
                def _():
                    cp_fix(t, 0, 0, D).wait()


@jax.jit
def pallas_adaLN_cond__gqa_block_cached__moe_arch_mod__prompt_kernel(
    A_x: jax.Array,
    A_k_cache: jax.Array,
    A_v_cache: jax.Array,
    A_wq: jax.Array,
    A_wo: jax.Array,
    B_x: jax.Array,
    B_w_r: jax.Array,
    B_w_gate: jax.Array,
    B_w_up: jax.Array,
    B_w_down: jax.Array,
    c: jax.Array,
    w_mod: jax.Array,
):
    del B_x
    B, S, D = A_x.shape
    _, Hkv, Sk, Dh = A_k_cache.shape
    G = A_wq.shape[1] // Hkv
    Fd = B_w_gate.shape[1]
    nblk = S // TQ
    assert B == 1 and G == 2 * Dh and TOPC * nblk == TQ and Fd % FW == 0 and Fd // FW < Hkv
    assert pl.cdiv(D, 128) == LU + 1 and (2 * D) % 128 == 0 and 6 * 128 < 2 * D and (4 * D) % (MT * 128) == 0
    hbm = pl.BlockSpec(memory_space=pl.ANY)
    out_t = pl.pallas_call(
        _kernel,
        grid=(2,),
        in_specs=[hbm] * 11,
        out_specs=hbm,
        out_shape=jax.ShapeDtypeStruct((D, S), BF16),
        scratch_shapes=[
            pltpu.VMEM((D, S), BF16),
            pltpu.VMEM((D, 6 * D), BF16),
            pltpu.VMEM((2, 2 * Sk, Dh), BF16),
            pltpu.VMEM((2, D, 2 * G + FW), BF16),
            pltpu.VMEM((Sk // 2, Dh), U32),
            pltpu.VMEM((Dh // 2, Sk), U32),
            pltpu.VMEM((D // 2, G), U32),
            pltpu.VMEM((D // 2, G), U32),
            pltpu.VMEM((S // 2, D), U32),
            pltpu.VMEM((2, TQ, Dh), U32),
            pltpu.VMEM((nblk, Sk + 8, 2 * TQ), F32),
            pltpu.VMEM((nblk, D, TQ), F32),
            pltpu.VMEM((8, D), F32),
            pltpu.VMEM((4 * D, 128), F32),
            pltpu.VMEM((S // 2 + TQ, D), F32),
            pltpu.VMEM((nblk + 1, D, TQ), BF16),
            pltpu.VMEM((2, D + 16, TQ), F32),
            pltpu.VMEM((2, D + 16, TQ), F32),
            pltpu.VMEM((1, D + 16, TQ), F32),
            pltpu.VMEM((TOPC, D), F32),
            pltpu.VMEM((3, nblk, TQ), F32),
            pltpu.VMEM((8, 128), U32),
            pltpu.SMEM((1,), I32),
            pltpu.SMEM((TOPC,), I32),
            pltpu.VMEM((Dh, TQ), U32),
            pltpu.VMEM((1, D), BF16),
            pltpu.VMEM((D,), BF16),
            pltpu.VMEM((8, 6 * D), F32),
            pltpu.VMEM((D, Fd), BF16),
            pltpu.VMEM((D, Fd), BF16),
            pltpu.VMEM((Fd // 2, D), U32),
            pltpu.VMEM((pl.cdiv(D, 128), 2 * TQ + 8, 128), F32),
            pltpu.SemaphoreType.DMA((12,)),
            pltpu.SemaphoreType.DMA((nblk // 2,)),
            pltpu.SemaphoreType.DMA((2,)),
            pltpu.SemaphoreType.DMA((nblk,)),
            pltpu.SemaphoreType.DMA((pl.cdiv(D, 128),)),
        ],
        compiler_params=pltpu.CompilerParams(dimension_semantics=("arbitrary",),
                                             vmem_limit_bytes=110 * 1024 * 1024,
                                             disable_bounds_checks=True,
                                             disable_semaphore_checks=True),
    )(c, B_w_r, A_x.reshape(S, D).T, A_k_cache.reshape(Hkv, Sk, Dh), A_v_cache.reshape(Hkv, Sk, Dh),
      A_wq, A_wo.T, w_mod, B_w_gate, B_w_up, B_w_down.T)
    return out_t.T.reshape(B, S, D)
```

```python
import math

import jax
import jax.numpy as jnp
from jax import lax
import jax.experimental.pallas as pl
import jax.experimental.pallas.tpu as pltpu

F32 = jnp.float32
BF16 = jnp.bfloat16
U32 = jnp.uint32
I32 = jnp.int32
EPS = 1e-05
TOPC = 8
NT = (((1,), (1,)), ((), ()))
TQ = 128
LG = 7
LU = 4
FW = 3 * 128
MT = 3
KEY_BIAS = 0x20000000
KS = 8
NC = 2
TICKS = (2, 72, 224)


def _pk(x):
    return pltpu.bitcast(x, U32)


def _upk(x):
    return pltpu.bitcast(x, BF16)


def _rb(x):
    return x.astype(BF16).astype(F32)


def _tree(xs, op):
    while len(xs) > 1:
        xs = [op(xs[i], xs[i + 1]) if i + 1 < len(xs) else xs[i] for i in range(0, len(xs), 2)]
    return xs[0]


def _red0(x, op, red, grp):
    n = x.shape[0]
    acc = None
    for t in range(0, n, 8 * grp):
        part = _tree([x[j:j + 8, :] for j in range(t, min(t + 8 * grp, n), 8)], op)
        acc = part if acc is None else op(acc, part)
    return red(acc, axis=0, keepdims=True)


def _ln_finish(piv, s1, s2):
    var = jnp.maximum(s2 - s1 * s1, 0.0)
    return _rb(piv + s1), 1.0 / _rb(jnp.sqrt(_rb(_rb(var) + EPS)))


def _stats_t(x, w=None):
    d = x.shape[0]
    piv = x[0:1, :]
    xd = x - piv
    s1 = _red0(xd, jnp.add, jnp.sum, 8) * (1.0 / d)
    s2 = _red0(xd * xd, jnp.add, jnp.sum, 8) * (1.0 / d)
    mu, inv = _ln_finish(piv, s1, s2)
    if w is None:
        return mu, inv
    return mu, inv, _red0(xd * w, jnp.add, jnp.sum, 8), piv


def _kernel(c_hbm, wr_hbm, xt_hbm, k_hbm, v_hbm, wq_hbm, wot_hbm, wmod_hbm,
            wg_hbm, wu_hbm, wdt_hbm, out_hbm,
            x_sc, wmod_sc, kvst, wst, k_sc, vt_sc, wq_sc, wot_sc,
            h_sc, q_sc, s_sc, acc_sc, mod_sc, modt_sc, w_sc, out_sc, x1a_sc, x1b_sc, x1c_sc, xs_sc, st_sc,
            zv_sc, z_ref, ix_ref, o_sc, c_sc, wr_sc, mrow_sc, wg_sc, wu_sc, wd_sc, u_sc,
            wl_sc, hb_sc, wb_sc, ql_sc, wt_sc, af_sc, sct_sc,
            sems, xsems, lsems, osem):
    D, S = x_sc.shape
    Hkv, Sk, Dh = k_hbm.shape
    G = 2 * Dh
    nblk = S // TQ
    ngrp = nblk // 2
    GW = 2 * TQ
    NF = wdt_hbm.shape[1] // FW
    qscale = (Dh ** -0.5) * math.log2(math.e)
    ftiles = [(n, f0, min(128, D - f0)) for n, f0 in enumerate(range(0, D, 128))]

    def ds(i, n):
        return slice(i * n, (i + 1) * n) if isinstance(i, int) else pl.ds(pl.multiple_of(i * n, n), n)

    def cp_k(g, slot, sem):
        return pltpu.make_async_copy(k_hbm.at[g], kvst.at[slot, 0:Sk, :], sem)

    def cp_v(g, slot, sem):
        return pltpu.make_async_copy(v_hbm.at[g], kvst.at[slot, Sk:2 * Sk, :], sem)

    def cp_wq(g, slot, sem):
        return pltpu.make_async_copy(wq_hbm.at[:, ds(g, G)], wst.at[slot, :, 0:G], sem)

    def cp_wo(g, slot, sem):
        return pltpu.make_async_copy(wot_hbm.at[:, ds(g, G)], wst.at[slot, :, G:2 * G], sem)

    def start_head(i, slot):
        cp_wq(i, slot, lsems.at[0]).start()
        cp_wo(i - 1, slot, lsems.at[0]).start()
        pltpu.make_async_copy(wdt_hbm.at[:, ds(jnp.minimum(i - 1, NF - 1), FW)],
                              wst.at[slot, :, 2 * G:2 * G + FW], lsems.at[0]).start()
        cp_k(i, slot, lsems.at[1]).start()
        cp_v(i, slot, lsems.at[1]).start()

    def wait_head(slot):
        pltpu.make_async_copy(wst.at[slot], wst.at[slot], lsems.at[0]).wait()
        pltpu.make_async_copy(kvst.at[slot], kvst.at[slot], lsems.at[1]).wait()

    def cp_x(j):
        return pltpu.make_async_copy(xt_hbm.at[:, ds(j, GW)], x_sc.at[:, ds(j, GW)], xsems.at[j])

    def cp_out(b):
        return pltpu.make_async_copy(out_sc.at[b + 1], out_hbm.at[:, ds(b, TQ)], osem.at[0])

    moe = [pltpu.make_async_copy(wg_hbm, wg_sc, sems.at[0]),
           pltpu.make_async_copy(wu_hbm, wu_sc, sems.at[1])]
    MA = 6 * 128
    cp_m0a = pltpu.make_async_copy(wmod_hbm.at[:, 0:MA], wmod_sc.at[:, 0:MA], sems.at[2])
    cp_m0b = pltpu.make_async_copy(wmod_hbm.at[:, MA:2 * D], wmod_sc.at[:, MA:2 * D], sems.at[11])
    cp_m1 = pltpu.make_async_copy(wmod_hbm.at[:, 2 * D:6 * D], wmod_sc.at[:, 2 * D:6 * D], sems.at[3])
    cp_c = pltpu.make_async_copy(c_hbm, c_sc, sems.at[4])
    cp_wr = pltpu.make_async_copy(wr_hbm, wr_sc, sems.at[5])
    cp_v0 = cp_v(0, 0, sems.at[6])
    KA = 3 * Sk // 8
    cp_k0a = pltpu.make_async_copy(k_hbm.at[0, 0:KA, :], kvst.at[0, 0:KA, :], sems.at[7])
    cp_k0b = pltpu.make_async_copy(k_hbm.at[0, KA:Sk, :], kvst.at[0, KA:Sk, :], sems.at[10])
    cp_wq0 = cp_wq(0, 0, sems.at[8])
    cp_wol = cp_wo(Hkv - 1, Hkv % 2, sems.at[9])
    DM = D // 128 * 128
    DL = D - DM
    cp_wla = pltpu.make_async_copy(wq_hbm.at[DM:D, G:3 * G], wl_sc.at[:, G:3 * G], sems.at[12])
    cp_wlb = pltpu.make_async_copy(wq_hbm.at[DM:D, 3 * G:], wl_sc.at[:, 3 * G:], sems.at[13])

    def tie(v, dep):
        return pltpu.bitcast(pltpu.bitcast(v, U32) | (dep & zv_sc[:, 0:dep.shape[1]]), v.dtype)

    def ln1_pair(g, after=None):
        piv = jnp.broadcast_to(x_sc[0:16, ds(g, GW)].astype(F32)[0:1], (8, GW))
        if after is not None:
            piv = jnp.concatenate([tie(piv[:, :TQ], after), tie(piv[:, TQ:], after)], axis=1)
        s1 = s2 = None
        for r0 in range(0, D, 16):
            pw = piv
            if s2 is not None:
                b2 = pltpu.bitcast(s2, U32)
                pw = jnp.concatenate([tie(piv[:, :TQ], b2[:, :TQ]), tie(piv[:, TQ:], b2[:, TQ:])], axis=1)
            xd = x_sc[r0:r0 + 16, ds(g, GW)].astype(F32) - jnp.concatenate([pw, pw], axis=0)
            xq = xd * xd
            p1 = xd[0:8] + xd[8:16]
            p2 = xq[0:8] + xq[8:16]
            s1 = p1 if s1 is None else s1 + p1
            s2 = p2 if s2 is None else s2 + p2
        mu, inv = _ln_finish(piv, jnp.sum(s1, axis=0, keepdims=True) * (1.0 / D),
                             jnp.sum(s2, axis=0, keepdims=True) * (1.0 / D))
        g2 = g + z_ref[0]
        for _, f0, fw in ftiles:
            x = x_sc[f0:f0 + fw, ds(g2, GW)].astype(F32)
            n = (x - jnp.concatenate([mu] * (fw // 8), axis=0)) * inv
            h = n.T * mod_sc[1:2, f0:f0 + fw] + mod_sc[0:1, f0:f0 + fw]
            h_sc[ds(g, TQ), f0:f0 + fw] = _pk(h.astype(BF16))

    def mod_rest(ticks):
        total = (4 * D // (MT * 128)) * (D // 16)
        i = 0
        for c0 in range(2 * D, 6 * D, MT * 128):
            acc = None
            for r0 in range(0, D, 16):
                sc = sct_sc[r0:r0 + 16, :]
                sc = jnp.concatenate([tie(sc[0:8], ticks[i * len(ticks) // total]), sc[8:16]], axis=0)
                i += 1
                pr = wmod_sc[r0:r0 + 16, c0:c0 + MT * 128].astype(F32) * jnp.concatenate([sc] * MT, axis=1)
                acc = pr[0:8] if acc is None else acc + pr[0:8]
                acc = acc + pr[8:16]
            mrow_sc[:, c0:c0 + MT * 128] = acc

    def mod_finish():
        m = _rb(jnp.sum(mrow_sc[:, 2 * D:6 * D], axis=0, keepdims=True))
        ga = m[0:1, 0:D]
        sb = m[0:1, D:2 * D]
        cb1 = _rb(1.0 + m[0:1, 2 * D:3 * D])
        gb = m[0:1, 3 * D:4 * D]
        wr = wr_sc[...].astype(F32).reshape(1, D)
        mod_sc[2:3, :] = gb
        mod_sc[3:4, :] = sb
        mod_sc[4:5, :] = cb1
        mod_sc[5:6, :] = jnp.broadcast_to(jnp.sum(wr * cb1, axis=1, keepdims=True), (1, D))
        mod_sc[6:7, :] = jnp.broadcast_to(jnp.sum(wr * sb, axis=1, keepdims=True), (1, D))
        for i, vec in enumerate((ga, gb * cb1, gb * sb, wr * cb1)):
            mod_sc[8 + i:9 + i, :] = vec

    def qproj(c, rest=None):
        h = _upk(h_sc[ds(c, TQ // 2), :])
        if rest is None:
            q = jnp.dot(h, _upk(wq_sc[...]), preferred_element_type=F32)
            q = (q * qscale).astype(BF16)
            return jnp.concatenate([q[:, :Dh], q[:, Dh:]], axis=0)
        qb = jnp.dot(h[:, 0:DM], _upk(wq_sc[0:DM // 2, Dh:G]), preferred_element_type=F32) + rest
        qa = jnp.dot(h, _upk(wq_sc[:, 0:Dh]), preferred_element_type=F32)
        return (jnp.concatenate([qa, qb], axis=0) * qscale).astype(BF16)

    def wl_t(g):
        return wl_sc[:, ds(2 * g + 1, Dh)].astype(F32).T

    def hb_group(g, ticks):
        ht = _upk(h_sc[ds(g, TQ), DM:D]).astype(F32).T
        for u in range(2):
            for k0 in range(0, DL, 8):
                h8 = tie(ht[k0:k0 + 8, u * TQ:(u + 1) * TQ], ticks[(u * DL + k0) * len(ticks) // (2 * DL)])
                hb_sc[2 * g + u, 8 * k0:8 * k0 + 64, :] = jnp.concatenate(
                    [jnp.broadcast_to(h8[k:k + 1], (8, TQ)) for k in range(8)], axis=0)

    def wb_group(n, wt, ticks):
        for k0 in range(0, DL, 4):
            w = tie(wt, ticks[k0 * len(ticks) // DL][:, 0:DL])
            wb_sc[n, 8 * k0:8 * k0 + 32, :] = jnp.concatenate(
                [jnp.broadcast_to(w[:, k:k + 1], (8, 128)) for k in range(k0, k0 + 4)], axis=0)

    def marks(st):
        return [pltpu.bitcast(st[r:r + 8, 0:128], U32) for r in range(0, st.shape[0], 8)]

    def qk(c, q, split=False):
        if split:
            st = jnp.concatenate([
                lax.dot_general(_upk(k_sc[ds(j, Sk // 4), :]), q, NT, preferred_element_type=F32)
                for j in range(2)], axis=0)
        else:
            st = lax.dot_general(_upk(k_sc[...]), q, NT, preferred_element_type=F32)
        s_sc[c, 0:Sk, :] = st
        s_sc[c, Sk:Sk + 8, :] = jnp.broadcast_to(_red0(st, jnp.maximum, jnp.max, 1), (8, 2 * TQ))
        return marks(st[0:Sk // 2] if split else st)

    def qk_rows(c, q, r0, r1):
        st = lax.dot_general(_upk(k_sc[r0 // 2:r1 // 2, :]), q, NT, preferred_element_type=F32)
        s_sc[c, r0:r1, :] = st
        m = jnp.broadcast_to(_red0(st, jnp.maximum, jnp.max, 1), (8, 2 * TQ))
        s_sc[c, Sk:Sk + 8, :] = m if r0 == 0 else jnp.maximum(m, s_sc[c, Sk:Sk + 8, :])
        return marks(st)

    def pv_cols(c, cols, ticks=None):
        p = jnp.exp2(s_sc[c, 0:Sk, cols] - s_sc[c, Sk:Sk + 1, cols])
        l = _red0(p, jnp.add, jnp.sum, 2)
        if ticks is None:
            ot = jnp.dot(_upk(vt_sc[...]), p.astype(BF16), preferred_element_type=F32)
        else:
            ot = None
            for r in range(0, Sk, Sk // 4):
                d = jnp.dot(_upk(vt_sc[:, r:r + Sk // 4]), p[r:r + Sk // 4].astype(BF16),
                            preferred_element_type=F32)
                ticks.extend(pltpu.bitcast(d[i:i + 8, 0:128], U32) for i in range(0, Dh, Dh // 4))
                ot = d if ot is None else ot + d
        return ot * (1.0 / l)

    def pv(c):
        ot = pv_cols(c, slice(0, 2 * TQ)).astype(BF16)
        return jnp.concatenate([ot[:, :TQ], ot[:, TQ:]], axis=0)

    def oproj(c, o2t, split=False, slot=None):
        if split:
            d = jnp.concatenate([
                jnp.dot(_upk(wot_sc[ds(j, D // 4), :]), o2t, preferred_element_type=F32)
                for j in range(2)], axis=0)
        else:
            d = jnp.dot(_upk(wot_sc[...]), o2t, preferred_element_type=F32)
        if slot is None:
            acc_sc[c] += d
        else:
            x1 = _rb(x_sc[:, ds(c, TQ)].astype(F32) + modt_sc[0:D, :] * (acc_sc[c] + d))
            xb = (x1a_sc, x1b_sc, x1c_sc)[slot // 2].at[slot % 2]
            xb[0:D, :] = x1
            mu, inv, rw, piv = _stats_t(x1, modt_sc[3 * D:4 * D, :])
            xb[D:D + 8, :] = jnp.broadcast_to(mu, (8, TQ))
            xb[D + 8:D + 16, :] = jnp.broadcast_to(inv, (8, TQ))
            st_sc[0, pl.ds(c, 1), :] = mu
            st_sc[1, pl.ds(c, 1), :] = inv
            st_sc[2, pl.ds(c, 1), :] = (rw - (mu - piv) * mod_sc[5:6, 0:TQ]) * inv + mod_sc[6:7, 0:TQ]

    def post(v0, xb, ticks=None, ch=None, cw=None, fresh=False):
        slots = [u + z_ref[0] if fresh else u for u in range(xb.shape[0])]
        mu0 = [xb[u, D:D + 8, :] for u in slots]
        inv0 = [xb[u, D + 8:D + 16, :] for u in slots]
        for _, f0, fw in ftiles:
            words = []
            for r0 in range(f0, f0 + fw, 32):
                gc = modt_sc[D + r0:D + r0 + 32, :]
                gs = modt_sc[2 * D + r0:2 * D + r0 + 32, :]
                if ticks is not None:
                    dep = ticks[r0 * len(ticks) // D]
                else:
                    dep = ch[-2] if len(ch) >= 2 else None
                    if r0 == f0 and len(cw) >= 3:
                        dep = dep | cw[-3]
                xs = []
                for u in range(len(slots)):
                    x1 = xb[slots[u], r0:r0 + 32, :]
                    xs.append(x1)
                    mu = mu0[u] if dep is None else tie(mu0[u], dep)
                    mu = jnp.concatenate([mu] * 4, axis=0)
                    inv = jnp.concatenate([inv0[u]] * 4, axis=0)
                    o = x1 + ((x1 - mu) * inv * gc + gs)
                    out_sc[v0 + u, r0:r0 + 32, :] = o.astype(BF16)
                wd = pltpu.bitcast(xs[0], U32)
                if ticks is not None:
                    wd = jnp.concatenate([tie(wd[0:8], dep), wd[8:]], axis=0)
                if len(xs) > 1:
                    wd = wd | (pltpu.bitcast(xs[1], U32) >> 16)
                words.append(wd)
                if ticks is None:
                    ch.append(_pk(out_sc[z_ref[0], 0:16, :]))
            w_sc[ds(v0 // 2, TQ), f0:f0 + fw] = pltpu.bitcast(jnp.concatenate(words, axis=0), F32).T
            if ticks is None:
                cw.append(pltpu.bitcast(w_sc[pl.ds(pl.multiple_of(z_ref[0], 8), 8), 0:128], U32))

    @pl.when(pl.program_id(0) == 0)
    def _():
        for cp in (cp_c, cp_x(0), cp_m0a):
            cp.start()

        def zero(i, carry):
            acc_sc[i] = jnp.zeros(acc_sc.shape[1:], F32)
            return carry
        lax.fori_loop(0, nblk, zero, 0)
        cp_m0b.start()

        def zero2(i, carry):
            x1b_sc[i & 1] = jnp.zeros(x1b_sc.shape[1:], F32)
            u_sc[i] = jnp.zeros(u_sc.shape[1:], F32)
            return carry
        lax.fori_loop(0, LU + 1, zero2, 0)
        o_sc[...] = jnp.zeros(o_sc.shape, U32)
        st_sc[...] = jnp.zeros(st_sc.shape, F32)
        zv_sc[...] = jnp.zeros(zv_sc.shape, U32)
        z_ref[0] = 0
        cp_c.wait()
        cp_wq0.start()
        cp_x(0).wait()
        cp_k0a.start()
        c = c_sc[...].astype(F32)
        scb = (c * jax.nn.sigmoid(c)).astype(BF16)
        sct_sc[...] = jnp.broadcast_to(scb.astype(F32), (128, D)).T

        def norm0(cc, carry):
            x = x_sc[:, ds(cc, TQ)].astype(F32)
            mu, inv = _stats_t(x)
            w_sc[ds(cc, TQ), :] = ((x - mu) * inv).T
            return carry
        lax.fori_loop(0, 2, norm0, 0)
        sc8 = jnp.broadcast_to(scb, (8, D))
        cp_m0a.wait()
        cp_x(1).start()
        mrow_sc[:, 0:MA] = jnp.dot(sc8, wmod_sc[:, 0:MA], preferred_element_type=F32)
        cp_m0b.wait()
        cp_k0b.start()
        mrow_sc[:, MA:2 * D] = jnp.dot(sc8, wmod_sc[:, MA:2 * D], preferred_element_type=F32)
        m = _rb(mrow_sc[:, 0:2 * D])
        sa = m[0:1, 0:D]
        ca1 = _rb(1.0 + m[0:1, D:2 * D])
        mod_sc[0:1, :] = sa
        mod_sc[1:2, :] = ca1
        h_sc[0:TQ, :] = _pk((w_sc[0:2 * TQ, :] * ca1 + sa).astype(BF16))
        cp_wq0.wait()
        cp_x(2).start()
        cp_x(3).start()
        wq_sc[...] = _pk(wst[0, :, 0:G])
        q_sc[0] = _pk(qproj(0))
        q_sc[1] = _pk(qproj(1))
        cp_k0a.wait()
        cp_wla.start()
        k_sc[0:KA // 2, :] = _pk(kvst[0, 0:KA, :])
        qk_rows(0, _upk(q_sc[0]), 0, KA)
        hb_group(0, qk_rows(1, _upk(q_sc[1]), 0, KA)[24:-8])
        cp_x(1).wait()
        cp_k0b.wait()
        for jj in range(4, ngrp):
            cp_x(jj).start()
        k_sc[KA // 2:Sk // 2, :] = _pk(kvst[0, KA:Sk, :])
        qk_rows(0, _upk(q_sc[0]), KA, Sk)
        qk_rows(1, _upk(q_sc[1]), KA, Sk)
        ln1_pair(1)
        q_sc[0] = _pk(qproj(2 + z_ref[0]))
        q_sc[1] = _pk(qproj(3 + z_ref[0]))

        def group(g, q0, q1, split):
            after = qk(2 * g, q0, split)
            later = qk(2 * g + 1, q1, split)
            m = after + later if split else after
            hb_group(g + z_ref[0], m[168:240])
            for n in range(3):
                nn = jnp.minimum(3 * (g - 1) + n, Dh // 8 - 1)
                wb_group(nn, wt_sc[ds(nn, 8), :], m[24 + 72 * n:96 + 72 * n])
            ln1_pair(g + 1, after[0] if split else None)
            return qproj(2 * g + 2 + z_ref[0]), qproj(2 * g + 3 + z_ref[0])

        cp_wla.wait()

        def first(j, carry):
            cp_x(2 * j + 2).wait()
            cp_x(2 * j + 3).wait()
            wt_sc[...] = wl_t(2)

            @pl.when(j == 0)
            def _():
                cp_m1.start()
                cp_wlb.start()
                cp_v0.start()
                cp_wr.start()
                start_head(1, 1)
            q0, q1 = group(2 * j + 1, _upk(q_sc[0]), _upk(q_sc[1]), False)
            q0, q1 = group(2 * j + 2, q0, q1, True)
            q_sc[0] = _pk(q0)
            q_sc[1] = _pk(q1)
            return carry
        lax.fori_loop(0, ngrp // 2 - 1, first, 0)

        cp_wr.wait()
        cp_m1.wait()
        cp_wlb.wait()
        cp_v0.wait()
        for cp in moe:
            cp.start()
        vt_sc[...] = _pk(kvst[0, Sk:2 * Sk, :].T)
        tk = qk(nblk - 2, _upk(q_sc[0]))
        qk(nblk - 1, _upk(q_sc[1]))
        hb_group(ngrp - 1, tk[32:192])
        mod_rest(tk)
        mod_finish()
        w1 = wl_t(1).astype(BF16)
        for c in range(nblk):
            ql_sc[c] = lax.dot_general(w1, _upk(h_sc[ds(c, TQ // 2), DM:D]), NT, preferred_element_type=F32)

        def main(i, carry):
            slot = i & 1
            wait_head(slot)
            wq_sc[...] = _pk(wst[slot, :, 0:G])

            @pl.when(i + 1 < Hkv)
            def _():
                start_head(i + 1, 1 - slot)

            @pl.when(i + 1 == Hkv)
            def _():
                cp_wol.start()

            k_sc[...] = _pk(kvst[slot, 0:Sk, :])
            wot_sc[...] = _pk(wst[slot, :, G:2 * G])
            rest = [ql_sc[c].T for c in range(nblk)]
            wt = wl_t(jnp.minimum(i + 2, Hkv - 1))
            work = [(n, j, k0) for n in range(Dh // 8) for j in range(nblk // NC) for k0 in range(0, DL, KS)]
            per = -(-len(work) // (nblk - 1))
            accs, built = None, 0
            q = qproj(0, rest[0])
            for c in range(nblk):
                end = c == nblk - 1
                o = pv(c)
                qn = None if end else qproj(c + 1, rest[c + 1])
                tk = qk(c, q, split=end)
                done = work[per * c][0] if per * c < len(work) else Dh // 8
                free = tk[len(tk) // 3:len(tk) - 16]
                for n in range(built, done):
                    w_ = len(free) // (done - built)
                    wb_group(n, wt[8 * n:8 * n + 8, :], free[(n - built) * w_:(n - built + 1) * w_])
                built = max(built, done)
                tw = [t for t in tk[:TICKS[1]] for _ in range(TICKS[0])] + tk[TICKS[1]:TICKS[2]]
                todo = work[per * c:per * (c + 1)]
                for idx, (n, j, k0) in enumerate(todo):
                    if k0 == 0:
                        accs = [None] * NC
                    w = wb_sc[n, 8 * k0:8 * (k0 + KS), :]
                    w = jnp.concatenate([tie(w[0:8], tw[idx * len(tw) // per]), w[8:]], axis=0)
                    ps = [w * hb_sc[j * NC + u, 8 * k0:8 * (k0 + KS), :] for u in range(NC)]
                    for r in range(0, 8 * KS, 8):
                        for u in range(NC):
                            p = ps[u][r:r + 8]
                            accs[u] = p if accs[u] is None else accs[u] + p
                    if k0 + KS == DL:
                        for u in range(NC):
                            ql_sc[j * NC + u, 8 * n:8 * n + 8, :] = accs[u]
                oproj(c, o, split=end)
                q = qn
            vt_sc[...] = _pk(kvst[slot, Sk:2 * Sk, :].T)
            modt_sc[ds(i & 3, D), :] = jnp.broadcast_to(mod_sc[pl.ds(8 + (i & 3), 1), :], (128, D)).T
            wd_sc[ds(jnp.minimum(i - 1, NF - 1), FW // 2), :] = _pk(wst[slot, :, 2 * G:2 * G + FW].T)
            return carry
        lax.fori_loop(1, Hkv, main, 0)

    @pl.when(pl.program_id(0) == 1)
    def _():
        cp_wol.wait()
        wot_sc[...] = _pk(wst[Hkv % 2, :, G:2 * G])

        def last(j, carry):
            ticks = []
            o = _upk(o_sc[...])
            for u in range(LU):
                c = LU * j + u - 1
                if u == 0:
                    oproj(jnp.maximum(c, 0), o, slot=u)
                    o0 = pv_cols(c + 1, slice(0, TQ), ticks)
                else:
                    o0 = pv_cols(c + 1, slice(0, TQ), ticks)
                    if u == 2:
                        post(LU * jnp.maximum(j - 1, 0) + 2, x1b_sc, ticks[8:48])
                    oproj(c, o, slot=u)
                o1 = pv_cols(c + 1, slice(TQ, 2 * TQ), ticks)
                o = jnp.concatenate([o0, o1], axis=0).astype(BF16)
            post(LU * j, x1a_sc, ticks[68:104], fresh=True)
            o_sc[...] = _pk(o)
            return carry
        lax.fori_loop(0, nblk // LU, last, 0)

        oproj(nblk - 1, _upk(o_sc[...]), split=True, slot=LU)

        r = _rb(st_sc[2]) + 0.0
        b16 = pltpu.bitcast(r, U32) >> 16
        ordk = jnp.where(b16 >= 0x8000, 0xFFFF - b16, b16 + 0x8000)
        tok = lax.broadcasted_iota(U32, r.shape, 0) * TQ + lax.broadcasted_iota(U32, r.shape, 1)
        key = pltpu.bitcast((ordk << 11) + (S - 1 - tok) + KEY_BIAS, F32)

        def rank(row, col):
            return _red0(jnp.where(col > row, 1.0, 0.0), jnp.add, jnp.sum, 16)

        lm = jnp.max(key, axis=0, keepdims=True)
        lrank = rank(lm, jnp.broadcast_to(lm, (TQ, TQ)).T)
        cand = jnp.concatenate([jnp.where(lrank == float(t), key, 0.0) for t in range(TOPC)], axis=0)
        cand = jnp.broadcast_to(jnp.max(cand, axis=1, keepdims=True), (TOPC * nblk, TQ))
        eye = lax.broadcasted_iota(I32, cand.shape, 0) == lax.broadcasted_iota(I32, cand.shape, 1)
        crow = _red0(jnp.where(eye, cand, 0.0), jnp.maximum, jnp.max, 16)
        crank = rank(crow, cand)
        subf = lax.broadcasted_iota(I32, (TOPC, TQ), 0).astype(F32)
        top = jnp.max(jnp.where(crank == subf, crow, 0.0), axis=1, keepdims=True)
        top = jnp.broadcast_to(top, (TOPC, TQ))
        mus = jnp.zeros((TOPC, TQ), F32)
        invs = jnp.zeros((TOPC, TQ), F32)
        for cc in range(nblk):
            sel = key[cc:cc + 1, :] == top
            mus = jnp.where(sel, st_sc[0, cc:cc + 1, :], mus)
            invs = jnp.where(sel, st_sc[1, cc:cc + 1, :], invs)
        ch, cw = [], []
        post(nblk - 2, x1b_sc, ch=ch, cw=cw)
        post(nblk, x1c_sc, ch=ch, cw=cw)
        topi = S - 1 - (pltpu.bitcast(top, I32) & (S - 1))
        rowi = ((((topi >> LG) + 1) >> 1) << LG) + (topi & (TQ - 1))
        for t in range(TOPC):
            xs_sc[t:t + 1, :] = w_sc[pl.ds(jnp.clip(rowi[t, 0], 0, w_sc.shape[0] - 1), 1), :]
        idxs = [jnp.clip(topi[t, 0], 0, S - 1) for t in range(TOPC)]
        blks = [ix >> LG for ix in idxs]
        hmask = 0
        for t in range(TOPC):
            hmask = hmask | (1 << blks[t])
        clean = [((hmask >> b) & 1) == 0 for b in range(nblk)]
        for b in range(nblk):
            @pl.when(clean[b])
            def _():
                cp_out(b).start()
        ordt = (pltpu.bitcast(top, U32) - KEY_BIAS) >> 11
        rsel = pltpu.bitcast(jnp.where(ordt >= 0x8000, ordt - 0x8000, 0xFFFF - ordt) << 16, F32)[:, 0:1]
        mus = jnp.sum(mus, axis=1, keepdims=True)
        invs = jnp.sum(invs, axis=1, keepdims=True)
        words = pltpu.bitcast(xs_sc[...], U32)
        low = ((topi[:, 0:1] >> LG) & 1) == 0
        x1s = pltpu.bitcast(jnp.where(low, words << 16, words & jnp.uint32(0xFFFF0000)), F32)
        h2s = _rb(_rb(_rb(_rb(x1s - mus) * invs) * mod_sc[4:5, :]) + mod_sc[3:4, :])
        xsel = h2s.astype(BF16)

        for cp in moe:
            cp.wait()
        FH = wg_sc.shape[1] // 2

        def glu(i, carry):
            gt = _rb(jnp.dot(xsel, wg_sc[:, ds(i, FH)], preferred_element_type=F32))
            ut = _rb(jnp.dot(xsel, wu_sc[:, ds(i, FH)], preferred_element_type=F32))
            af_sc[:, ds(i, FH)] = _rb(gt * jax.nn.sigmoid(gt)) * ut
            return carry
        lax.fori_loop(0, 2, glu, 0)
        af = af_sc[...]
        gate = _rb(jax.nn.sigmoid(rsel))
        lns = [ix & (TQ - 1) for ix in idxs]
        color, lead = [], []
        for t in range(TOPC):
            cl, dup = 0, False
            for s_ in range(t):
                cl = cl + (lns[s_] == lns[t]).astype(I32)
                dup = jnp.logical_or(dup, blks[s_] == blks[t])
            color.append(cl)
            lead.append(jnp.logical_not(dup))
        cmax = color[TOPC - 1]
        for t in range(1, TOPC - 1):
            cmax = jnp.maximum(cmax, color[t])

        def cp_fix(t, f0, fw):
            return pltpu.make_async_copy(out_sc.at[blks[t] + 1, f0:f0 + fw, :],
                                         out_hbm.at[f0:f0 + fw, ds(blks[t], TQ)], osem.at[0])

        def merge(blk, ln, f0, fw, val):
            cur = out_sc[blk + 1, f0:f0 + fw, :].astype(F32)
            lane = lax.broadcasted_iota(I32, (fw, TQ), 1)
            out_sc[blk + 1, f0:f0 + fw, :] = jnp.where(lane == ln, val, cur).astype(BF16)

        def scatter(n, f0, fw, new):
            now = [(color[t] >> 1) == 0 for t in range(TOPC)]
            for t in range(TOPC):
                row = jnp.where(now[t], lns[t] + (color[t] & 1) * TQ, 2 * TQ)
                u_sc[n, pl.ds(row, 1), 0:fw] = new[t:t + 1, :]
            ut_ = u_sc[n, 0:2 * TQ, 0:fw].T
            for t in range(TOPC):
                val = ut_[:, :TQ] if t == 0 else jnp.where((color[t] & 1) == 0, ut_[:, :TQ], ut_[:, TQ:])
                merge(blks[t], jnp.where(now[t], lns[t], TQ), f0, fw, val)

        kb = (af.shape[1] // 128) * 8 // 9 * 128
        fence, news = [], []
        for n, f0, fw in ftiles:
            an = af
            if n >= 2:
                an = jnp.concatenate([af[:, :kb], tie(af[:, kb:kb + 128], fence[n - 2]), af[:, kb + 128:]],
                                     axis=1)
            y = _rb(jnp.dot(an.astype(BF16), _upk(wd_sc[:, f0:f0 + fw]), preferred_element_type=F32))
            y = _rb(y * gate)
            new = x1s[:, f0:f0 + fw] + mod_sc[2:3, f0:f0 + fw] * _rb(h2s[:, f0:f0 + fw] + y)
            news.append(new)
            scatter(n, f0, fw, new)
            fence.append(_pk(out_sc[z_ref[0], 0:16, :]))
            for t in range(TOPC):
                @pl.when(lead[t])
                def _():
                    cp_fix(t, f0, fw).start()
        xs_sc[...] = jnp.concatenate(news, axis=1)

        pltpu.make_async_copy(out_hbm, out_hbm, osem.at[0]).wait()

        @pl.when(cmax >= 2)
        def _():
            for t in range(TOPC):
                ix_ref[t] = idxs[t]

            def redo(t, carry):
                ln = ix_ref[t] & (TQ - 1)
                row = xs_sc[pl.ds(t, 1), :]
                for n, f0, fw in ftiles:
                    u_sc[n, pl.ds(ln, 1), 0:fw] = row[:, f0:f0 + fw]
                    merge(ix_ref[t] >> LG, ln, f0, fw, u_sc[n, 0:TQ, 0:fw].T)
                return carry
            lax.fori_loop(2, TOPC, redo, 0)
            for t in range(TOPC):
                @pl.when(lead[t])
                def _():
                    cp_fix(t, 0, D).start()
            for t in range(TOPC):
                @pl.when(lead[t])
                def _():
                    cp_fix(t, 0, D).wait()


@jax.jit
def pallas_adaLN_cond__gqa_block_cached__moe_arch_mod__prompt_kernel(
    A_x: jax.Array,
    A_k_cache: jax.Array,
    A_v_cache: jax.Array,
    A_wq: jax.Array,
    A_wo: jax.Array,
    B_x: jax.Array,
    B_w_r: jax.Array,
    B_w_gate: jax.Array,
    B_w_up: jax.Array,
    B_w_down: jax.Array,
    c: jax.Array,
    w_mod: jax.Array,
):
    del B_x
    B, S, D = A_x.shape
    _, Hkv, Sk, Dh = A_k_cache.shape
    G = A_wq.shape[1] // Hkv
    Fd = B_w_gate.shape[1]
    nblk = S // TQ
    assert B == 1 and G == 2 * Dh and TOPC * nblk == TQ and Fd % FW == 0 and Fd // FW < Hkv
    assert pl.cdiv(D, 128) == LU + 1 and (2 * D) % 128 == 0 and 6 * 128 < 2 * D and (4 * D) % (MT * 128) == 0
    assert Hkv >= 5 and Sk == S and (D % 128) % KS == 0 and D % 128 > 0
    hbm = pl.BlockSpec(memory_space=pl.ANY)
    out_t = pl.pallas_call(
        _kernel,
        grid=(2,),
        in_specs=[hbm] * 11,
        out_specs=hbm,
        out_shape=jax.ShapeDtypeStruct((D, S), BF16),
        scratch_shapes=[
            pltpu.VMEM((D, S), BF16),
            pltpu.VMEM((D, 6 * D), BF16),
            pltpu.VMEM((2, 2 * Sk, Dh), BF16),
            pltpu.VMEM((2, D, 2 * G + FW), BF16),
            pltpu.VMEM((Sk // 2, Dh), U32),
            pltpu.VMEM((Dh // 2, Sk), U32),
            pltpu.VMEM((D // 2, G), U32),
            pltpu.VMEM((D // 2, G), U32),
            pltpu.VMEM((S // 2, D), U32),
            pltpu.VMEM((2, TQ, Dh), U32),
            pltpu.VMEM((nblk, Sk + 8, 2 * TQ), F32),
            pltpu.VMEM((nblk, D, TQ), F32),
            pltpu.VMEM((16, D), F32),
            pltpu.VMEM((4 * D, 128), F32),
            pltpu.VMEM((S // 2 + TQ, D), F32),
            pltpu.VMEM((nblk + 1, D, TQ), BF16),
            pltpu.VMEM((2, D + 16, TQ), F32),
            pltpu.VMEM((2, D + 16, TQ), F32),
            pltpu.VMEM((1, D + 16, TQ), F32),
            pltpu.VMEM((TOPC, D), F32),
            pltpu.VMEM((3, nblk, TQ), F32),
            pltpu.VMEM((8, 128), U32),
            pltpu.SMEM((1,), I32),
            pltpu.SMEM((TOPC,), I32),
            pltpu.VMEM((Dh, TQ), U32),
            pltpu.VMEM((1, D), BF16),
            pltpu.VMEM((D,), BF16),
            pltpu.VMEM((8, 6 * D), F32),
            pltpu.VMEM((D, Fd), BF16),
            pltpu.VMEM((D, Fd), BF16),
            pltpu.VMEM((Fd // 2, D), U32),
            pltpu.VMEM((pl.cdiv(D, 128), 2 * TQ + 8, 128), F32),
            pltpu.VMEM((D % 128, A_wq.shape[1]), BF16),
            pltpu.VMEM((nblk, (D % 128) * 8, TQ), F32),
            pltpu.VMEM((Dh // 8, (D % 128) * 8, 128), F32),
            pltpu.VMEM((nblk, Dh, TQ), F32),
            pltpu.VMEM((Dh, D % 128), F32),
            pltpu.VMEM((TOPC, Fd), F32),
            pltpu.VMEM((D, 128), F32),
            pltpu.SemaphoreType.DMA((14,)),
            pltpu.SemaphoreType.DMA((nblk // 2,)),
            pltpu.SemaphoreType.DMA((2,)),
            pltpu.SemaphoreType.DMA((1,)),
        ],
        compiler_params=pltpu.CompilerParams(dimension_semantics=("arbitrary",),
                                             vmem_limit_bytes=110 * 1024 * 1024,
                                             disable_bounds_checks=True,
                                             disable_semaphore_checks=True),
    )(c, B_w_r, A_x.reshape(S, D).T, A_k_cache.reshape(Hkv, Sk, Dh), A_v_cache.reshape(Hkv, Sk, Dh),
      A_wq, A_wo.T, w_mod, B_w_gate, B_w_up, B_w_down.T)
    return out_t.T.reshape(B, S, D)
```

```python
import math

import jax
import jax.numpy as jnp
from jax import lax
import jax.experimental.pallas as pl
import jax.experimental.pallas.tpu as pltpu

F32 = jnp.float32
BF16 = jnp.bfloat16
U32 = jnp.uint32
I32 = jnp.int32
EPS = 1e-05
TOPC = 8
NT = (((1,), (1,)), ((), ()))
TQ = 128
LG = 7
LU = 4
FW = 3 * 128
MT = 3
KEY_BIAS = 0x20000000
KS = 8
NC = 2
TICKS = (2, 72, 224)


def _pk(x):
    return pltpu.bitcast(x, U32)


def _upk(x):
    return pltpu.bitcast(x, BF16)


def _rb(x):
    return x.astype(BF16).astype(F32)


def _tree(xs, op):
    while len(xs) > 1:
        xs = [op(xs[i], xs[i + 1]) if i + 1 < len(xs) else xs[i] for i in range(0, len(xs), 2)]
    return xs[0]


def _red0(x, op, red, grp):
    n = x.shape[0]
    acc = None
    for t in range(0, n, 8 * grp):
        part = _tree([x[j:j + 8, :] for j in range(t, min(t + 8 * grp, n), 8)], op)
        acc = part if acc is None else op(acc, part)
    return red(acc, axis=0, keepdims=True)


def _ln_finish(piv, s1, s2):
    var = jnp.maximum(s2 - s1 * s1, 0.0)
    return _rb(piv + s1), 1.0 / _rb(jnp.sqrt(_rb(_rb(var) + EPS)))


def _stats_t(x, w=None):
    d = x.shape[0]
    piv = x[0:1, :]
    xd = x - piv
    s1 = _red0(xd, jnp.add, jnp.sum, 8) * (1.0 / d)
    s2 = _red0(xd * xd, jnp.add, jnp.sum, 8) * (1.0 / d)
    mu, inv = _ln_finish(piv, s1, s2)
    if w is None:
        return mu, inv
    return mu, inv, _red0(xd * w, jnp.add, jnp.sum, 8), piv


def _kernel(c_hbm, wr_hbm, xt_hbm, k_hbm, v_hbm, wq_hbm, wot_hbm, wmod_hbm,
            wg_hbm, wu_hbm, wdt_hbm, out_hbm,
            x_sc, wmod_sc, kvst, wst, k_sc, vt_sc, wq_sc, wot_sc,
            h_sc, q_sc, s_sc, acc_sc, mod_sc, modt_sc, w_sc, out_sc, x1a_sc, x1b_sc, x1c_sc, xs_sc, st_sc,
            zv_sc, z_ref, ix_ref, o_sc, c_sc, wr_sc, mrow_sc, wg_sc, wu_sc, wd_sc, u_sc,
            wl_sc, hb_sc, wb_sc, ql_sc, wt_sc, af_sc, sct_sc,
            sems, xsems, lsems, osem):
    D, S = x_sc.shape
    Hkv, Sk, Dh = k_hbm.shape
    G = 2 * Dh
    nblk = S // TQ
    ngrp = nblk // 2
    GW = 2 * TQ
    NF = wdt_hbm.shape[1] // FW
    qscale = (Dh ** -0.5) * math.log2(math.e)
    ftiles = [(n, f0, min(128, D - f0)) for n, f0 in enumerate(range(0, D, 128))]

    def ds(i, n):
        return slice(i * n, (i + 1) * n) if isinstance(i, int) else pl.ds(pl.multiple_of(i * n, n), n)

    def cp_k(g, slot, sem):
        return pltpu.make_async_copy(k_hbm.at[g], kvst.at[slot, 0:Sk, :], sem)

    def cp_v(g, slot, sem):
        return pltpu.make_async_copy(v_hbm.at[g], kvst.at[slot, Sk:2 * Sk, :], sem)

    def cp_wq(g, slot, sem):
        return pltpu.make_async_copy(wq_hbm.at[:, ds(g, G)], wst.at[slot, :, 0:G], sem)

    def cp_wo(g, slot, sem):
        return pltpu.make_async_copy(wot_hbm.at[:, ds(g, G)], wst.at[slot, :, G:2 * G], sem)

    def start_head(i, slot):
        cp_wq(i, slot, lsems.at[0]).start()
        cp_wo(i - 1, slot, lsems.at[0]).start()
        pltpu.make_async_copy(wdt_hbm.at[:, ds(jnp.minimum(i - 1, NF - 1), FW)],
                              wst.at[slot, :, 2 * G:2 * G + FW], lsems.at[0]).start()
        cp_k(i, slot, lsems.at[1]).start()
        cp_v(i, slot, lsems.at[1]).start()

    def wait_head(slot):
        pltpu.make_async_copy(wst.at[slot], wst.at[slot], lsems.at[0]).wait()
        pltpu.make_async_copy(kvst.at[slot], kvst.at[slot], lsems.at[1]).wait()

    def cp_x(j):
        return pltpu.make_async_copy(xt_hbm.at[:, ds(j, GW)], x_sc.at[:, ds(j, GW)], xsems.at[j])

    def cp_out(b):
        return pltpu.make_async_copy(out_sc.at[b + 1], out_hbm.at[:, ds(b, TQ)], osem.at[0])

    moe = [pltpu.make_async_copy(wg_hbm, wg_sc, sems.at[0]),
           pltpu.make_async_copy(wu_hbm, wu_sc, sems.at[1])]
    MA = 6 * 128
    cp_m0a = pltpu.make_async_copy(wmod_hbm.at[:, 0:MA], wmod_sc.at[:, 0:MA], sems.at[2])
    cp_m0b = pltpu.make_async_copy(wmod_hbm.at[:, MA:2 * D], wmod_sc.at[:, MA:2 * D], sems.at[11])
    cp_m1 = pltpu.make_async_copy(wmod_hbm.at[:, 2 * D:6 * D], wmod_sc.at[:, 2 * D:6 * D], sems.at[3])
    cp_c = pltpu.make_async_copy(c_hbm, c_sc, sems.at[4])
    cp_wr = pltpu.make_async_copy(wr_hbm, wr_sc, sems.at[5])
    cp_v0 = cp_v(0, 0, sems.at[6])
    KA = 3 * Sk // 8
    cp_k0a = pltpu.make_async_copy(k_hbm.at[0, 0:KA, :], kvst.at[0, 0:KA, :], sems.at[7])
    cp_k0b = pltpu.make_async_copy(k_hbm.at[0, KA:Sk, :], kvst.at[0, KA:Sk, :], sems.at[10])
    cp_wq0 = cp_wq(0, 0, sems.at[8])
    cp_wol = cp_wo(Hkv - 1, Hkv % 2, sems.at[9])
    DM = D // 128 * 128
    DL = D - DM
    cp_wla = pltpu.make_async_copy(wq_hbm.at[DM:D, G:3 * G], wl_sc.at[:, G:3 * G], sems.at[12])
    cp_wlb = pltpu.make_async_copy(wq_hbm.at[DM:D, 3 * G:], wl_sc.at[:, 3 * G:], sems.at[13])

    def tie(v, dep):
        return pltpu.bitcast(pltpu.bitcast(v, U32) | (dep & zv_sc[:, 0:dep.shape[1]]), v.dtype)

    def ln1_pair(g, after=None):
        piv = jnp.broadcast_to(x_sc[0:16, ds(g, GW)].astype(F32)[0:1], (8, GW))
        if after is not None:
            piv = jnp.concatenate([tie(piv[:, :TQ], after), tie(piv[:, TQ:], after)], axis=1)
        s1 = s2 = None
        for r0 in range(0, D, 16):
            pw = piv
            if s2 is not None:
                b2 = pltpu.bitcast(s2, U32)
                pw = jnp.concatenate([tie(piv[:, :TQ], b2[:, :TQ]), tie(piv[:, TQ:], b2[:, TQ:])], axis=1)
            xd = x_sc[r0:r0 + 16, ds(g, GW)].astype(F32) - jnp.concatenate([pw, pw], axis=0)
            xq = xd * xd
            p1 = xd[0:8] + xd[8:16]
            p2 = xq[0:8] + xq[8:16]
            s1 = p1 if s1 is None else s1 + p1
            s2 = p2 if s2 is None else s2 + p2
        mu, inv = _ln_finish(piv, jnp.sum(s1, axis=0, keepdims=True) * (1.0 / D),
                             jnp.sum(s2, axis=0, keepdims=True) * (1.0 / D))
        g2 = g + z_ref[0]
        for _, f0, fw in ftiles:
            x = x_sc[f0:f0 + fw, ds(g2, GW)].astype(F32)
            n = (x - jnp.concatenate([mu] * (fw // 8), axis=0)) * inv
            h = n.T * mod_sc[1:2, f0:f0 + fw] + mod_sc[0:1, f0:f0 + fw]
            h_sc[ds(g, TQ), f0:f0 + fw] = _pk(h.astype(BF16))

    def mod_rest(ticks):
        total = (4 * D // (MT * 128)) * (D // 16)
        i = 0
        for c0 in range(2 * D, 6 * D, MT * 128):
            acc = None
            for r0 in range(0, D, 16):
                sc = sct_sc[r0:r0 + 16, :]
                sc = jnp.concatenate([tie(sc[0:8], ticks[i * len(ticks) // total]), sc[8:16]], axis=0)
                i += 1
                pr = wmod_sc[r0:r0 + 16, c0:c0 + MT * 128].astype(F32) * jnp.concatenate([sc] * MT, axis=1)
                acc = pr[0:8] if acc is None else acc + pr[0:8]
                acc = acc + pr[8:16]
            mrow_sc[:, c0:c0 + MT * 128] = acc

    def mod_finish():
        m = _rb(jnp.sum(mrow_sc[:, 2 * D:6 * D], axis=0, keepdims=True))
        ga = m[0:1, 0:D]
        sb = m[0:1, D:2 * D]
        cb1 = _rb(1.0 + m[0:1, 2 * D:3 * D])
        gb = m[0:1, 3 * D:4 * D]
        wr = wr_sc[...].astype(F32).reshape(1, D)
        mod_sc[2:3, :] = gb
        mod_sc[3:4, :] = sb
        mod_sc[4:5, :] = cb1
        mod_sc[5:6, :] = jnp.broadcast_to(jnp.sum(wr * cb1, axis=1, keepdims=True), (1, D))
        mod_sc[6:7, :] = jnp.broadcast_to(jnp.sum(wr * sb, axis=1, keepdims=True), (1, D))
        for i, vec in enumerate((ga, gb * cb1, gb * sb, wr * cb1)):
            mod_sc[8 + i:9 + i, :] = vec

    def qproj(c, rest=None):
        h = _upk(h_sc[ds(c, TQ // 2), :])
        if rest is None:
            q = jnp.dot(h, _upk(wq_sc[...]), preferred_element_type=F32)
            q = (q * qscale).astype(BF16)
            return jnp.concatenate([q[:, :Dh], q[:, Dh:]], axis=0)
        qb = jnp.dot(h[:, 0:DM], _upk(wq_sc[0:DM // 2, Dh:G]), preferred_element_type=F32) + rest
        qa = jnp.dot(h, _upk(wq_sc[:, 0:Dh]), preferred_element_type=F32)
        return (jnp.concatenate([qa, qb], axis=0) * qscale).astype(BF16)

    def wl_t(g):
        return wl_sc[:, ds(2 * g + 1, Dh)].astype(F32).T

    def hb_group(g, ticks):
        ht = _upk(h_sc[ds(g, TQ), DM:D]).astype(F32).T
        for u in range(2):
            for k0 in range(0, DL, 8):
                h8 = tie(ht[k0:k0 + 8, u * TQ:(u + 1) * TQ], ticks[(u * DL + k0) * len(ticks) // (2 * DL)])
                hb_sc[2 * g + u, 8 * k0:8 * k0 + 64, :] = jnp.concatenate(
                    [jnp.broadcast_to(h8[k:k + 1], (8, TQ)) for k in range(8)], axis=0)

    def wb_group(n, wt, ticks):
        for k0 in range(0, DL, 4):
            w = tie(wt, ticks[k0 * len(ticks) // DL][:, 0:DL])
            wb_sc[n, 8 * k0:8 * k0 + 32, :] = jnp.concatenate(
                [jnp.broadcast_to(w[:, k:k + 1], (8, 128)) for k in range(k0, k0 + 4)], axis=0)

    def marks(st):
        return [pltpu.bitcast(st[r:r + 8, 0:128], U32) for r in range(0, st.shape[0], 8)]

    def qk(c, q, split=False):
        if split:
            st = jnp.concatenate([
                lax.dot_general(_upk(k_sc[ds(j, Sk // 4), :]), q, NT, preferred_element_type=F32)
                for j in range(2)], axis=0)
        else:
            st = lax.dot_general(_upk(k_sc[...]), q, NT, preferred_element_type=F32)
        s_sc[c, 0:Sk, :] = st
        s_sc[c, Sk:Sk + 8, :] = jnp.broadcast_to(_red0(st, jnp.maximum, jnp.max, 1), (8, 2 * TQ))
        return marks(st[0:Sk // 2] if split else st)

    def qk_rows(c, q, r0, r1):
        st = lax.dot_general(_upk(k_sc[r0 // 2:r1 // 2, :]), q, NT, preferred_element_type=F32)
        s_sc[c, r0:r1, :] = st
        m = jnp.broadcast_to(_red0(st, jnp.maximum, jnp.max, 1), (8, 2 * TQ))
        s_sc[c, Sk:Sk + 8, :] = m if r0 == 0 else jnp.maximum(m, s_sc[c, Sk:Sk + 8, :])
        return marks(st)

    def pv_cols(c, cols, ticks=None):
        p = jnp.exp2(s_sc[c, 0:Sk, cols] - s_sc[c, Sk:Sk + 1, cols])
        l = _red0(p, jnp.add, jnp.sum, 2)
        if ticks is None:
            ot = jnp.dot(_upk(vt_sc[...]), p.astype(BF16), preferred_element_type=F32)
        else:
            ot = None
            for r in range(0, Sk, Sk // 4):
                d = jnp.dot(_upk(vt_sc[:, r:r + Sk // 4]), p[r:r + Sk // 4].astype(BF16),
                            preferred_element_type=F32)
                ticks.extend(pltpu.bitcast(d[i:i + 8, 0:128], U32) for i in range(0, Dh, Dh // 4))
                ot = d if ot is None else ot + d
        return ot * (1.0 / l)

    def pv(c):
        ot = pv_cols(c, slice(0, 2 * TQ)).astype(BF16)
        return jnp.concatenate([ot[:, :TQ], ot[:, TQ:]], axis=0)

    def oproj(c, o2t, split=False, slot=None):
        if split:
            d = jnp.concatenate([
                jnp.dot(_upk(wot_sc[ds(j, D // 4), :]), o2t, preferred_element_type=F32)
                for j in range(2)], axis=0)
        else:
            d = jnp.dot(_upk(wot_sc[...]), o2t, preferred_element_type=F32)
        if slot is None:
            acc_sc[c] += d
        else:
            x1 = _rb(x_sc[:, ds(c, TQ)].astype(F32) + modt_sc[0:D, :] * (acc_sc[c] + d))
            xb = (x1a_sc, x1b_sc, x1c_sc)[slot // 2].at[slot % 2]
            xb[0:D, :] = x1
            mu, inv, rw, piv = _stats_t(x1, modt_sc[3 * D:4 * D, :])
            xb[D:D + 8, :] = jnp.broadcast_to(mu, (8, TQ))
            xb[D + 8:D + 16, :] = jnp.broadcast_to(inv, (8, TQ))
            st_sc[0, pl.ds(c, 1), :] = mu
            st_sc[1, pl.ds(c, 1), :] = inv
            st_sc[2, pl.ds(c, 1), :] = (rw - (mu - piv) * mod_sc[5:6, 0:TQ]) * inv + mod_sc[6:7, 0:TQ]

    def post(v0, xb, ticks=None, ch=None, cw=None, fresh=False):
        slots = [u + z_ref[0] if fresh else u for u in range(xb.shape[0])]
        mu0 = [xb[u, D:D + 8, :] for u in slots]
        inv0 = [xb[u, D + 8:D + 16, :] for u in slots]
        for _, f0, fw in ftiles:
            words = []
            for r0 in range(f0, f0 + fw, 32):
                gc = modt_sc[D + r0:D + r0 + 32, :]
                gs = modt_sc[2 * D + r0:2 * D + r0 + 32, :]
                if ticks is not None:
                    dep = ticks[r0 * len(ticks) // D]
                else:
                    dep = ch[-2] if len(ch) >= 2 else None
                    if r0 == f0 and len(cw) >= 3:
                        dep = dep | cw[-3]
                xs = []
                for u in range(len(slots)):
                    x1 = xb[slots[u], r0:r0 + 32, :]
                    xs.append(x1)
                    mu = mu0[u] if dep is None else tie(mu0[u], dep)
                    mu = jnp.concatenate([mu] * 4, axis=0)
                    inv = jnp.concatenate([inv0[u]] * 4, axis=0)
                    o = x1 + ((x1 - mu) * inv * gc + gs)
                    out_sc[v0 + u, r0:r0 + 32, :] = o.astype(BF16)
                wd = pltpu.bitcast(xs[0], U32)
                if ticks is not None:
                    wd = jnp.concatenate([tie(wd[0:8], dep), wd[8:]], axis=0)
                if len(xs) > 1:
                    wd = wd | (pltpu.bitcast(xs[1], U32) >> 16)
                words.append(wd)
                if ticks is None:
                    ch.append(_pk(out_sc[z_ref[0], 0:16, :]))
            w_sc[ds(v0 // 2, TQ), f0:f0 + fw] = pltpu.bitcast(jnp.concatenate(words, axis=0), F32).T
            if ticks is None:
                cw.append(pltpu.bitcast(w_sc[pl.ds(pl.multiple_of(z_ref[0], 8), 8), 0:128], U32))

    @pl.when(pl.program_id(0) == 0)
    def _():
        for cp in (cp_c, cp_x(0), cp_m0a):
            cp.start()

        def zero(i, carry):
            acc_sc[i] = jnp.zeros(acc_sc.shape[1:], F32)
            return carry
        lax.fori_loop(0, nblk, zero, 0)
        cp_m0b.start()

        def zero2(i, carry):
            x1b_sc[i & 1] = jnp.zeros(x1b_sc.shape[1:], F32)
            u_sc[i] = jnp.zeros(u_sc.shape[1:], F32)
            return carry
        lax.fori_loop(0, LU + 1, zero2, 0)
        o_sc[...] = jnp.zeros(o_sc.shape, U32)
        st_sc[...] = jnp.zeros(st_sc.shape, F32)
        zv_sc[...] = jnp.zeros(zv_sc.shape, U32)
        z_ref[0] = 0
        cp_c.wait()
        cp_wq0.start()
        cp_x(0).wait()
        cp_k0a.start()
        c = c_sc[...].astype(F32)
        scb = (c * jax.nn.sigmoid(c)).astype(BF16)
        sct_sc[...] = jnp.broadcast_to(scb.astype(F32), (128, D)).T

        def norm0(cc, carry):
            x = x_sc[:, ds(cc, TQ)].astype(F32)
            mu, inv = _stats_t(x)
            w_sc[ds(cc, TQ), :] = ((x - mu) * inv).T
            return carry
        lax.fori_loop(0, 2, norm0, 0)
        sc8 = jnp.broadcast_to(scb, (8, D))
        cp_m0a.wait()
        cp_x(1).start()
        mrow_sc[:, 0:MA] = jnp.dot(sc8, wmod_sc[:, 0:MA], preferred_element_type=F32)
        cp_m0b.wait()
        cp_k0b.start()
        mrow_sc[:, MA:2 * D] = jnp.dot(sc8, wmod_sc[:, MA:2 * D], preferred_element_type=F32)
        m = _rb(mrow_sc[:, 0:2 * D])
        sa = m[0:1, 0:D]
        ca1 = _rb(1.0 + m[0:1, D:2 * D])
        mod_sc[0:1, :] = sa
        mod_sc[1:2, :] = ca1
        h_sc[0:TQ, :] = _pk((w_sc[0:2 * TQ, :] * ca1 + sa).astype(BF16))
        cp_wq0.wait()
        cp_x(2).start()
        cp_x(3).start()
        wq_sc[...] = _pk(wst[0, :, 0:G])
        q_sc[0] = _pk(qproj(0))
        q_sc[1] = _pk(qproj(1))
        cp_k0a.wait()
        cp_wla.start()
        k_sc[0:KA // 2, :] = _pk(kvst[0, 0:KA, :])
        qk_rows(0, _upk(q_sc[0]), 0, KA)
        hb_group(0, qk_rows(1, _upk(q_sc[1]), 0, KA)[24:-8])
        cp_x(1).wait()
        cp_k0b.wait()
        for jj in range(4, ngrp):
            cp_x(jj).start()
        k_sc[KA // 2:Sk // 2, :] = _pk(kvst[0, KA:Sk, :])
        qk_rows(0, _upk(q_sc[0]), KA, Sk)
        qk_rows(1, _upk(q_sc[1]), KA, Sk)
        ln1_pair(1)
        q_sc[0] = _pk(qproj(2 + z_ref[0]))
        q_sc[1] = _pk(qproj(3 + z_ref[0]))

        def group(g, q0, q1, split):
            after = qk(2 * g, q0, split)
            later = qk(2 * g + 1, q1, split)
            m = after + later if split else after
            hb_group(g + z_ref[0], m[200:254])
            for n in range(2):
                nn = 2 * (g - 1) + n
                wb_group(nn, wt_sc[ds(nn, 8), :], m[130 + 40 * n:170 + 40 * n])
            ln1_pair(g + 1, after[0] if split else None)
            return qproj(2 * g + 2 + z_ref[0]), qproj(2 * g + 3 + z_ref[0])

        cp_wla.wait()

        def first(j, carry):
            cp_x(2 * j + 2).wait()
            cp_x(2 * j + 3).wait()
            wt_sc[...] = wl_t(2)

            @pl.when(j == 0)
            def _():
                cp_m1.start()
                cp_wlb.start()
                cp_v0.start()
                cp_wr.start()
                start_head(1, 1)
            q0, q1 = group(2 * j + 1, _upk(q_sc[0]), _upk(q_sc[1]), False)
            q0, q1 = group(2 * j + 2, q0, q1, True)
            q_sc[0] = _pk(q0)
            q_sc[1] = _pk(q1)
            return carry
        lax.fori_loop(0, ngrp // 2 - 1, first, 0)

        cp_wr.wait()
        cp_m1.wait()
        cp_wlb.wait()
        cp_v0.wait()
        for cp in moe:
            cp.start()
        vt_sc[...] = _pk(kvst[0, Sk:2 * Sk, :].T)
        tk = qk(nblk - 2, _upk(q_sc[0]))
        qk(nblk - 1, _upk(q_sc[1]))
        hb_group(ngrp - 1, tk[32:192])
        for i, n in enumerate(range(2 * (ngrp - 2), Dh // 8)):
            wb_group(n, wt_sc[ds(n, 8), :], tk[16 + 56 * i:72 + 56 * i])
        mod_rest(tk)
        mod_finish()
        w1 = wl_t(1).astype(BF16)
        for c in range(nblk):
            ql_sc[c] = lax.dot_general(w1, _upk(h_sc[ds(c, TQ // 2), DM:D]), NT, preferred_element_type=F32)

        def main(i, carry):
            slot = i & 1
            wait_head(slot)
            wq_sc[...] = _pk(wst[slot, :, 0:G])

            @pl.when(i + 1 < Hkv)
            def _():
                start_head(i + 1, 1 - slot)

            @pl.when(i + 1 == Hkv)
            def _():
                cp_wol.start()

            k_sc[...] = _pk(kvst[slot, 0:Sk, :])
            wot_sc[...] = _pk(wst[slot, :, G:2 * G])
            rest = [ql_sc[c].T for c in range(nblk)]
            wt = wl_t(jnp.minimum(i + 2, Hkv - 1))
            work = [(n, j, k0) for n in range(Dh // 8) for j in range(nblk // NC) for k0 in range(0, DL, KS)]
            per = -(-len(work) // (nblk - 1))
            accs, built = None, 0
            q = qproj(0, rest[0])
            for c in range(nblk):
                end = c == nblk - 1
                o = pv(c)
                qn = None if end else qproj(c + 1, rest[c + 1])
                tk = qk(c, q, split=end)
                done = work[per * c][0] if per * c < len(work) else Dh // 8
                free = tk[len(tk) // 3:len(tk) - 16]
                for n in range(built, done):
                    w_ = len(free) // (done - built)
                    wb_group(n, wt[8 * n:8 * n + 8, :], free[(n - built) * w_:(n - built + 1) * w_])
                built = max(built, done)
                tw = [t for t in tk[:TICKS[1]] for _ in range(TICKS[0])] + tk[TICKS[1]:TICKS[2]]
                todo = work[per * c:per * (c + 1)]
                for idx, (n, j, k0) in enumerate(todo):
                    if k0 == 0:
                        accs = [None] * NC
                    w = wb_sc[n, 8 * k0:8 * (k0 + KS), :]
                    w = jnp.concatenate([tie(w[0:8], tw[idx * len(tw) // per]), w[8:]], axis=0)
                    ps = [w * hb_sc[j * NC + u, 8 * k0:8 * (k0 + KS), :] for u in range(NC)]
                    for r in range(0, 8 * KS, 8):
                        for u in range(NC):
                            p = ps[u][r:r + 8]
                            accs[u] = p if accs[u] is None else accs[u] + p
                    if k0 + KS == DL:
                        for u in range(NC):
                            ql_sc[j * NC + u, 8 * n:8 * n + 8, :] = accs[u]
                oproj(c, o, split=end)
                q = qn
            vt_sc[...] = _pk(kvst[slot, Sk:2 * Sk, :].T)
            modt_sc[ds(i & 3, D), :] = jnp.broadcast_to(mod_sc[pl.ds(8 + (i & 3), 1), :], (128, D)).T
            wd_sc[ds(jnp.minimum(i - 1, NF - 1), FW // 2), :] = _pk(wst[slot, :, 2 * G:2 * G + FW].T)
            return carry
        lax.fori_loop(1, Hkv, main, 0)

    @pl.when(pl.program_id(0) == 1)
    def _():
        cp_wol.wait()
        wot_sc[...] = _pk(wst[Hkv % 2, :, G:2 * G])

        def last(j, carry):
            ticks = []
            o = _upk(o_sc[...])
            for u in range(LU):
                c = LU * j + u - 1
                if u == 0:
                    oproj(jnp.maximum(c, 0), o, slot=u)
                    o0 = pv_cols(c + 1, slice(0, TQ), ticks)
                else:
                    o0 = pv_cols(c + 1, slice(0, TQ), ticks)
                    if u == 2:
                        post(LU * jnp.maximum(j - 1, 0) + 2, x1b_sc, ticks[8:48])
                    oproj(c, o, slot=u)
                o1 = pv_cols(c + 1, slice(TQ, 2 * TQ), ticks)
                o = jnp.concatenate([o0, o1], axis=0).astype(BF16)
            post(LU * j, x1a_sc, ticks[68:104], fresh=True)
            o_sc[...] = _pk(o)
            return carry
        lax.fori_loop(0, nblk // LU, last, 0)

        oproj(nblk - 1, _upk(o_sc[...]), split=True, slot=LU)

        r = _rb(st_sc[2]) + 0.0
        b16 = pltpu.bitcast(r, U32) >> 16
        ordk = jnp.where(b16 >= 0x8000, 0xFFFF - b16, b16 + 0x8000)
        tok = lax.broadcasted_iota(U32, r.shape, 0) * TQ + lax.broadcasted_iota(U32, r.shape, 1)
        key = pltpu.bitcast((ordk << 11) + (S - 1 - tok) + KEY_BIAS, F32)

        def rank(row, col):
            return _red0(jnp.where(col > row, 1.0, 0.0), jnp.add, jnp.sum, 16)

        lm = jnp.max(key, axis=0, keepdims=True)
        lrank = rank(lm, jnp.broadcast_to(lm, (TQ, TQ)).T)
        cand = jnp.concatenate([jnp.where(lrank == float(t), key, 0.0) for t in range(TOPC)], axis=0)
        cand = jnp.broadcast_to(jnp.max(cand, axis=1, keepdims=True), (TOPC * nblk, TQ))
        eye = lax.broadcasted_iota(I32, cand.shape, 0) == lax.broadcasted_iota(I32, cand.shape, 1)
        crow = _red0(jnp.where(eye, cand, 0.0), jnp.maximum, jnp.max, 16)
        crank = rank(crow, cand)
        subf = lax.broadcasted_iota(I32, (TOPC, TQ), 0).astype(F32)
        top = jnp.max(jnp.where(crank == subf, crow, 0.0), axis=1, keepdims=True)
        top = jnp.broadcast_to(top, (TOPC, TQ))
        mus = jnp.zeros((TOPC, TQ), F32)
        invs = jnp.zeros((TOPC, TQ), F32)
        for cc in range(nblk):
            sel = key[cc:cc + 1, :] == top
            mus = jnp.where(sel, st_sc[0, cc:cc + 1, :], mus)
            invs = jnp.where(sel, st_sc[1, cc:cc + 1, :], invs)
        ch, cw = [], []
        post(nblk - 2, x1b_sc, ch=ch, cw=cw)
        post(nblk, x1c_sc, ch=ch, cw=cw)
        topi = S - 1 - (pltpu.bitcast(top, I32) & (S - 1))
        rowi = ((((topi >> LG) + 1) >> 1) << LG) + (topi & (TQ - 1))
        for t in range(TOPC):
            xs_sc[t:t + 1, :] = w_sc[pl.ds(jnp.clip(rowi[t, 0], 0, w_sc.shape[0] - 1), 1), :]
        idxs = [jnp.clip(topi[t, 0], 0, S - 1) for t in range(TOPC)]
        blks = [ix >> LG for ix in idxs]
        hmask = 0
        for t in range(TOPC):
            hmask = hmask | (1 << blks[t])
        clean = [((hmask >> b) & 1) == 0 for b in range(nblk)]
        for b in range(nblk):
            @pl.when(clean[b])
            def _():
                cp_out(b).start()
        ordt = (pltpu.bitcast(top, U32) - KEY_BIAS) >> 11
        rsel = pltpu.bitcast(jnp.where(ordt >= 0x8000, ordt - 0x8000, 0xFFFF - ordt) << 16, F32)[:, 0:1]
        mus = jnp.sum(mus, axis=1, keepdims=True)
        invs = jnp.sum(invs, axis=1, keepdims=True)
        words = pltpu.bitcast(xs_sc[...], U32)
        low = ((topi[:, 0:1] >> LG) & 1) == 0
        x1s = pltpu.bitcast(jnp.where(low, words << 16, words & jnp.uint32(0xFFFF0000)), F32)
        h2s = _rb(_rb(_rb(_rb(x1s - mus) * invs) * mod_sc[4:5, :]) + mod_sc[3:4, :])
        xsel = h2s.astype(BF16)

        for cp in moe:
            cp.wait()
        FH = wg_sc.shape[1] // 2

        def glu(i, carry):
            gt = _rb(jnp.dot(xsel, wg_sc[:, ds(i, FH)], preferred_element_type=F32))
            ut = _rb(jnp.dot(xsel, wu_sc[:, ds(i, FH)], preferred_element_type=F32))
            af_sc[:, ds(i, FH)] = _rb(gt * jax.nn.sigmoid(gt)) * ut
            return carry
        lax.fori_loop(0, 2, glu, 0)
        af = af_sc[...]
        gate = _rb(jax.nn.sigmoid(rsel))
        lns = [ix & (TQ - 1) for ix in idxs]
        color, lead = [], []
        for t in range(TOPC):
            cl, dup = 0, False
            for s_ in range(t):
                cl = cl + (lns[s_] == lns[t]).astype(I32)
                dup = jnp.logical_or(dup, blks[s_] == blks[t])
            color.append(cl)
            lead.append(jnp.logical_not(dup))
        cmax = color[TOPC - 1]
        for t in range(1, TOPC - 1):
            cmax = jnp.maximum(cmax, color[t])

        def cp_fix(t, f0, fw):
            return pltpu.make_async_copy(out_sc.at[blks[t] + 1, f0:f0 + fw, :],
                                         out_hbm.at[f0:f0 + fw, ds(blks[t], TQ)], osem.at[0])

        def merge(blk, ln, f0, fw, val):
            cur = out_sc[blk + 1, f0:f0 + fw, :].astype(F32)
            lane = lax.broadcasted_iota(I32, (fw, TQ), 1)
            out_sc[blk + 1, f0:f0 + fw, :] = jnp.where(lane == ln, val, cur).astype(BF16)

        def scatter(n, f0, fw, new):
            now = [(color[t] >> 1) == 0 for t in range(TOPC)]
            for t in range(TOPC):
                row = jnp.where(now[t], lns[t] + (color[t] & 1) * TQ, 2 * TQ)
                u_sc[n, pl.ds(row, 1), 0:fw] = new[t:t + 1, :]
            ut_ = u_sc[n, 0:2 * TQ, 0:fw].T
            for t in range(TOPC):
                val = ut_[:, :TQ] if t == 0 else jnp.where((color[t] & 1) == 0, ut_[:, :TQ], ut_[:, TQ:])
                merge(blks[t], jnp.where(now[t], lns[t], TQ), f0, fw, val)

        kb = (af.shape[1] // 128) * 8 // 9 * 128
        fence, news = [], []
        for n, f0, fw in ftiles:
            an = af
            if n >= 2:
                an = jnp.concatenate([af[:, :kb], tie(af[:, kb:kb + 128], fence[n - 2]), af[:, kb + 128:]],
                                     axis=1)
            y = _rb(jnp.dot(an.astype(BF16), _upk(wd_sc[:, f0:f0 + fw]), preferred_element_type=F32))
            y = _rb(y * gate)
            new = x1s[:, f0:f0 + fw] + mod_sc[2:3, f0:f0 + fw] * _rb(h2s[:, f0:f0 + fw] + y)
            news.append(new)
            scatter(n, f0, fw, new)
            fence.append(_pk(out_sc[z_ref[0], 0:16, :]))
            for t in range(TOPC):
                @pl.when(lead[t])
                def _():
                    cp_fix(t, f0, fw).start()
        xs_sc[...] = jnp.concatenate(news, axis=1)

        pltpu.make_async_copy(out_hbm, out_hbm, osem.at[0]).wait()

        @pl.when(cmax >= 2)
        def _():
            for t in range(TOPC):
                ix_ref[t] = idxs[t]

            def redo(t, carry):
                ln = ix_ref[t] & (TQ - 1)
                row = xs_sc[pl.ds(t, 1), :]
                for n, f0, fw in ftiles:
                    u_sc[n, pl.ds(ln, 1), 0:fw] = row[:, f0:f0 + fw]
                    merge(ix_ref[t] >> LG, ln, f0, fw, u_sc[n, 0:TQ, 0:fw].T)
                return carry
            lax.fori_loop(2, TOPC, redo, 0)
            for t in range(TOPC):
                @pl.when(lead[t])
                def _():
                    cp_fix(t, 0, D).start()
            for t in range(TOPC):
                @pl.when(lead[t])
                def _():
                    cp_fix(t, 0, D).wait()


@jax.jit
def pallas_adaLN_cond__gqa_block_cached__moe_arch_mod__prompt_kernel(
    A_x: jax.Array,
    A_k_cache: jax.Array,
    A_v_cache: jax.Array,
    A_wq: jax.Array,
    A_wo: jax.Array,
    B_x: jax.Array,
    B_w_r: jax.Array,
    B_w_gate: jax.Array,
    B_w_up: jax.Array,
    B_w_down: jax.Array,
    c: jax.Array,
    w_mod: jax.Array,
):
    del B_x
    B, S, D = A_x.shape
    _, Hkv, Sk, Dh = A_k_cache.shape
    G = A_wq.shape[1] // Hkv
    Fd = B_w_gate.shape[1]
    nblk = S // TQ
    assert B == 1 and G == 2 * Dh and TOPC * nblk == TQ and Fd % FW == 0 and Fd // FW < Hkv
    assert pl.cdiv(D, 128) == LU + 1 and (2 * D) % 128 == 0 and 6 * 128 < 2 * D and (4 * D) % (MT * 128) == 0
    assert Hkv >= 5 and Sk == S and (D % 128) % KS == 0 and D % 128 > 0
    hbm = pl.BlockSpec(memory_space=pl.ANY)
    out_t = pl.pallas_call(
        _kernel,
        grid=(2,),
        in_specs=[hbm] * 11,
        out_specs=hbm,
        out_shape=jax.ShapeDtypeStruct((D, S), BF16),
        scratch_shapes=[
            pltpu.VMEM((D, S), BF16),
            pltpu.VMEM((D, 6 * D), BF16),
            pltpu.VMEM((2, 2 * Sk, Dh), BF16),
            pltpu.VMEM((2, D, 2 * G + FW), BF16),
            pltpu.VMEM((Sk // 2, Dh), U32),
            pltpu.VMEM((Dh // 2, Sk), U32),
            pltpu.VMEM((D // 2, G), U32),
            pltpu.VMEM((D // 2, G), U32),
            pltpu.VMEM((S // 2, D), U32),
            pltpu.VMEM((2, TQ, Dh), U32),
            pltpu.VMEM((nblk, Sk + 8, 2 * TQ), F32),
            pltpu.VMEM((nblk, D, TQ), F32),
            pltpu.VMEM((16, D), F32),
            pltpu.VMEM((4 * D, 128), F32),
            pltpu.VMEM((S // 2 + TQ, D), F32),
            pltpu.VMEM((nblk + 1, D, TQ), BF16),
            pltpu.VMEM((2, D + 16, TQ), F32),
            pltpu.VMEM((2, D + 16, TQ), F32),
            pltpu.VMEM((1, D + 16, TQ), F32),
            pltpu.VMEM((TOPC, D), F32),
            pltpu.VMEM((3, nblk, TQ), F32),
            pltpu.VMEM((8, 128), U32),
            pltpu.SMEM((1,), I32),
            pltpu.SMEM((TOPC,), I32),
            pltpu.VMEM((Dh, TQ), U32),
            pltpu.VMEM((1, D), BF16),
            pltpu.VMEM((D,), BF16),
            pltpu.VMEM((8, 6 * D), F32),
            pltpu.VMEM((D, Fd), BF16),
            pltpu.VMEM((D, Fd), BF16),
            pltpu.VMEM((Fd // 2, D), U32),
            pltpu.VMEM((pl.cdiv(D, 128), 2 * TQ + 8, 128), F32),
            pltpu.VMEM((D % 128, A_wq.shape[1]), BF16),
            pltpu.VMEM((nblk, (D % 128) * 8, TQ), F32),
            pltpu.VMEM((Dh // 8, (D % 128) * 8, 128), F32),
            pltpu.VMEM((nblk, Dh, TQ), F32),
            pltpu.VMEM((Dh, D % 128), F32),
            pltpu.VMEM((TOPC, Fd), F32),
            pltpu.VMEM((D, 128), F32),
            pltpu.SemaphoreType.DMA((14,)),
            pltpu.SemaphoreType.DMA((nblk // 2,)),
            pltpu.SemaphoreType.DMA((2,)),
            pltpu.SemaphoreType.DMA((1,)),
        ],
        compiler_params=pltpu.CompilerParams(dimension_semantics=("arbitrary",),
                                             vmem_limit_bytes=110 * 1024 * 1024,
                                             disable_bounds_checks=True,
                                             disable_semaphore_checks=True),
    )(c, B_w_r, A_x.reshape(S, D).T, A_k_cache.reshape(Hkv, Sk, Dh), A_v_cache.reshape(Hkv, Sk, Dh),
      A_wq, A_wo.T, w_mod, B_w_gate, B_w_up, B_w_down.T)
    return out_t.T.reshape(B, S, D)
```
